```python
import os as _os
_os.environ.setdefault("JAX_PLATFORMS", "cpu")
import jax
import jax.numpy as jnp

def _softmax(x, axis=-1):
    return jax.nn.softmax(x, axis=axis)
def _gelu(x):
    return jax.nn.gelu(x, approximate=True)
def _silu(x):
    return jax.nn.silu(x)
def _sigmoid(x):
    return jax.nn.sigmoid(x)
def _layernorm(x, axis=-1, eps=1e-5):
    m = jnp.mean(x, axis=axis, keepdims=True)
    v = jnp.var(x, axis=axis, keepdims=True)
    return (x - m) / jnp.sqrt(v + eps)
def _scatter_add(tgt, idx, src, axis=0):
    return tgt.at[idx].add(src)
def _segment_sum(src, seg, n):
    return jax.ops.segment_sum(src, seg, n)
class _Rng:
    def __init__(self, key):
        self._k = key
    def _next(self):
        self._k, sub = jax.random.split(self._k)
        return sub
    def normal(self, shape):
        return jax.random.normal(self._next(), shape, dtype=jnp.bfloat16)
    def randint(self, lo, hi, shape):
        return jax.random.randint(self._next(), shape, lo, hi, dtype=jnp.int32)
    def uniform(self, shape, lo=0.0, hi=1.0):
        return jax.random.uniform(self._next(), shape, jnp.bfloat16, lo, hi)
    def permutation(self, n):
        return jax.random.permutation(self._next(), n)


kernel_name = 'parallel_sum__sliding_local_dilated__geglu_ffn__prompt'

def setup_inputs():
    _rng = _Rng(jax.random.key(int.from_bytes(__import__("os").urandom(4), "little")))
    _w = (lambda a: (lambda t: t.astype(jnp.bfloat16) if jnp.issubdtype(t.dtype, jnp.floating) else t)(jnp.asarray(a)))
    def _A_setup():
        B, S, D = 1, 2048, 640
        return {
            "x": _w((lambda *s: _rng.normal(s) * 0.05)(B, S, D)),
            "wqkv": _w((lambda *s: _rng.normal(s) * 0.05)(D, 3 * D)),
            "wo": _w((lambda *s: _rng.normal(s) * 0.05)(D, D)),
        }
    _A_in = _A_setup()

    def _B_setup():
        B, S, D, F = 1, 2048, 640, 1728
        return {
            "x": _w((lambda *s: _rng.normal(s) * 0.05)(B, S, D)),
            "w_gate": _w((lambda *s: _rng.normal(s) * 0.05)(D, F)),
            "w_up": _w((lambda *s: _rng.normal(s) * 0.05)(D, F)),
            "w_down": _w((lambda *s: _rng.normal(s) * 0.05)(F, D)),
        }
    _B_in = _B_setup()

    return {
        "A_x": _A_in["x"],
        "A_wqkv": _A_in["wqkv"],
        "A_wo": _A_in["wo"],
        "B_x": _B_in["x"],
        "B_w_gate": _B_in["w_gate"],
        "B_w_up": _B_in["w_up"],
        "B_w_down": _B_in["w_down"],
    }

def reference(A_x, A_wqkv, A_wo, B_x, B_w_gate, B_w_up, B_w_down):
    def _A_ref(x, wqkv, wo):
        B, S, D = x.shape
        H = 32; Dh = D // H
        W, dil = 8, 2
        qkv = (lambda x, *d: x.transpose(*d))((x @ wqkv).reshape(B, S, 3, H, Dh), 2, 0, 3, 1, 4)
        q, k, v = qkv[0], qkv[1], qkv[2]
        scale = Dh ** -0.5
        pos = jnp.arange(S)
        off = jnp.arange(W) * dil
        idx = pos[:, None] - off[None, :]
        mask = idx >= 0
        idx_c = jnp.where(mask, idx, 0).reshape(-1)
        kg = k[:, :, idx_c, :].reshape(B, H, S, W, Dh)
        vg = v[:, :, idx_c, :].reshape(B, H, S, W, Dh)
        logits = jnp.einsum("bhsd,bhswd->bhsw", q, kg) * scale
        logits = jnp.where(mask[None, None, :, :], logits, -1e9)
        attn = _softmax(logits, axis=-1)
        o = jnp.einsum("bhsw,bhswd->bhsd", attn, vg)
        return (lambda x, *d: x.transpose(*d))(o, 0, 2, 1, 3).reshape(B, S, D) @ wo

    def _B_ref(x, w_gate, w_up, w_down):
        return (_gelu(x @ w_gate) * (x @ w_up)) @ w_down

    x = A_x
    xn = _layernorm(x, axis=-1)
    return x + _A_ref(xn, A_wqkv, A_wo) + _B_ref(xn, B_w_gate, B_w_up, B_w_down)
```

```python
import functools
import os
import jax
import jax.numpy as jnp
import jax.experimental.pallas as pl
import jax.experimental.pallas.tpu as pltpu

S, D, H, DH, W, DIL, F = 2048, 640, 32, 20, 8, 2, 1728
TM = int(os.environ.get('TM', 256))
NB = S // TM
HALO = int(os.environ.get('HALO', 64))
NJ = D // 128
LOG2E = 1.4426950408889634
FM = 1664
FC = 256
F_CHUNKS = [(c, min(FC, FM - c)) for c in range(0, FM, FC)]
RC = int(os.environ.get('RC', 16))
GATE = int(os.environ.get('GATE', 0))
LC = int(os.environ.get('LC', 32))
INTER = int(os.environ.get('INTER', 1))
SCOPES = int(os.environ.get('SCOPES', 0))
BF = jnp.bfloat16
F32 = jnp.float32
NT = (((1,), (1,)), ((), ()))

import contextlib
def scope(name):
    return jax.named_scope(name) if SCOPES else contextlib.nullcontext()


def _gelu_mul(g, u):
    c0 = 0.7978845608028654
    c1 = c0 * 0.044715
    t = jnp.tanh(g * (c0 + c1 * (g * g)))
    hg = 0.5 * g
    return (hg + hg * t) * u


def _kernel(x_hbm, wqkv_hbm, wo_hbm, wg_hbm, wu_hbm, wd_hbm, out_hbm,
            x_s, xn_s, out_s, wqkv_r, wqkv_p, wo_r, wo_f, wo_p, wg_s, wu_s, wt_s, wd_s,
            q_s, k_s, v_s, h_s, a_s, zero_s, sem_x, sem_o, sem_w):
    ncf = len(F_CHUNKS)

    def cp_x(b):
        return pltpu.make_async_copy(x_hbm.at[pl.ds(b * TM, TM)], x_s.at[pl.ds(b * TM, TM)], sem_w.at[2 * len(F_CHUNKS) + 5 + b])

    def cp_o(b):
        return pltpu.make_async_copy(out_s.at[pl.ds(b * TM, TM)], out_hbm.at[pl.ds(b * TM, TM)], sem_o.at[b])

    cp_g = [pltpu.make_async_copy(wg_hbm.at[pl.ds(c, n)], wg_s.at[pl.ds(c, n)], sem_w.at[i])
            for i, (c, n) in enumerate(F_CHUNKS)]
    cp_u = [pltpu.make_async_copy(wu_hbm.at[pl.ds(c, n)], wu_s.at[pl.ds(c, n)], sem_w.at[ncf + i])
            for i, (c, n) in enumerate(F_CHUNKS)]
    cp_tg = pltpu.make_async_copy(wg_hbm.at[pl.ds(FM, 64)], wt_s.at[pl.ds(0, 64)], sem_w.at[2 * ncf])
    cp_tu = pltpu.make_async_copy(wu_hbm.at[pl.ds(FM, 64)], wt_s.at[pl.ds(64, 64)], sem_w.at[2 * ncf + 1])
    cp_qkv = pltpu.make_async_copy(wqkv_hbm, wqkv_r, sem_w.at[2 * ncf + 2])
    cp_wo = pltpu.make_async_copy(wo_hbm, wo_r, sem_w.at[2 * ncf + 3])
    cp_wd = pltpu.make_async_copy(wd_hbm, wd_s, sem_w.at[2 * ncf + 4])

    def permute_qkv():
        lane = jax.lax.broadcasted_iota(jnp.int32, (32, 128), 1)
        l5 = lane % 5
        masks = [l5 == r for r in range(5)]
        hh = lane % H
        gg = lane // H
        idx = [(DH * hh + 5 * gg + j) % 128 for j in range(NJ)]
        for t in range(3):
            for r0 in range(0, D, 64):
                src = [pltpu.bitcast(wqkv_r[r0:r0 + 64, t * D + s * 128:t * D + (s + 1) * 128], jnp.uint32)
                       for s in range(NJ)]
                for j in range(NJ):
                    mg = src[4]
                    for s in range(3, -1, -1):
                        mg = jnp.where(masks[(j - 3 * s) % 5], src[s], mg)
                    res = jnp.take_along_axis(mg, idx[j], axis=1, mode="promise_in_bounds")
                    wqkv_p[r0:r0 + 64, t * D + j * 128:t * D + (j + 1) * 128] = pltpu.bitcast(res, BF)

    def permute_wo():
        for jj in range(NJ):
            wo_f[jj] = wo_r[:, jj * 128:(jj + 1) * 128].astype(F32)
        for jj in range(NJ):
            for j in range(NJ):
                for g in range(4):
                    rows = wo_f[jj, pl.ds(5 * g + j, H, stride=DH), :]
                    wo_p[j * 128 + g * H:j * 128 + (g + 1) * H, jj * 128:(jj + 1) * 128] = rows.astype(BF)

    def ln_chunk(base, r0):
        x = x_s[pl.ds(base + r0, LC), :].astype(F32)
        m = jnp.mean(x, axis=-1, keepdims=True)
        xc = x - m
        var = jnp.mean(xc * xc, axis=-1, keepdims=True)
        xn = (xc * jax.lax.rsqrt(var + 1e-5)).astype(BF)
        xn_s[pl.ds(base + r0, LC), :] = xn
        u = pltpu.bitcast(xn, jnp.uint32)
        tok = None
        for r in range(0, LC // 2, 8):
            for j in range(NJ):
                p = u[r:r + 8, j * 128:(j + 1) * 128]
                tok = p if tok is None else tok | p
        return tok

    def layernorm(base):
        for r0 in range(0, TM, LC):
            ln_chunk(base, r0)

    def gated(ref, r0, n, gates):
        if not gates:
            return ref[r0:r0 + n, :]
        true8 = jax.lax.broadcasted_iota(jnp.int32, (8, 128), 1) >= zero_s[0]
        ncol = ref.shape[1]
        gates = sorted(gates, key=lambda g: g[0])
        rows = []
        cur = 0
        for (gr, gc, tok) in gates:
            if gr > cur:
                rows.append(ref[r0 + cur:r0 + gr, :])
            piece = pltpu.bitcast(ref[r0 + gr:r0 + gr + 16, gc:gc + 128], jnp.uint32)
            piece = pltpu.bitcast(jnp.where(true8, piece, tok), BF)
            cols = []
            if gc > 0:
                cols.append(ref[r0 + gr:r0 + gr + 16, 0:gc])
            cols.append(piece)
            if gc + 128 < ncol:
                cols.append(ref[r0 + gr:r0 + gr + 16, gc + 128:ncol])
            rows.append(jnp.concatenate(cols, axis=1))
            cur = gr + 16
        if cur < n:
            rows.append(ref[r0 + cur:r0 + n, :])
        return jnp.concatenate(rows, axis=0)

    def step(b, first):
        base = b * TM if first else pl.multiple_of(b * TM, TM)
        if first:
            nbase = TM
        else:
            nbase = pl.multiple_of(jnp.minimum(b + 1, NB - 1) * TM, TM)
        xn = xn_s[pl.ds(base, TM), :]
        true_vec = jax.lax.broadcasted_iota(jnp.int32, (RC, 128), 1) >= zero_s[0]

        def ffn_chunk(i, gg=(), gu=()):
            if i < ncf:
                c, n = F_CHUNKS[i]
                if first:
                    with scope('waitgu'):
                        cp_g[i].wait()
                        cp_u[i].wait()
                g = jax.lax.dot_general(xn, gated(wg_s, c, n, gg), NT, preferred_element_type=F32)
                u = jax.lax.dot_general(xn, gated(wu_s, c, n, gu), NT, preferred_element_type=F32)
                h_s[:, c:c + n] = _gelu_mul(g, u).astype(BF)
            else:
                if first:
                    cp_tg.wait()
                    cp_tu.wait()
                t = jax.lax.dot_general(xn, gated(wt_s, 0, 128, gg), NT, preferred_element_type=F32)
                ht = _gelu_mul(t, pltpu.roll(t, 64, 1))
                h_s[:, FM:F] = ht[:, 0:64].astype(BF)

        def qkv_proj():
            qkv = jnp.dot(xn, wqkv_p[...], preferred_element_type=F32)
            for j in range(NJ):
                q_s[j] = qkv[:, j * 128:(j + 1) * 128]
                k_s[j, pl.ds(base + HALO, TM), :] = qkv[:, D + j * 128:D + (j + 1) * 128]
                v_s[j, pl.ds(base + HALO, TM), :] = qkv[:, 2 * D + j * 128:2 * D + (j + 1) * 128]

        def attn_chunk(rc, token):
            scale = DH ** -0.5
            r0 = rc * RC
            q = [q_s[j, r0:r0 + RC, :] for j in range(NJ)]
            if token is not None:
                q = [jnp.where(true_vec, qq, token) for qq in q]
            logits = []
            for w in range(W):
                st = base + (HALO + r0 - DIL * w)
                acc = q[0] * k_s[0, pl.ds(st, RC), :]
                for j in range(1, NJ):
                    acc = acc + q[j] * k_s[j, pl.ds(st, RC), :]
                acc = acc + pltpu.roll(acc, 64, 1)
                acc = acc + pltpu.roll(acc, 32, 1)
                if first and r0 < DIL * w:
                    rows = r0 + jax.lax.broadcasted_iota(jnp.int32, (RC, 128), 0)
                    acc = jnp.where(rows >= DIL * w, acc, -1e9 / scale)
                logits.append(acc)
            mx = logits[0]
            for w in range(1, W):
                mx = jnp.maximum(mx, logits[w])
            ps = [jnp.exp2((l - mx) * (scale * LOG2E)) for l in logits]
            den = ps[0]
            for w in range(1, W):
                den = den + ps[w]
            inv = 1.0 / den
            last = None
            for j in range(NJ):
                acc = ps[0] * v_s[j, pl.ds(base + HALO + r0, RC), :]
                for w in range(1, W):
                    st = base + (HALO + r0 - DIL * w)
                    acc = acc + ps[w] * v_s[j, pl.ds(st, RC), :]
                res = (acc * inv).astype(BF)
                a_s[r0:r0 + RC, j * 128:(j + 1) * 128] = res
                p = pltpu.bitcast(res, jnp.uint32)
                last = p if last is None else last | p
            return last

        nrc = TM // RC
        if first:
            for i in range(ncf + 1):
                ffn_chunk(i)
            with scope('waitqkv'):
                cp_qkv.wait()
            permute_qkv()
            qkv_proj()
            with scope('waitwd'):
                cp_wd.wait()
                cp_wo.wait()
                cp_x(1).wait()
            permute_wo()
            for rc in range(nrc):
                attn_chunk(rc, None)
            layernorm(nbase)
            gd = []
        else:
            qkv_proj()
            toks = [attn_chunk(rc, None) for rc in range(nrc)]
            pts = []
            for i in range(1, ncf):
                n = F_CHUNKS[i][1]
                for which in range(2):
                    for r in range(0, n, 128):
                        pts.append((i, which, r, 0))
            sel = [pts[(k * len(pts)) // nrc] for k in range(nrc)]
            for i in range(ncf + 1):
                gg = [(r, c, toks[k]) for k, (ii, wh, r, c) in enumerate(sel) if ii == i and wh == 0]
                gu = [(r, c, toks[k]) for k, (ii, wh, r, c) in enumerate(sel) if ii == i and wh == 1]
                ffn_chunk(i, gg, gu)
            lt = [ln_chunk(nbase, r0) for r0 in range(0, TM, LC)]
            gd = [(128 * (k + 2), 0, t) for k, t in enumerate(lt)]
        ffn = jnp.dot(h_s[...], gated(wd_s, 0, F, gd), preferred_element_type=F32)
        att = jnp.dot(a_s[...], wo_p[...], preferred_element_type=F32)
        x = x_s[pl.ds(base, TM), :].astype(F32)
        out_s[pl.ds(base, TM), :] = (x + att + ffn).astype(BF)
        cp_o(b).start()

    cp_x(0).start()
    for i in range(ncf):
        cp_g[i].start()
        cp_u[i].start()
    cp_tg.start()
    cp_tu.start()
    cp_qkv.start()
    cp_wd.start()
    cp_wo.start()
    for b in range(1, NB):
        cp_x(b).start()
    zero_s[0] = 0
    k_s[:, 0:HALO, :] = jnp.zeros((NJ, HALO, 128), F32)
    v_s[:, 0:HALO, :] = jnp.zeros((NJ, HALO, 128), F32)

    with scope('waitx'):
        cp_x(0).wait()
    layernorm(0)
    with scope('step0'):
        step(0, True)
    for b in range(2, NB):
        cp_x(b).wait()

    def body(b, carry):
        with scope('stepb'):
            step(b, False)
        return carry
    jax.lax.fori_loop(1, NB, body, 0)

    with scope('waitout'):
        for b in range(NB):
            cp_o(b).wait()


@jax.jit
def pallas_parallel_sum__sliding_local_dilated__geglu_ffn__prompt_kernel(
    A_x, A_wqkv, A_wo, B_x, B_w_gate, B_w_up, B_w_down,
):
    x = A_x.reshape(S, D)
    hbm = pl.BlockSpec(memory_space=pltpu.MemorySpace.HBM)
    ncf = len(F_CHUNKS)
    out = pl.pallas_call(
        _kernel,
        in_specs=[hbm] * 6,
        out_specs=hbm,
        out_shape=jax.ShapeDtypeStruct((S, D), BF),
        scratch_shapes=[
            pltpu.VMEM((S, D), BF),
            pltpu.VMEM((S, D), BF),
            pltpu.VMEM((S, D), BF),
            pltpu.VMEM((D, 3 * D), BF),
            pltpu.VMEM((D, 3 * D), BF),
            pltpu.VMEM((D, D), BF),
            pltpu.VMEM((NJ, D, 128), F32),
            pltpu.VMEM((D, D), BF),
            pltpu.VMEM((FM, D), BF),
            pltpu.VMEM((FM, D), BF),
            pltpu.VMEM((128, D), BF),
            pltpu.VMEM((F, D), BF),
            pltpu.VMEM((NJ, TM, 128), F32),
            pltpu.VMEM((NJ, S + HALO, 128), F32),
            pltpu.VMEM((NJ, S + HALO, 128), F32),
            pltpu.VMEM((TM, F), BF),
            pltpu.VMEM((TM, D), BF),
            pltpu.SMEM((1,), jnp.int32),
            pltpu.SemaphoreType.DMA((NB,)),
            pltpu.SemaphoreType.DMA((NB,)),
            pltpu.SemaphoreType.DMA((2 * ncf + 5 + NB,)),
        ],
        compiler_params=pltpu.CompilerParams(
            vmem_limit_bytes=100 * 1024 * 1024,
            disable_bounds_checks=True, disable_semaphore_checks=True,
        ),
    )(x, A_wqkv, A_wo, B_w_gate.T, B_w_up.T, B_w_down)
    return out.reshape(1, S, D)
```

```python
import contextlib
import functools
import os
import jax
import jax.numpy as jnp
import jax.experimental.pallas as pl
import jax.experimental.pallas.tpu as pltpu

S, D, H, DH, W, DIL, F = 2048, 640, 32, 20, 8, 2, 1728
TM0 = int(os.environ.get('TM0', 384))
NL = int(os.environ.get('NL', 4))
TM1 = (S - TM0) // NL
assert TM0 + NL * TM1 == S and TM1 % 32 == 0 and TM0 % 64 == 0
HM1 = TM1 // 2
HP = HM1 // 2
TMX = max(TM0, TM1)
TMP = (TMX + 63) // 64 * 64
HALO = 16
NJ = D // 128
LOG2E = 1.4426950408889634
FM = 1664
FP = 1792
FH = FP // 2
G_EARLY = [[0], [7, 1], [8, 2, 9]]
G_Q, G_KV, G_R, G_D = [3], [10], [4, 11, 5, 12], [6]
RC = 16
LC = 16
SCOPES = int(os.environ.get('SCOPES', 0))
LN4 = float(os.environ.get('LN4', 2))
LNSPAN = float(os.environ.get('LNSPAN', 28))
NA2 = int(os.environ.get('NA2', 7))
A2SPAN = float(os.environ.get('A2SPAN', 9))
X1SEG = int(os.environ.get('X1SEG', 0))
NAR = int(os.environ.get('NAR', 9))
DSPAN = float(os.environ.get('DSPAN', 16))
GJ = int(os.environ.get('GJ', 2))
NOGATE = int(os.environ.get('NOGATE', 53))
S0S = int(os.environ.get('S0S', 1))
NAA = int(os.environ.get('NAA', 5))
NAB = int(os.environ.get('NAB', 8))
SPANC = float(os.environ.get('SPANC', 4))
WOSEG = int(os.environ.get('WOSEG', 1))
NPD = int(os.environ.get('NPD', 0))
NPRE = int(os.environ.get('NPRE', 2))
NPRER = int(os.environ.get('NPRER', 0))
HTRIG = int(os.environ.get('HTRIG', 0))
SPANA = float(os.environ.get('SPANA', 9))
XSPLIT = 2
BF = jnp.bfloat16
F32 = jnp.float32
U32 = jnp.uint32
NT = (((1,), (1,)), ((), ()))
P = functools.partial


def scope(name):
    return jax.named_scope(name) if SCOPES else contextlib.nullcontext()


def _gelu_mul(g, u):
    c0 = 0.7978845608028654
    c1 = c0 * 0.044715
    t = jnp.tanh(g * (c0 + c1 * (g * g)))
    hg = 0.5 * g
    return (hg + hg * t) * u


def _pack(x):
    return pltpu.bitcast(x.astype(BF), U32)


def _unpack(u):
    return pltpu.bitcast(u, BF)


def _lhs_sums(a11, a12, a21, a22):
    return [a11 + a22, a21 + a22, a11 + a12, a21 - a11, a12 - a22]


def _rhs_sums(b11, b12, b21, b22):
    return [b11 + b22, b12 - b22, b21 - b11, b11 + b12, b21 + b22]


LS = {1: 0, 2: 1, 5: 2, 6: 3, 7: 4}
RS = {1: 0, 3: 1, 4: 2, 6: 3, 7: 4}


def _nn(a, b):
    return jnp.dot(a, b, preferred_element_type=F32)


def _nt(a, b):
    return jax.lax.dot_general(a, b, NT, preferred_element_type=F32)


def _weave(*lists):
    items = []
    for lst in lists:
        items += [((k + 0.5) / len(lst), w) for k, w in enumerate(lst)]
    items.sort(key=lambda t: t[0])
    return [t[1] for t in items]


def _kernel(x_hbm, wqkv_hbm, wo_hbm, wg_hbm, wu_hbm, wd_hbm, out_hbm,
            x_s, xn_s, xs_s, xn2_s, xs2_s, out_s, wqkv_r, wqkv_p, wo_r, wo_f, wo_p,
            wg_s, wu_s, wt_s, wd_s, tq_s, tg_s, td_s, to_s, q_s, k_s, v_s, h_s, a_s,
            zero_s, sem_i, sem_o):

    def zrow():
        return pl.multiple_of(zero_s[0] * 8, 8)

    def after(val, trig):
        if trig is None:
            return val
        n = val.shape[0] // 8
        t = pltpu.bitcast(trig, val.dtype) if trig.dtype != val.dtype else trig
        if n > 1:
            t = jnp.concatenate([t] * n, axis=0)
        keep = jax.lax.broadcasted_iota(jnp.int32, val.shape, 1) >= zero_s[0]
        return jnp.where(keep, val, t)

    def after_head(val, trig):
        if trig is None:
            return val
        if val.shape[1] == 128:
            return after(val, trig)
        return jnp.concatenate([after(val[:, 0:128], trig), val[:, 128:]], axis=1)

    toks = []
    gate_no = [-1]

    def note(ref, row):
        if all(r is not ref for r, _ in toks):
            toks.append((ref, row))

    def gate(lhs):
        if not toks:
            return lhs
        gate_no[0] += 1
        if (NOGATE >> gate_no[0]) & 1:
            del toks[:]
            return lhs
        tok = functools.reduce(lambda p, q: p | q, [ref[pl.ds(zrow() + row, 8), 0:128] for ref, row in toks])
        del toks[:]
        u = pltpu.bitcast(lhs[0:16], U32)
        return jnp.concatenate([_unpack(after_head(u, tok)), lhs[16:]], axis=0)

    credit = [0.0]

    def fire(work, res, per_col=1):
        tm = res.shape[0]
        if not work:
            credit[0] = 0.0
        for c in range(0, res.shape[1], 128):
            pos = credit[0]
            while pos < 1.0 and work:
                r = int((tm - 8) * pos) // 8 * 8
                work.pop(0)(res[r:r + 8, c:c + 128])
                pos += 1.0 / per_col
            credit[0] = max(pos - 1.0, 0.0)

    lane = jax.lax.broadcasted_iota(jnp.int32, (32, 128), 1)
    l5 = lane % 5
    masks = [l5 == r for r in range(5)]
    idx = [(DH * (lane % H) + 5 * (lane // H) + j) % 128 for j in range(NJ)]

    def permute_qkv(t, r0, trig):
        src = [pltpu.bitcast(wqkv_r[r0:r0 + 64, t * D + s * 128:t * D + (s + 1) * 128], U32)
               for s in range(NJ)]
        src[4] = after(src[4], trig)
        for j in range(NJ):
            mg = src[4]
            for s in range(3, -1, -1):
                mg = jnp.where(masks[(j - 3 * s) % 5], src[s], mg)
            res = jnp.take_along_axis(mg, idx[j], axis=1, mode="promise_in_bounds")
            wqkv_p[r0 // 2:r0 // 2 + 32, t * D + j * 128:t * D + (j + 1) * 128] = res

    def permute_wo(jj, trig):
        w = after(pltpu.bitcast(wo_r[:, jj * 128:(jj + 1) * 128], U32), trig)
        wo_f[jj] = _unpack(w).astype(F32)
        for j in range(NJ):
            for g in range(4):
                rows = wo_f[jj, pl.ds(5 * g + j, H, stride=DH), :]
                r0 = (j * 128 + g * H) // 2
                wo_p[r0:r0 + H // 2, jj * 128:(jj + 1) * 128] = _pack(rows)

    def prep(b11, b12, b21, b22, store, trig):
        b11, b12, b21, b22 = [b.astype(F32) for b in (b11, b12, b21, b22)]
        b11 = after(b11, trig)
        b22 = after(b22, trig)
        for i, s in enumerate(_rhs_sums(b11, b12, b21, b22)):
            store(i, _pack(s))

    def prep_gu(which, p, r0, kc, trig):
        ref = (wg_s, wu_s)[which]
        ra, rb = p * 128 + r0, (p + 7) * 128 + r0

        def store(i, o):
            row = ((which * 6 + p) * 5 + i) * 64 + r0 // 2
            tg_s[row:row + 32, kc:kc + 128] = o
            if kc == 0:
                note(tg_s, row)
        prep(ref[ra:ra + 64, kc:kc + 128], ref[rb:rb + 64, kc:kc + 128],
             ref[ra:ra + 64, 256 + kc:384 + kc], ref[rb:rb + 64, 256 + kc:384 + kc], store, trig)

    def prep_q(p, r0, trig):
        ca, cb = p * 128, (p + 7) * 128

        def store(i, o):
            row = (p * 5 + i) * 128 + r0
            tq_s[row:row + 32, :] = o
            note(tq_s, row)
        prep(_unpack(wqkv_p[r0:r0 + 32, ca:ca + 128]), _unpack(wqkv_p[r0:r0 + 32, cb:cb + 128]),
             _unpack(wqkv_p[128 + r0:160 + r0, ca:ca + 128]), _unpack(wqkv_p[128 + r0:160 + r0, cb:cb + 128]),
             store, trig)

    def prep_d(r0, c, trig):
        def store(i, o):
            row = i * (FH // 2) + r0 // 2
            td_s[row:row + 32, c:c + 128] = o
            if c == 0:
                note(td_s, row)
        prep(wd_s[r0:r0 + 64, c:c + 128], wd_s[r0:r0 + 64, 256 + c:384 + c],
             wd_s[FH + r0:FH + r0 + 64, c:c + 128], wd_s[FH + r0:FH + r0 + 64, 256 + c:384 + c], store, trig)

    def prep_o(r0, c, trig):
        def store(i, o):
            row = i * 128 + r0
            to_s[row:row + 32, c:c + 128] = o
            if c == 0:
                note(to_s, row)
        prep(_unpack(wo_p[r0:r0 + 32, c:c + 128]), _unpack(wo_p[r0:r0 + 32, 256 + c:384 + c]),
             _unpack(wo_p[128 + r0:160 + r0, c:c + 128]), _unpack(wo_p[128 + r0:160 + r0, 256 + c:384 + c]),
             store, trig)

    def ln_rows(blk, r0, trig=None):
        x = after_head(x_s[blk, r0:r0 + LC, :].astype(F32), trig)
        m = jnp.mean(x, axis=-1, keepdims=True)
        xc = x - m
        var = jnp.mean(xc * xc, axis=-1, keepdims=True)
        return xc * jax.lax.rsqrt(var + 1e-5)

    def ln_pair(blk, r0, xn_d, xs_d, trig):
        top = ln_rows(blk, r0, trig)
        bot = ln_rows(blk, HM1 + r0, trig)
        xn_d[r0 // 2:(r0 + LC) // 2, :] = _pack(top)
        xn_d[(HM1 + r0) // 2:(HM1 + r0 + LC) // 2, :] = _pack(bot)
        for i, s in enumerate(_lhs_sums(top[:, 0:256], top[:, 256:512], bot[:, 0:256], bot[:, 256:512])):
            xs_d[i * HP + r0 // 2:i * HP + (r0 + LC) // 2, :] = _pack(s)
        note(xn_d, r0 // 2)
        note(xs_d, r0 // 2)

    def tail_h(t):
        ht = _gelu_mul(t, pltpu.roll(t, 64, 1))
        lo = jax.lax.broadcasted_iota(jnp.int32, ht.shape, 1) < 64
        return jnp.where(lo, ht, 0.0)

    def store_qkv(c, row0, val):
        t, j = divmod(c, NJ)
        n = val.shape[0]
        if t == 0:
            q_s[j, row0:row0 + n, :] = val * (DH ** -0.5 * LOG2E)
        elif t == 1:
            k_s[j, HALO + row0:HALO + row0 + n, :] = val
        else:
            v_s[j, HALO + row0:HALO + row0 + n, :] = val

    def attn_core(r0, first, trig):
        q = [after(q_s[j, r0:r0 + 8, :], trig) for j in range(NJ)]
        logits = []
        for w in range(W):
            st = HALO + r0 - DIL * w
            acc = q[0] * k_s[0, st:st + 8, :]
            for j in range(1, NJ):
                acc = acc + q[j] * k_s[j, st:st + 8, :]
            acc = acc + pltpu.roll(acc, 64, 1)
            acc = acc + pltpu.roll(acc, 32, 1)
            if first and r0 < DIL * w:
                rows = r0 + jax.lax.broadcasted_iota(jnp.int32, (8, 128), 0)
                acc = jnp.where(rows >= DIL * w, acc, -1e9 * LOG2E)
            logits.append(acc)
        mx = logits[0]
        for w in range(1, W):
            mx = jnp.maximum(mx, logits[w])
        ps = [jnp.exp2(l - mx) for l in logits]
        den = ps[0]
        for w in range(1, W):
            den = den + ps[w]
        r = pl.reciprocal(den, approx=True)
        inv = r * (2.0 - den * r)
        outs = []
        for j in range(NJ):
            acc = ps[0] * v_s[j, HALO + r0:HALO + r0 + 8, :]
            for w in range(1, W):
                st = HALO + r0 - DIL * w
                acc = acc + ps[w] * v_s[j, st:st + 8, :]
            outs.append(acc * inv)
        return outs, mx

    def attn_rows(r0, first, trig):
        o1, t1 = attn_core(r0, first, trig)
        o2, _ = attn_core(r0 + 8, first, t1)
        for j in range(NJ):
            a_s[r0 // 2:(r0 + RC) // 2, j * 128:(j + 1) * 128] = _pack(jnp.concatenate([o1[j], o2[j]], axis=0))

    def roll_halo(tm):
        k_s[:, 0:HALO, :] = k_s[:, tm:tm + HALO, :]
        v_s[:, 0:HALO, :] = v_s[:, tm:tm + HALO, :]

    def cp_o(blk, base, r0, n, j):
        return pltpu.make_async_copy(out_s.at[blk, pl.ds(r0, n), pl.ds(j * 128, 128)],
                                     out_hbm.at[pl.ds(base + r0, n), pl.ds(j * 128, 128)], sem_o.at[0])

    def emit(blk, base, r0, j, val):
        n = val.shape[0]
        x = x_s[blk, r0:r0 + n, j * 128:(j + 1) * 128].astype(F32)
        out_s[blk, r0:r0 + n, j * 128:(j + 1) * 128] = (x + val).astype(BF)
        cp_o(blk, base, r0, n, j).start()

    def strassen(prod, left, work, per):
        def p(i):
            m = prod(i)
            fire(work, m, per)
            return m
        if left is None:
            m4 = p(4)
            m2 = p(2)
            m1 = p(1)
            t11 = m1 + m4
            t22 = m1 - m2
            m3 = p(3)
            m5 = p(5)
            return t11 - m5 + p(7), m3 + m5, m4 + m2, t22 + m3 + p(6)
        l21 = left(1, 0)
        m4 = p(4)
        m2 = p(2)
        c21 = l21 + m4 + m2
        m1 = p(1)
        t11 = m1 + m4
        t22 = m1 - m2
        m3 = p(3)
        m5 = p(5)
        c12 = m3 + m5 + left(0, 1)
        c11 = t11 - m5 + p(7) + left(0, 0)
        c22 = t22 + m3 + p(6) + left(1, 1)
        return c11, c12, c21, c22

    def stage2(blk, base, tm, works, pers):
        hm, hp = tm // 2, tm // 4

        def half(ref, r, c0, c1):
            return _unpack(ref[r * hp:(r + 1) * hp, c0:c1])

        memo = {}

        def lhs(plain, kh, i):
            if i == 3:
                return half(plain, 0, 0, kh)
            if i == 4:
                return half(plain, 1, kh, 2 * kh)
            if (kh, i) not in memo:
                def b(r, c):
                    return _unpack(plain[pl.ds(zrow(), 2 * hp), c * kh:(c + 1) * kh][r * hp:(r + 1) * hp]).astype(F32)
                s = {1: lambda: b(0, 0) + b(1, 1), 2: lambda: b(1, 0) + b(1, 1), 5: lambda: b(0, 0) + b(0, 1),
                     6: lambda: b(1, 0) - b(0, 0), 7: lambda: b(0, 1) - b(1, 1)}[i]()
                memo[(kh, i)] = s.astype(BF)
            return memo[(kh, i)]

        f4 = []
        for r in range(2):
            if works[0] is works[1]:
                f = _nn(half(h_s, r, 0, FP), wd_s[:, 512:D])
                fire(works[0], f, pers[0])
            else:
                f = None
                for k0 in range(0, FP, 512):
                    k1 = min(k0 + 512, FP)
                    part = _nn(half(h_s, r, k0, k1), wd_s[k0:k1, 512:D])
                    fire(works[0], part, pers[0])
                    f = part if f is None else f + part
            f4.append(f)
        ffn = []
        for c in range(2):
            assert works[c] is works[c + 1] or not works[c]
            if c == 0 or works[1] is not works[2]:
                credit[0] = 0.0
            cs = (c * 128, 256 + c * 128)

            def prod(i):
                if i == 2:
                    wd = wd_s[0:FH, cs[0]:cs[0] + 128]
                elif i == 5:
                    wd = wd_s[FH:FP, cs[1]:cs[1] + 128]
                else:
                    wd = _unpack(td_s[RS[i] * (FH // 2):(RS[i] + 1) * (FH // 2), cs[0]:cs[0] + 128])
                return _nn(lhs(h_s, FH, i), wd)
            ffn.append(strassen(prod, None, works[c + 1], pers[c + 1]))
        assert not works[2]
        roll_halo(tm)
        for r in range(2):
            emit(blk, base, r * hm, 4, f4[r] + _nn(gate(half(a_s, r, 0, D)), _unpack(wo_p[:, 512:D])))
        for c in range(2):
            cs = (c * 128, 256 + c * 128)

            def prod(i):
                if i == 2:
                    wo = wo_p[0:128, cs[0]:cs[0] + 128]
                elif i == 5:
                    wo = wo_p[128:256, cs[1]:cs[1] + 128]
                else:
                    wo = to_s[RS[i] * 128:(RS[i] + 1) * 128, cs[0]:cs[0] + 128]
                return _nn(lhs(a_s, 256, i), _unpack(wo))

            def left(r, cc):
                return ffn[c][2 * r + cc] + _nn(half(a_s, r, 512, D), _unpack(wo_p[256:320, cs[cc]:cs[cc] + 128]))
            c11, c12, c21, c22 = strassen(prod, left, None, 1)
            emit(blk, base, hm, c, c21)
            emit(blk, base, 0, c + 2, c12)
            emit(blk, base, 0, c, c11)
            emit(blk, base, hm, c + 2, c22)
        assert not toks

    def step(b):
        blk = b + 1
        base = pl.multiple_of(TM0 + b * TM1, 16)
        nblk = jnp.minimum(blk + 1, NL)

        def half(r, c0, c1):
            return _unpack(xn_s[r * HP:(r + 1) * HP, c0:c1])

        def lhs(i):
            if i == 3:
                return half(0, 0, 256)
            if i == 4:
                return half(1, 256, 512)
            return _unpack(xs_s[LS[i] * HP:(LS[i] + 1) * HP, :])

        work = [P(ln_pair, nblk, k * LC, xn2_s, xs2_s) for k in range(HM1 // LC)]
        per = len(work) / LNSPAN
        for r in range(2):
            store_qkv(14, r * HM1, _nn(half(r, 0, D), _unpack(wqkv_p[:, 14 * 128:15 * 128])))
        for p in range(7):
            cols = (p, p + 7)

            def prod(i):
                if i == 2:
                    w = wqkv_p[0:128, p * 128:(p + 1) * 128]
                elif i == 5:
                    w = wqkv_p[128:256, (p + 7) * 128:(p + 8) * 128]
                else:
                    w = tq_s[(p * 5 + RS[i]) * 128:(p * 5 + RS[i] + 1) * 128, :]
                return _nn(lhs(i), _unpack(w))

            def left(r, c):
                return _nn(half(r, 512, D), _unpack(wqkv_p[256:320, cols[c] * 128:(cols[c] + 1) * 128]))
            c11, c12, c21, c22 = strassen(prod, left, work, per)
            store_qkv(cols[0], 0, c11)
            store_qkv(cols[1], 0, c12)
            store_qkv(cols[0], HM1, c21)
            store_qkv(cols[1], HM1, c22)
        assert not work

        work = [P(attn_rows, c * RC + r * HM1, False) for c in range(HM1 // RC) for r in range(2)]
        per = (len(work) - 2 - NA2) / (12 * 7.0)

        def store_h(p, h11, h12, h21, h22):
            for r, c, v in ((0, p, h11), (0, p + 7, h12), (1, p, h21), (1, p + 7, h22)):
                h_s[r * HP:(r + 1) * HP, c * 128:(c + 1) * 128] = _pack(v)

        hh = []
        for r in range(2):
            xr = half(r, 0, D)
            g = _nt(xr, wg_s[6 * 128:7 * 128, :])
            fire(work, g, 1)
            u = _nt(xr, wu_s[6 * 128:7 * 128, :])
            t = _nt(gate(xr) if r == 1 else xr, wt_s[...])
            hh += [_gelu_mul(g, u), tail_h(t)]
        store_h(6, *hh)
        credit[0] = 0.0
        for p in range(6):
            res = []
            for which in range(2):
                ref = (wg_s, wu_s)[which]
                rows = (p * 128, (p + 7) * 128)

                def prod(i):
                    if i == 2:
                        w = ref[rows[0]:rows[0] + 128, 0:256]
                    elif i == 5:
                        w = ref[rows[1]:rows[1] + 128, 256:512]
                    else:
                        row = ((which * 6 + p) * 5 + RS[i]) * 64
                        w = _unpack(tg_s[row:row + 64, :])
                    return _nt(lhs(i), w)

                def left(r, c):
                    return _nt(half(r, 512, D), ref[rows[c]:rows[c] + 128, 512:D])
                res.append(strassen(prod, left, work, per))
            store_h(p, *[_gelu_mul(g, u) for g, u in zip(*res)])

        def copy_xn(dst, src, r0, trig):
            for c in range(0, dst.shape[1], 128):
                dst[r0:r0 + HP, c:c + 128] = after(src[pl.ds(zrow(), r0 + HP), c:c + 128][r0:r0 + HP], trig)
            note(dst, r0)
        copies = [P(copy_xn, xn_s, xn2_s, r) for r in (0, HP)]
        copies += [P(copy_xn, xs_s, xs2_s, i * HP) for i in range(5)]
        mixed = []
        while work or copies:
            if work:
                mixed.append(work.pop(0))
            if copies:
                mixed.append(copies.pop(0))
        per = max(len(mixed) - 2 * LN4, 1) / A2SPAN
        stage2(blk, base, TM1, [mixed] * 3, [LN4, per, per])

    def cp(src, dst, s):
        return pltpu.make_async_copy(src, dst, sem_i.at[s])

    def gu(groups, s):
        return [cp(h.at[pl.ds(g * 128, 128)], d.at[pl.ds(g * 128, 128)], s)
                for g in groups for h, d in ((wg_hbm, wg_s), (wu_hbm, wu_s))]

    HM = TM0 // 2
    QM = TM0 // 4
    XM = TM0 // XSPLIT

    def wcol(t, s):
        return cp(wqkv_hbm.at[:, pl.ds(t * D, D)], wqkv_r.at[:, pl.ds(t * D, D)], s)

    def xblk(b, s):
        return cp(x_hbm.at[pl.ds(TM0 + b * TM1, TM1)], x_s.at[b + 1, pl.ds(0, TM1)], s)

    cp_x0 = [cp(x_hbm.at[pl.ds(i * XM, XM)], x_s.at[0, pl.ds(i * XM, XM)], i) for i in range(XSPLIT)]
    s0 = XSPLIT
    cp_gu = [gu(g, s0 + k) for k, g in enumerate(G_EARLY)]
    s0 += len(G_EARLY)
    cp_q = gu(G_Q, s0) + [cp(wg_hbm.at[pl.ds(FM, 64)], wt_s.at[pl.ds(0, 64)], s0),
                          cp(wu_hbm.at[pl.ds(FM, 64)], wt_s.at[pl.ds(64, 64)], s0), wcol(0, s0)]
    cp_kv = gu(G_KV, s0 + 1) + [wcol(1, s0 + 1), wcol(2, s0 + 1)]
    cp_r = gu(G_R + G_D, s0 + 2) + [cp(wo_hbm, wo_r, s0 + 2)]
    cp_d = [cp(wd_hbm, wd_s.at[pl.ds(0, F)], s0 + 3)]
    [cp_q, cp_kv, cp_r, cp_d][X1SEG].append(xblk(0, s0 + X1SEG))
    cp_xs = [xblk(b, s0 + 4) for b in range(1, NL)]

    for c in cp_x0 + sum(cp_gu, []) + cp_q + cp_kv + cp_r + cp_d + cp_xs:
        c.start()
    zero_s[0] = 0
    k_s[:, 0:HALO, :] = jnp.zeros((NJ, HALO, 128), F32)
    v_s[:, 0:HALO, :] = jnp.zeros((NJ, HALO, 128), F32)
    wd_s[F:FP, :] = jnp.zeros((FP - F, D), BF)

    def first_block():
        def wait(cps, name):
            with scope(name):
                for c in cps:
                    c.wait()

        parts = []
        for i in range(XSPLIT):
            wait(cp_x0[i:i + 1], 'waitx')
            parts += [ln_rows(0, i * XM + k * LC).astype(BF) for k in range(XM // LC)]
        xn = jnp.concatenate(parts, axis=0)

        def head_trig():
            return pltpu.bitcast(xn[0:16, 0:128], U32) if HTRIG else None

        def ffn_group(x, row0, g0, work, per, last=False):
            g = _nt(x, wg_s[g0 * 128:(g0 + 1) * 128, :])
            fire(work, g, per)
            u = _nt(gate(x) if last else x, wu_s[g0 * 128:(g0 + 1) * 128, :])
            fire(work, u, per)
            h_s[row0 // 2:(row0 + x.shape[0]) // 2, g0 * 128:(g0 + 1) * 128] = _pack(_gelu_mul(g, u))

        def ffn_groups(groups, work=None, per=1, gate_last=False):
            groups = list(groups)
            if len(groups) % 2:
                g0 = groups.pop(0)
                ffn_group(xn[0:HM], 0, g0, work, per)
                ffn_group(xn[HM:], HM, g0, work, per, gate_last and not groups)
            for k, g0 in enumerate(groups):
                ffn_group(xn, 0, g0, work, per, gate_last and k == len(groups) - 1)

        have, done = set(), set()

        def new_pairs(groups):
            have.update(groups)
            pairs = [p for p in range(6) if p in have and p + 7 in have and p not in done]
            done.update(pairs)
            return [P(prep_gu, which, p, r0, kc)
                    for p in pairs for which in range(2) for r0 in (0, 64) for kc in (0, 128)]

        ln = [P(ln_pair, 1, k * LC, xn_s, xs_s) for k in range(HM1 // LC)]
        ln_at = lambda s: ln if s == X1SEG else []
        perm = [[P(permute_qkv, t, r0) for r0 in range(0, D, 64)] for t in range(3)]

        for cps, groups in zip(cp_gu, G_EARLY):
            wait(cps, 'waitgu')
            work = new_pairs(groups)
            nres = 2 * len(groups) + 2 * (len(groups) % 2)
            ffn_groups(groups, work, max(len(work), 1) / max(nres - 2.0, 1.0), True)
            assert not work and not toks

        wait(cp_q, 'waitq')
        wq = perm[0]
        for w_ in wq[0:3]:
            w_(None)
        wq = wq[3:]
        t = _nt(xn, wt_s[...])
        fire(wq, t, 4)
        h_s[0:TM0 // 2, FM:FP] = _pack(tail_h(t))
        for g0 in G_Q:
            ffn_group(xn, 0, g0, wq, 3)
        assert not wq
        work = new_pairs(G_Q) + ln_at(0)
        for j in range(NJ):
            r = _nn(gate(xn) if j == NJ - 1 else xn, _unpack(wqkv_p[:, j * 128:(j + 1) * 128]))
            fire(work, r, max(len(ln), 1) / 3.0)
            store_qkv(j, 0, r)
        assert not work and not toks

        wait(cp_kv, 'waitkv')
        wk = perm[1]
        for w_ in wk[0:4]:
            w_(None)
        wk = wk[4:]
        for g0 in G_KV:
            g = _nt(xn, wg_s[g0 * 128:(g0 + 1) * 128, :])
            fire(wk, g, 6)
            u = _nt(xn, wu_s[g0 * 128:(g0 + 1) * 128, :])
            h_s[0:TM0 // 2, g0 * 128:(g0 + 1) * 128] = _pack(_gelu_mul(g, u))
        assert not wk
        work = perm[2] + _weave(new_pairs(G_KV) + ln_at(1),
                                [P(prep_q, p, r0) for p in range(7) for r0 in range(0, 128, 32)])
        per = len(work) / 8.0
        fire(work, u, per)
        for c in range(NJ, 3 * NJ):
            r = _nn(gate(xn) if c == 3 * NJ - 1 else xn, _unpack(wqkv_p[:, c * 128:(c + 1) * 128]))
            fire(work, r, per)
            store_qkv(c, 0, r)
        assert not work and not toks

        wait(cp_r, 'waitr')
        att = [P(attn_rows, rc * RC, True) for rc in range(TM0 // RC)]
        wo_work = [P(permute_wo, jj) for jj in range(NJ)]
        side = new_pairs(G_R + G_D) + ln_at(2)
        if WOSEG == 0:
            side, wo_work = _weave(side, wo_work), []
        work = _weave(side, att[:NAR])
        att = att[NAR:]
        for _ in range(NPRER):
            work.pop(0)(head_trig())
        ffn_groups(G_R, work, len(work) / (2 * len(G_R) - 2.0), True)
        assert not work and not toks

        wait(cp_d, 'waitd')
        pd = [[P(prep_d, r0, c) for r0 in range(0, FH, 64)] for c in (0, 128)]
        po = [P(prep_o, r0, c) for r0 in range(0, 128, 32) for c in (0, 128)]
        if S0S:
            if WOSEG == 2:
                wa = _weave(pd[0] + pd[1][:NPD], wo_work, att[:NAA])
                wb = _weave(pd[1][NPD:] + po, att[NAA:NAA + NAB])
                wc = att[NAA + NAB:]
            else:
                wa = _weave(pd[0], att[:NAA])
                wb = _weave(wo_work + pd[1], att[NAA:NAA + NAB])
                wc = _weave(po, att[NAA + NAB:])
            for _ in range(NPRE):
                wa.pop(0)(head_trig())
            per = len(wa) / SPANA
            ffn_groups(G_D, wa, per)
            stage2(0, 0, TM0, [wa, wb, wc], [per, len(wb) / 6.0, max(len(wc), 1) / SPANC])
            return
        work = _weave(wo_work + ln_at(3) + _weave(*pd) + po, att)
        per = len(work) / DSPAN
        for g0 in G_D:
            ffn_group(xn, 0, g0, work, per)
        cols = []
        for j in range(NJ):
            acc = None
            for k0 in range(0, FP, 512):
                k1 = min(k0 + 512, FP)
                part = _nn(_unpack(h_s[0:TM0 // 2, k0:k1]), wd_s[k0:k1, j * 128:(j + 1) * 128])
                fire(work, part, per)
                acc = part if acc is None else acc + part
            cols.append(acc)
        assert not work
        roll_halo(TM0)
        a = _unpack(a_s[0:TM0 // 2, :])
        for j in range(NJ - 1):
            res = cols[j] + _nn(gate(a) if j == GJ else a, _unpack(wo_p[:, j * 128:(j + 1) * 128]))
            emit(0, 0, 0, j, res[0:HM])
            emit(0, 0, HM, j, res[HM:])
        last = [_nn(a[i * QM:(i + 1) * QM], _unpack(wo_p[:, D - 128:D])) for i in range(4)]
        res = cols[NJ - 1] + jnp.concatenate(last, axis=0)
        emit(0, 0, 0, NJ - 1, res[0:HM])
        emit(0, 0, HM, NJ - 1, res[HM:])
        assert not toks

    def main(i, carry):
        with scope('step0'):
            first_block()
        for c in cp_xs:
            c.wait()

        def body(b, c):
            with scope('stepb'):
                step(b)
            return c
        return jax.lax.fori_loop(0, NL, body, carry)

    jax.lax.fori_loop(0, zero_s[0] + 1, main, 0)

    with scope('waitout'):
        for j in range(NJ):
            for r in range(2):
                cp_o(0, 0, r * HM, HM, j).wait()
        for b in range(NL):
            for j in range(NJ):
                for r in range(2):
                    cp_o(b + 1, TM0 + b * TM1, r * HM1, HM1, j).wait()


@jax.jit
def pallas_parallel_sum__sliding_local_dilated__geglu_ffn__prompt_kernel(
    A_x, A_wqkv, A_wo, B_x, B_w_gate, B_w_up, B_w_down,
):
    x = A_x.reshape(S, D)
    hbm = pl.BlockSpec(memory_space=pltpu.MemorySpace.HBM)
    out = pl.pallas_call(
        _kernel,
        in_specs=[hbm] * 6,
        out_specs=hbm,
        out_shape=jax.ShapeDtypeStruct((S, D), BF),
        scratch_shapes=[
            pltpu.VMEM((NL + 1, TMP, D), BF),
            pltpu.VMEM((TM1 // 2, D), U32),
            pltpu.VMEM((5 * HP, 256), U32),
            pltpu.VMEM((TM1 // 2, D), U32),
            pltpu.VMEM((5 * HP, 256), U32),
            pltpu.VMEM((NL + 1, TMP, D), BF),
            pltpu.VMEM((D, 3 * D), BF),
            pltpu.VMEM((D // 2, 3 * D), U32),
            pltpu.VMEM((D, D), BF),
            pltpu.VMEM((NJ, D, 128), F32),
            pltpu.VMEM((D // 2, D), U32),
            pltpu.VMEM((FM, D), BF),
            pltpu.VMEM((FM, D), BF),
            pltpu.VMEM((128, D), BF),
            pltpu.VMEM((FP, D), BF),
            pltpu.VMEM((7 * 5 * 128, 128), U32),
            pltpu.VMEM((12 * 5 * 64, 256), U32),
            pltpu.VMEM((5 * FH // 2, 256), U32),
            pltpu.VMEM((5 * 128, 256), U32),
            pltpu.VMEM((NJ, TMX, 128), F32),
            pltpu.VMEM((NJ, TMX + HALO, 128), F32),
            pltpu.VMEM((NJ, TMX + HALO, 128), F32),
            pltpu.VMEM((TMX // 2, FP), U32),
            pltpu.VMEM((TMX // 2, D), U32),
            pltpu.SMEM((1,), jnp.int32),
            pltpu.SemaphoreType.DMA((XSPLIT + len(G_EARLY) + 5,)),
            pltpu.SemaphoreType.DMA((1,)),
        ],
        compiler_params=pltpu.CompilerParams(
            vmem_limit_bytes=100 * 1024 * 1024,
            disable_bounds_checks=True, disable_semaphore_checks=True,
        ),
    )(x, A_wqkv, A_wo, B_w_gate.T, B_w_up.T, B_w_down)
    return out.reshape(1, S, D)
```

```python
import contextlib
import functools

import jax
import jax.numpy as jnp
import jax.experimental.pallas as pl
import jax.experimental.pallas.tpu as pltpu

S, D, H, DH, W, DIL, F = 2048, 640, 32, 20, 8, 2, 1728
TM0 = 384
NL = 4
TM1 = (S - TM0) // NL
HM1 = TM1 // 2
HP = HM1 // 2
TMX = max(TM0, TM1)
TMP = (TMX + 63) // 64 * 64
HALO = 16
NJ = D // 128
LOG2E = 1.4426950408889634
FM = 1664
FP = 1792
FH = FP // 2
RC = 16
LC = 16
NHOLD = 12
G_EARLY = [[0], [1, 2], [3, 4, 5]]
G_Q, G_KV, G_R, G_D = [6], [7], [8, 9, 10, 11], [12]
LNSPAN = 24
NA2 = 6
A2SPAN = 9
AOFF = 1.5
GPOS = 24
NAR = 4
NAA = 8
NAB = 7
NPD = 40
SPANA = 11.8
SPANB = 6
SPANC = 4
KVSPAN = 8
QPER = 1.5
QSPAN = 3
CH0 = 3
UT = 16
UP = 32
UD = 16
UW = 64
SCOPES = 0

BF = jnp.bfloat16
F32 = jnp.float32
U32 = jnp.uint32
NT = (((1,), (1,)), ((), ()))
P = functools.partial


def _scope(name):
    return jax.named_scope(name) if SCOPES else contextlib.nullcontext()


def _gelu(g):
    c0 = 0.7978845608028654
    c1 = c0 * 0.044715
    t = jnp.tanh(g * (c0 + c1 * (g * g)))
    hg = 0.5 * g
    return hg + hg * t


def _pack(x):
    return pltpu.bitcast(x.astype(BF), U32)


def _unpack(u):
    return pltpu.bitcast(u, BF)


def _lhs_sums(a11, a12, a21, a22):
    return [a11 + a22, a21 + a22, a11 + a12, a21 - a11, a12 - a22]


def _rhs_sums(b11, b12, b21, b22):
    return [b11 + b22, b12 - b22, b21 - b11, b11 + b12, b21 + b22]


LS = {1: 0, 2: 1, 5: 2, 6: 3, 7: 4}
RS = {1: 0, 3: 1, 4: 2, 6: 3, 7: 4}

HK_R = {0: ((0, 0, 1), (0, 2, -1), (1, 0, 1)), 1: ((0, 0, 1), (0, 1, -1), (2, 0, 1)),
        2: ((1, 1, 1), (1, 0, -1), (2, 1, 1)), 3: ((0, 1, 1), (1, 1, 1), (1, 2, -1)),
        4: ((1, 2, 1), (2, 0, -1), (2, 2, 1)), 5: ((0, 2, 1), (2, 1, -1), (2, 2, 1)),
        6: ((0, 1, 1), (1, 0, 1)), 9: ((0, 2, 1), (2, 0, 1)), 12: ((1, 2, 1), (2, 1, 1))}
HK_RS = {r: i for i, r in enumerate(HK_R)}
HK_RP = {7: (1, 0), 8: (0, 1), 10: (2, 0), 11: (0, 2), 13: (2, 1), 14: (1, 2)}
HK_LP = {0: (0, 0), 3: (1, 1), 4: (0, 2), 5: (1, 2)}
HK_LS = {r: i for i, r in enumerate((1, 2, 6, 7, 8, 9, 10, 11, 12, 13, 14))}
NSUM = 16


def _hk_lhs_sums(x, y):
    s0, s1, s2 = x[0] + y[0], x[1] + y[1], x[2] + y[2]
    return [s0, s1, x[0] + y[1], x[1] - x[0], y[0] - y[1], s0 - y[2], s2 - s0, y[2] - y[0],
            s1 - x[2], s2 - s1, x[2] - x[1]]


def _nn(a, b):
    return jnp.dot(a, b, preferred_element_type=F32)


def _nt(a, b):
    return jax.lax.dot_general(a, b, NT, preferred_element_type=F32)


def _weave(*lists):
    items = []
    for lst in lists:
        items += [((k + 0.5) / len(lst), w) for k, w in enumerate(lst)]
    items.sort(key=lambda t: t[0])
    return [t[1] for t in items]


def _kernel(x_hbm, wqkv_hbm, wo_hbm, wg_hbm, wu_hbm, wd_hbm, out_hbm,
            x_s, xn_s, xs_s, xn2_s, xs2_s, out_s, wqkv_r, wqkv_p, wo_r, wo_f, wo_p,
            wg_s, wu_s, wt_s, wd_s, t1_s, td_s, to_s, q_s, k_s, v_s, h_s, a_s, hold_s,
            zero_s, sem_i, sem_o):

    def zrow():
        return pl.multiple_of(zero_s[0] * 8, 8)

    def after(val, trig):
        if trig is None:
            return val
        n = val.shape[0] // 8
        t = pltpu.bitcast(trig, val.dtype) if trig.dtype != val.dtype else trig
        if n > 1:
            t = jnp.concatenate([t] * n, axis=0)
        keep = jax.lax.broadcasted_iota(jnp.int32, val.shape, 1) >= zero_s[0]
        return jnp.where(keep, val, t)

    def after_head(val, trig):
        if trig is None:
            return val
        if val.shape[1] == 128:
            return after(val, trig)
        return jnp.concatenate([after(val[:, 0:128], trig), val[:, 128:]], axis=1)

    toks = []
    credit = [0.0]
    chain = [0]
    prev = []

    def reset(dist):
        del toks[:]
        del prev[:]
        credit[0] = 0.0
        chain[0] = dist

    def note(ref, row):
        if all(r is not ref for r, _ in toks):
            toks.append((ref, row))

    def gate(lhs):
        if not toks:
            return lhs
        tok = functools.reduce(lambda p, q: p | q,
                               [pltpu.bitcast(ref[pl.ds(zrow() + row, 8), 0:128], U32) for ref, row in toks])
        del toks[:]
        u = pltpu.bitcast(lhs[0:16], U32)
        return jnp.concatenate([_unpack(after_head(u, tok)), lhs[16:]], axis=0)

    def fire(work, res, per):
        if not work:
            credit[0] = 0.0
            return
        pos = credit[0]
        while pos < 1.0 and work:
            r = int((res.shape[0] - 8) * pos) // 8 * 8
            trig = pltpu.bitcast(res[r:r + 8, :], U32)
            item = work.pop(0)
            if item.func in (attn_rows, ln_pair) and len(prev) >= chain[0]:
                trig = trig | prev[-chain[0]]
            tok = item(trig)
            if tok is not None:
                prev.append(pltpu.bitcast(tok, U32))
            pos += 1.0 / per
        credit[0] = max(pos - 1.0, 0.0)

    lane = jax.lax.broadcasted_iota(jnp.int32, (32, 128), 1)
    l5 = lane % 5
    masks = [l5 == r for r in range(5)]
    idx = [(DH * (lane % H) + 5 * (lane // H) + j) % 128 for j in range(NJ)]

    def permute_qkv(t, r0, trig):
        src = [pltpu.bitcast(wqkv_r[r0:r0 + 64, t * D + s * 128:t * D + (s + 1) * 128], U32)
               for s in range(NJ)]
        src[4] = after(src[4], trig)
        for j in range(NJ):
            mg = src[4]
            for s in range(3, -1, -1):
                mg = jnp.where(masks[(j - 3 * s) % 5], src[s], mg)
            res = jnp.take_along_axis(mg, idx[j], axis=1, mode="promise_in_bounds")
            wqkv_p[r0 // 2:r0 // 2 + 32, t * D + j * 128:t * D + (j + 1) * 128] = res

    def widen_wo(jj, r0, trig):
        w = after(pltpu.bitcast(wo_r[r0:r0 + UW, jj * 128:(jj + 1) * 128], U32), trig)
        wo_f[jj * D + r0:jj * D + r0 + UW, :] = _unpack(w).astype(F32)

    def gather_wo(jj, j, trig):
        for g in range(4):
            rows = wo_f[pl.ds(jj * D + 5 * g + j, H, stride=DH), :]
            rows = jnp.concatenate([after(rows[r:r + 8], trig) if r % 16 == 0 else rows[r:r + 8]
                                    for r in range(0, H, 8)], axis=0)
            r0 = (j * 128 + g * H) // 2
            wo_p[r0:r0 + H // 2, jj * 128:(jj + 1) * 128] = _pack(rows)

    def prep(b11, b12, b21, b22, store, trig):
        b11, b12, b21, b22 = [b.astype(F32) for b in (b11, b12, b21, b22)]
        b11 = after(b11, trig)
        b22 = after(b22, trig)
        for i, s in enumerate(_rhs_sums(b11, b12, b21, b22)):
            store(i, _pack(s))

    def wtile(mat, k, n, r0=0, nr=128):
        if mat == 0:
            return _unpack(wqkv_p[k * 64 + r0 // 2:k * 64 + (r0 + nr) // 2, n * 128:(n + 1) * 128])
        return (wg_s, wu_s)[mat - 1][n * 128 + r0:n * 128 + r0 + nr, k * 128:(k + 1) * 128]

    def t_tri(mat, n0, i):
        return ((0, 80, 146)[mat] + n0 // 3 * 9 + i) * 64

    def t_pair(mat, n0, i):
        return ((45, 116, 182)[mat] + n0 // 2 * 5 + i) * 64

    def prep_tri(mat, n0, r0, trig):
        b = [[wtile(mat, k, n0 + n, r0, UT).astype(F32) for n in range(3)] for k in range(3)]
        for k, n in ((1, 0), (0, 1), (0, 2), (1, 2)):
            b[k][n] = after(b[k][n], trig)
        for r, terms in HK_R.items():
            s = None
            for k, n, c in terms:
                s = b[k][n] if s is None else (s + b[k][n] if c > 0 else s - b[k][n])
            row = t_tri(mat, n0, HK_RS[r]) + r0 // 2
            t1_s[row:row + UT // 2, :] = _pack(s)
            note(t1_s, row)

    def prep_pair(mat, n0, r0, trig):
        def store(i, o):
            row = t_pair(mat, n0, i) + r0 // 2
            t1_s[row:row + UP // 2, :] = o
            note(t1_s, row)
        prep(wtile(mat, 3, n0, r0, UP), wtile(mat, 3, n0 + 1, r0, UP),
             wtile(mat, 4, n0, r0, UP), wtile(mat, 4, n0 + 1, r0, UP), store, trig)

    def preps(mat, tris, pairs):
        return ([P(prep_tri, mat, n0, r0) for n0 in tris for r0 in range(0, 128, UT)]
                + [P(prep_pair, mat, n0, r0) for n0 in pairs for r0 in range(0, 128, UP)])

    def prep_d(r0, c, trig):
        def store(i, o):
            row = i * (FH // 2) + r0 // 2
            td_s[row:row + UD // 2, c:c + 128] = o
        prep(wd_s[r0:r0 + UD, c:c + 128], wd_s[r0:r0 + UD, 256 + c:384 + c],
             wd_s[FH + r0:FH + r0 + UD, c:c + 128], wd_s[FH + r0:FH + r0 + UD, 256 + c:384 + c], store, trig)

    def prep_o(r0, c, trig):
        n = UD // 2

        def store(i, o):
            to_s[i * 128 + r0:i * 128 + r0 + n, c:c + 128] = o
        prep(_unpack(wo_p[r0:r0 + n, c:c + 128]), _unpack(wo_p[r0:r0 + n, 256 + c:384 + c]),
             _unpack(wo_p[128 + r0:128 + r0 + n, c:c + 128]), _unpack(wo_p[128 + r0:128 + r0 + n, 256 + c:384 + c]),
             store, trig)

    def ln_rows(blk, r0, trig=None):
        x = after_head(x_s[blk, r0:r0 + LC, :].astype(F32), trig)
        m = jnp.sum(x, axis=-1, keepdims=True) * (1.0 / D)
        mb = m.astype(BF).astype(F32)
        xc = x - mb
        dm = m - mb
        var = jnp.sum(xc * xc, axis=-1, keepdims=True) * (1.0 / D) - dm * dm
        return xc * jax.lax.rsqrt(jnp.maximum(var, 0.0) + 1e-5)

    def ln_pair(blk, r0, xn_d, xs_d, trig):
        top = ln_rows(blk, r0, trig)
        bot = ln_rows(blk, HM1 + r0, trig)
        xn_d[r0 // 2:(r0 + LC) // 2, :] = _pack(top)
        xn_d[(HM1 + r0) // 2:(HM1 + r0 + LC) // 2, :] = _pack(bot)
        x = [top[:, k * 128:(k + 1) * 128] for k in range(NJ)]
        y = [bot[:, k * 128:(k + 1) * 128] for k in range(NJ)]
        for i, s in enumerate(_hk_lhs_sums(x, y) + _lhs_sums(x[3], x[4], y[3], y[4])):
            xs_d[i * HP + r0 // 2:i * HP + (r0 + LC) // 2, :] = _pack(s)
        note(xn_d, r0 // 2)
        note(xs_d, r0 // 2)
        s0 = x[0] + y[0]
        return s0[0:8] + s0[8:16]

    def tail_h(t):
        ht = _gelu(t) * pltpu.roll(t, 64, 1)
        lo = jax.lax.broadcasted_iota(jnp.int32, ht.shape, 1) < 64
        return jnp.where(lo, ht, 0.0)

    def store_qkv(c, row0, val):
        t, j = divmod(c, NJ)
        n = val.shape[0]
        if t == 0:
            q_s[j, row0:row0 + n, :] = val * (DH ** -0.5 * LOG2E)
        elif t == 1:
            k_s[j, HALO + row0:HALO + row0 + n, :] = val
        else:
            v_s[j, HALO + row0:HALO + row0 + n, :] = val

    def attn_core(r0, first, trig):
        q = [after(q_s[j, r0:r0 + 8, :], trig) for j in range(NJ)]
        logits = []
        for w in range(W):
            st = HALO + r0 - DIL * w
            acc = q[0] * k_s[0, st:st + 8, :]
            for j in range(1, NJ):
                acc = acc + q[j] * k_s[j, st:st + 8, :]
            acc = acc + pltpu.roll(acc, 64, 1)
            acc = acc + pltpu.roll(acc, 32, 1)
            if first and r0 < DIL * w:
                rows = r0 + jax.lax.broadcasted_iota(jnp.int32, (8, 128), 0)
                acc = jnp.where(rows >= DIL * w, acc, -1e9 * LOG2E)
            logits.append(acc)
        mx = logits[0]
        for w in range(1, W):
            mx = jnp.maximum(mx, logits[w])
        ps = [jnp.exp2(l - mx) for l in logits]
        den = ps[0]
        for w in range(1, W):
            den = den + ps[w]
        r = pl.reciprocal(den, approx=True)
        inv = r * (2.0 - den * r)
        outs = []
        for j in range(NJ):
            acc = ps[0] * v_s[j, HALO + r0:HALO + r0 + 8, :]
            for w in range(1, W):
                st = HALO + r0 - DIL * w
                acc = acc + ps[w] * v_s[j, st:st + 8, :]
            outs.append(acc * inv)
        return outs, mx

    def attn_rows(r0, first, trig):
        o1, t1 = attn_core(r0, first, trig)
        o2, t2 = attn_core(r0 + 8, first, t1)
        for j in range(NJ):
            a_s[r0 // 2:(r0 + RC) // 2, j * 128:(j + 1) * 128] = _pack(jnp.concatenate([o1[j], o2[j]], axis=0))
        return t2

    def cp_o(blk, base, r0, n, j):
        return pltpu.make_async_copy(out_s.at[blk, pl.ds(r0, n), pl.ds(j * 128, 128)],
                                     out_hbm.at[pl.ds(base + r0, n), pl.ds(j * 128, 128)], sem_o.at[0])

    def emit(blk, base, r0, j, val):
        n = val.shape[0]
        x = x_s[blk, r0:r0 + n, j * 128:(j + 1) * 128].astype(F32)
        out_s[blk, r0:r0 + n, j * 128:(j + 1) * 128] = (x + val).astype(BF)
        cp_o(blk, base, r0, n, j).start()

    def stage2(blk, base, tm, works, pers):
        hm, hp = tm // 2, tm // 4

        def half(ref, r, c0, c1):
            return _unpack(ref[r * hp:(r + 1) * hp, c0:c1])

        memo = {}

        def lhs(plain, kh, i):
            if i == 3:
                return half(plain, 0, 0, kh)
            if i == 4:
                return half(plain, 1, kh, 2 * kh)
            if (kh, i) not in memo:
                def b(r, c):
                    u = plain[pl.ds(zrow(), 2 * hp), c * kh:(c + 1) * kh]
                    return _unpack(u[r * hp:(r + 1) * hp]).astype(F32)
                s = {1: lambda: b(0, 0) + b(1, 1), 2: lambda: b(1, 0) + b(1, 1), 5: lambda: b(0, 0) + b(0, 1),
                     6: lambda: b(1, 0) - b(0, 0), 7: lambda: b(0, 1) - b(1, 1)}[i]()
                memo[(kh, i)] = s.astype(BF)
            return memo[(kh, i)]

        f4 = []
        for r in range(2):
            if works[0] is works[1]:
                f = _nn(half(h_s, r, 0, FP), wd_s[:, 512:D])
                fire(works[0], f, pers[0])
            else:
                f = None
                for k0 in range(0, FP, 512):
                    k1 = min(k0 + 512, FP)
                    part = _nn(half(h_s, r, k0, k1), wd_s[k0:k1, 512:D])
                    fire(works[0], part, pers[0])
                    f = part if f is None else f + part
            f4.append(f)
        ffn = []
        for c in range(2):
            assert works[c] is works[c + 1] or not works[c]
            if c == 0 or works[1] is not works[2]:
                credit[0] = 0.0
            cs = (c * 128, 256 + c * 128)

            def p(i):
                if i == 2:
                    wd = wd_s[0:FH, cs[0]:cs[0] + 128]
                elif i == 5:
                    wd = wd_s[FH:FP, cs[1]:cs[1] + 128]
                else:
                    wd = _unpack(td_s[RS[i] * (FH // 2):(RS[i] + 1) * (FH // 2), cs[0]:cs[0] + 128])
                m = _nn(lhs(h_s, FH, i), wd)
                fire(works[c + 1], m, pers[c + 1])
                return m
            m4 = p(4)
            m2 = p(2)
            m1 = p(1)
            t11 = m1 + m4
            t22 = m1 - m2
            m3 = p(3)
            m5 = p(5)
            ffn.append((t11 - m5 + p(7), m3 + m5, m4 + m2, t22 + m3 + p(6)))
        assert not works[2]
        k_s[:, 0:HALO, :] = k_s[:, tm:tm + HALO, :]
        v_s[:, 0:HALO, :] = v_s[:, tm:tm + HALO, :]
        for r in range(2):
            emit(blk, base, r * hm, 4, f4[r] + _nn(gate(half(a_s, r, 0, D)), _unpack(wo_p[:, 512:D])))
        for c in range(2):
            cs = (c * 128, 256 + c * 128)

            def p(i):
                if i == 2:
                    wo = wo_p[0:128, cs[0]:cs[0] + 128]
                elif i == 5:
                    wo = wo_p[128:256, cs[1]:cs[1] + 128]
                else:
                    wo = to_s[RS[i] * 128:(RS[i] + 1) * 128, cs[0]:cs[0] + 128]
                return _nn(lhs(a_s, 256, i), _unpack(wo))

            def left(r, cc):
                return ffn[c][2 * r + cc] + _nn(half(a_s, r, 512, D), _unpack(wo_p[256:320, cs[cc]:cs[cc] + 128]))
            l21 = left(1, 0)
            m4 = p(4)
            m2 = p(2)
            c21 = l21 + m4 + m2
            m1 = p(1)
            t11 = m1 + m4
            t22 = m1 - m2
            m3 = p(3)
            m5 = p(5)
            c12 = m3 + m5 + left(0, 1)
            c11 = t11 - m5 + p(7) + left(0, 0)
            c22 = t22 + m3 + p(6) + left(1, 1)
            emit(blk, base, hm, c, c21)
            emit(blk, base, 0, c + 2, c12)
            emit(blk, base, 0, c, c11)
            emit(blk, base, hm, c + 2, c22)

    def step(b):
        blk = b + 1
        base = pl.multiple_of(TM0 + b * TM1, 16)
        nblk = jnp.minimum(blk + 1, NL)
        reset(1)
        side = {}

        def xt(r, k):
            return _unpack(xn_s[r * HP:(r + 1) * HP, k * 128:(k + 1) * 128])

        def xsum(i):
            return _unpack(xs_s[i * HP:(i + 1) * HP, :])

        def mm(mat, l, w):
            return (_nn if mat == 0 else _nt)(l, w)

        def tick(v):
            fire(side['work'], v, side['per'])

        def hk(mat, n0, r):
            l = xt(*HK_LP[r]) if r in HK_LP else xsum(HK_LS[r])
            if r in HK_RP:
                w = wtile(mat, HK_RP[r][0], n0 + HK_RP[r][1])
            else:
                row = t_tri(mat, n0, HK_RS[r])
                w = _unpack(t1_s[row:row + 64, :])
            return mm(mat, l, w)

        def st(mat, n0, i):
            l = xt(0, 3) if i == 3 else xt(1, 4) if i == 4 else xsum(11 + LS[i])
            if i == 2:
                w = wtile(mat, 3, n0)
            elif i == 5:
                w = wtile(mat, 4, n0 + 1)
            else:
                row = t_pair(mat, n0, RS[i])
                w = _unpack(t1_s[row:row + 64, :])
            return mm(mat, l, w)

        def add(acc, key, v):
            acc[key] = v if key not in acc else acc[key] + v

        def s_a(acc, mat, n0):
            m1, m4, m5, m7 = [st(mat, n0, i) for i in (1, 4, 5, 7)]
            add(acc, (0, n0), (m1 + m4) + (m7 - m5))
            tick(acc[(0, n0)])
            add(acc, (1, n0 + 1), m1)
            add(acc, (1, n0), m4)
            add(acc, (0, n0 + 1), m5)

        def s_b(acc, mat, n0):
            m2, m3, m6 = [st(mat, n0, i) for i in (2, 3, 6)]
            add(acc, (1, n0), m2)
            add(acc, (0, n0 + 1), m3)
            add(acc, (1, n0 + 1), (m3 - m2) + m6)
            tick(acc[(1, n0 + 1)])

        def h_a(acc, mat, n0):
            r0, r9, r11, r10 = [hk(mat, n0, r) for r in (0, 9, 11, 10)]
            t = r9 + r11
            w0 = r0 + t
            add(acc, (0, n0), w0 + r10)
            tick(acc[(0, n0)])
            acc[(1, n0)] = acc[(1, n0)] - w0
            add(acc, (0, n0 + 2), t + r10)
            acc[(1, n0 + 2)] = acc[(1, n0 + 2)] - r11 if (1, n0 + 2) in acc else -r11

        def h_b(acc, mat, n0):
            r7, r6, r8, r1 = [hk(mat, n0, r) for r in (7, 6, 8, 1)]
            add(acc, (0, n0), r7)
            add(acc, (1, n0), (r1 + r6) + r8)
            tick(acc[(1, n0)])
            add(acc, (0, n0 + 1), r6 + r7)
            add(acc, (1, n0 + 1), r8)

        def h_c(acc, mat, n0):
            r3, r12, r14, r13 = [hk(mat, n0, r) for r in (3, 12, 14, 13)]
            t = r12 + r14
            w1 = r3 + t
            acc[(0, n0 + 1)] = acc[(0, n0 + 1)] - w1
            add(acc, (1, n0 + 1), w1 + r13)
            tick(acc[(1, n0 + 1)])
            acc[(0, n0 + 2)] = acc[(0, n0 + 2)] - r14
            add(acc, (1, n0 + 2), t + r13)

        def h_1(acc, mat, n0, r):
            add(acc, {2: (0, n0 + 1), 4: (0, n0 + 2), 5: (1, n0 + 2)}[r], hk(mat, n0, r))

        def group6(mat, n0, done, filler):
            acc = {}

            def fin(*keys):
                for key in keys:
                    done(key[0], key[1], acc.pop(key))
            s_a(acc, mat, n0)
            s_b(acc, mat, n0)
            h_1(acc, mat, n0, 2)
            h_a(acc, mat, n0)
            h_b(acc, mat, n0)
            fin((0, n0), (1, n0))
            h_c(acc, mat, n0)
            fin((0, n0 + 1), (1, n0 + 1))
            s_a(acc, mat, n0 + 2)
            s_b(acc, mat, n0 + 2)
            h_1(acc, mat, n0, 5)
            fin((1, n0 + 2))
            s_a(acc, mat, n0 + 4)
            s_b(acc, mat, n0 + 4)
            h_1(acc, mat, n0, 4)
            fin((0, n0 + 2))
            h_a(acc, mat, n0 + 3)
            h_b(acc, mat, n0 + 3)
            fin((0, n0 + 3), (1, n0 + 3))
            h_c(acc, mat, n0 + 3)
            fin((1, n0 + 4))
            for r in (2, 4, 5):
                h_1(acc, mat, n0 + 3, r)
            fin((0, n0 + 4), (0, n0 + 5), (1, n0 + 5))
            assert not acc
            filler()

        work = [P(ln_pair, nblk, k * LC, xn2_s, xs2_s) for k in range(HM1 // LC)]
        side.update(work=work, per=len(work) / LNSPAN)
        acc = {}
        plain = [(r, k) for k in (3, 4) for r in range(2)]

        def fill_q():
            r, k = plain.pop(0)
            add(acc, (r, 14), mm(0, xt(r, k), wtile(0, k, 14)))

        def done_q(r, n, val):
            store_qkv(n, r * HM1, val)

        def fin_q(*keys):
            for key in keys:
                done_q(key[0], key[1], acc.pop(key))
        fill_q()
        fill_q()
        group6(0, 0, done_q, fill_q)
        group6(0, 6, done_q, fill_q)
        s_a(acc, 0, 12)
        s_b(acc, 0, 12)
        h_1(acc, 0, 12, 2)
        h_a(acc, 0, 12)
        h_b(acc, 0, 12)
        fin_q((0, 12), (1, 12))
        h_c(acc, 0, 12)
        fin_q((0, 13), (1, 13))
        h_1(acc, 0, 12, 4)
        h_1(acc, 0, 12, 5)
        fin_q((0, 14), (1, 14))
        assert not work and not acc

        work = [P(attn_rows, c * RC, False) for c in range(TM1 // RC)]
        side.update(work=work, per=(len(work) - NA2) / 53.0)
        credit[0] = AOFF

        def store_h(r, n, v):
            h_s[r * HP:(r + 1) * HP, n * 128:(n + 1) * 128] = _pack(v)

        pl_list = [(2, r, k) for r in range(2) for k in range(NJ)]
        pl_list += [(w, r, k) for r in range(2) for w in range(2) for k in range(NJ)]

        def fill_g(n=1):
            for _ in range(n):
                w, r, k = pl_list.pop(0)
                wt = wt_s[:, k * 128:(k + 1) * 128] if w == 2 else wtile(w + 1, k, 12)
                l = xt(r, k)
                if len(pl_list) == 29 - GPOS:
                    l = gate(l)
                add(acc, (w, r), mm(1, l, wt))
                if k == NJ - 1:
                    tick(acc[(w, r)])
                    if w == 1:
                        store_h(r, 12, _gelu(acc.pop((0, r))) * acc.pop((1, r)))
                    if w == 2:
                        store_h(r, 13, tail_h(acc.pop((2, r))))
        fill_g(26)
        for n0 in (0, 6):
            def slot(r, n):
                s = (n - n0) * 2 + r
                return slice(s * HM1, (s + 1) * HM1)

            def done_g(r, n, v):
                hold_s[slot(r, n), :] = _gelu(v) if (r + n) % 2 == 0 else v

            def done_u(r, n, v):
                g = hold_s[slot(r, n), :]
                store_h(r, n, (g if (r + n) % 2 == 0 else _gelu(g)) * v)
            group6(1, n0, done_g, fill_g)
            group6(2, n0, done_u, fill_g)
        assert not pl_list and not acc
        note(hold_s, 0)

        def copy_xn(dst, src, r0, c, trig):
            dst[r0:r0 + HP, c:c + 128] = after(src[pl.ds(zrow(), r0 + HP), c:c + 128][r0:r0 + HP], trig)
            if c == 0:
                note(dst, r0)
        copies = [P(copy_xn, xn_s, xn2_s, r, c) for r in (0, HP) for c in range(0, D, 128)]
        copies += [P(copy_xn, xs_s, xs2_s, i * HP, 0) for i in range(NSUM)]
        mixed = _weave(work, copies)
        per = len(mixed) / (A2SPAN + 4.0)
        stage2(blk, base, TM1, [mixed] * 3, [2 * per, per, per])

    def cp(src, dst, s):
        return pltpu.make_async_copy(src, dst, sem_i.at[s])

    def gu(groups, s):
        return [cp(h.at[pl.ds(g * 128, 128)], d.at[pl.ds(g * 128, 128)], s)
                for g in groups for h, d in ((wg_hbm, wg_s), (wu_hbm, wu_s))]

    def wcol(t, s):
        return cp(wqkv_hbm.at[:, pl.ds(t * D, D)], wqkv_r.at[:, pl.ds(t * D, D)], s)

    def xblk(b, s):
        return cp(x_hbm.at[pl.ds(TM0 + b * TM1, TM1)], x_s.at[b + 1, pl.ds(0, TM1)], s)

    HM = TM0 // 2
    cp_x0 = [cp(x_hbm.at[pl.ds(i * HM, HM)], x_s.at[0, pl.ds(i * HM, HM)], i) for i in range(2)]
    cp_gu = [gu(g, 2 + k) for k, g in enumerate(G_EARLY)]
    cp_q = gu(G_Q, 5) + [cp(wg_hbm.at[pl.ds(FM, 64)], wt_s.at[pl.ds(0, 64)], 5),
                         cp(wu_hbm.at[pl.ds(FM, 64)], wt_s.at[pl.ds(64, 64)], 5), wcol(0, 5), xblk(0, 5)]
    cp_kv = gu(G_KV, 6) + [wcol(1, 6), wcol(2, 6)]
    cp_r = gu(G_R + G_D, 7) + [cp(wo_hbm, wo_r, 7)]
    cp_d = [cp(wd_hbm, wd_s.at[pl.ds(0, F)], 8)]
    cp_xs = [xblk(b, 9) for b in range(1, NL)]

    for c in cp_x0 + sum(cp_gu, []) + cp_q + cp_kv + cp_r + cp_d + cp_xs:
        c.start()
    zero_s[0] = 0
    k_s[:, 0:HALO, :] = jnp.zeros((NJ, HALO, 128), F32)
    v_s[:, 0:HALO, :] = jnp.zeros((NJ, HALO, 128), F32)
    wd_s[F:FP, :] = jnp.zeros((FP - F, D), BF)

    def first_block():
        def wait(cps, name):
            reset(CH0)
            with _scope(name):
                for c in cps:
                    c.wait()

        parts = []
        for i in range(2):
            wait(cp_x0[i:i + 1], 'waitx')
            parts += [ln_rows(0, i * HM + k * LC).astype(BF) for k in range(HM // LC)]
        xn = jnp.concatenate(parts, axis=0)

        def ffn_group(x, row0, g0, work, per, gated=False):
            g = _nt(x, wg_s[g0 * 128:(g0 + 1) * 128, :])
            fire(work, g, per)
            u = _nt(gate(x) if gated else x, wu_s[g0 * 128:(g0 + 1) * 128, :])
            fire(work, u, per)
            h_s[row0 // 2:(row0 + x.shape[0]) // 2, g0 * 128:(g0 + 1) * 128] = _pack(_gelu(g) * u)

        def ffn_groups(groups, work, per, gate_last=False):
            groups = list(groups)
            if len(groups) % 2:
                g0 = groups.pop(0)
                ffn_group(xn[0:HM], 0, g0, work, per)
                ffn_group(xn[HM:], HM, g0, work, per)
            for k, g0 in enumerate(groups):
                ffn_group(xn, 0, g0, work, per, gate_last and k == len(groups) - 1)

        have, done = set(), set()

        def new_preps(groups):
            have.update(groups)
            tris = [n for n in (0, 3, 6, 9) if {n, n + 1, n + 2} <= have and ('t', n) not in done]
            pairs = [n for n in range(0, 12, 2) if {n, n + 1} <= have and ('p', n) not in done]
            done.update([('t', n) for n in tris] + [('p', n) for n in pairs])
            return preps(1, tris, pairs) + preps(2, tris, pairs)

        perm = [[P(permute_qkv, t, r0) for r0 in range(0, D, 64)] for t in range(3)]

        for k, (cps, groups) in enumerate(zip(cp_gu, G_EARLY)):
            wait(cps, 'waitgu')
            work = new_preps(groups)
            nres = 2 * len(groups) + 2 * (len(groups) % 2)
            ffn_groups(groups, work, max(len(work), 1) / max(nres - 2.0, 1.0), k == 2)
            assert not work

        wait(cp_q, 'waitq')
        work = perm[0]
        for _ in range(3):
            work.pop(0)(None)
        t = _nt(xn, wt_s[...])
        fire(work, t, 4)
        h_s[0:TM0 // 2, FM:FP] = _pack(tail_h(t))
        work += new_preps(G_Q) + [P(ln_pair, 1, k * LC, xn_s, xs_s) for k in range(HM1 // LC)]
        for g0 in G_Q:
            ffn_group(xn, 0, g0, work, QPER)
        assert all(w.func is ln_pair for w in work)
        per = len(work) / QSPAN
        for j in range(NJ):
            r = _nn(xn, _unpack(wqkv_p[:, j * 128:(j + 1) * 128]))
            fire(work, r, per)
            store_qkv(j, 0, r)
        assert not work

        wait(cp_kv, 'waitkv')
        work = perm[1]
        for _ in range(4):
            work.pop(0)(None)
        for g0 in G_KV:
            g = _nt(xn, wg_s[g0 * 128:(g0 + 1) * 128, :])
            fire(work, g, 6)
            u = _nt(xn, wu_s[g0 * 128:(g0 + 1) * 128, :])
            h_s[0:TM0 // 2, g0 * 128:(g0 + 1) * 128] = _pack(_gelu(g) * u)
        assert not work
        work = perm[2] + _weave(new_preps(G_KV), _weave(preps(0, range(0, 15, 3), []),
                                                        preps(0, [], range(0, 14, 2))))
        per = len(work) / KVSPAN
        fire(work, u, per)
        for c in range(NJ, 3 * NJ):
            assert c < 2 * NJ or all(w.func is not permute_qkv for w in work)
            r = _nn(gate(xn) if c == 3 * NJ - 1 else xn, _unpack(wqkv_p[:, c * 128:(c + 1) * 128]))
            fire(work, r, per)
            store_qkv(c, 0, r)
        assert not work

        wait(cp_r, 'waitr')
        att = [P(attn_rows, rc * RC, True) for rc in range(TM0 // RC)]
        work = _weave(new_preps(G_R + G_D), att[:NAR])
        att = att[NAR:]
        ffn_groups(G_R, work, len(work) / (2 * len(G_R) - 2.0))
        assert not work

        wait(cp_d, 'waitd')
        wo_work = []
        for jj in range(NJ):
            wo_work += [P(widen_wo, jj, r0) for r0 in range(0, D, UW)]
            wo_work += [P(gather_wo, jj, j) for j in range(NJ)]
        pd = [[P(prep_d, r0, c) for r0 in range(0, FH, UD)] for c in (0, 128)]
        po = [P(prep_o, r0, c) for r0 in range(0, 128, UD // 2) for c in (0, 128)]
        wa = _weave(pd[0] + pd[1][:NPD], wo_work, att[:NAA])
        wb = _weave(pd[1][NPD:] + po, att[NAA:NAA + NAB])
        wc = att[NAA + NAB:]
        for _ in range(2):
            wa.pop(0)(None)
        per = len(wa) / SPANA
        ffn_groups(G_D, wa, per)
        stage2(0, 0, TM0, [wa, wb, wc], [per, len(wb) / SPANB, len(wc) / SPANC])

    def main(i, carry):
        with _scope('step0'):
            first_block()
        for c in cp_xs:
            c.wait()

        def body(b, c):
            with _scope('stepb'):
                step(b)
            return c
        return jax.lax.fori_loop(0, NL, body, carry)

    jax.lax.fori_loop(0, zero_s[0] + 1, main, 0)

    with _scope('waitout'):
        for j in range(NJ):
            for r in range(2):
                cp_o(0, 0, r * HM, HM, j).wait()
        for b in range(NL):
            for j in range(NJ):
                for r in range(2):
                    cp_o(b + 1, TM0 + b * TM1, r * HM1, HM1, j).wait()


@jax.jit
def pallas_parallel_sum__sliding_local_dilated__geglu_ffn__prompt_kernel(
    A_x: jax.Array,
    A_wqkv: jax.Array,
    A_wo: jax.Array,
    B_x: jax.Array,
    B_w_gate: jax.Array,
    B_w_up: jax.Array,
    B_w_down: jax.Array,
):
    x = A_x.reshape(S, D)
    hbm = pl.BlockSpec(memory_space=pltpu.MemorySpace.HBM)
    out = pl.pallas_call(
        _kernel,
        in_specs=[hbm] * 6,
        out_specs=hbm,
        out_shape=jax.ShapeDtypeStruct((S, D), BF),
        scratch_shapes=[
            pltpu.VMEM((NL + 1, TMP, D), BF),
            pltpu.VMEM((TM1 // 2, D), U32),
            pltpu.VMEM((NSUM * HP, 128), U32),
            pltpu.VMEM((TM1 // 2, D), U32),
            pltpu.VMEM((NSUM * HP, 128), U32),
            pltpu.VMEM((NL + 1, TMP, D), BF),
            pltpu.VMEM((D, 3 * D), BF),
            pltpu.VMEM((D // 2, 3 * D), U32),
            pltpu.VMEM((D, D), BF),
            pltpu.VMEM((NJ * D, 128), F32),
            pltpu.VMEM((D // 2, D), U32),
            pltpu.VMEM((FM, D), BF),
            pltpu.VMEM((FM, D), BF),
            pltpu.VMEM((128, D), BF),
            pltpu.VMEM((FP, D), BF),
            pltpu.VMEM((212 * 64, 128), U32),
            pltpu.VMEM((5 * FH // 2, 256), U32),
            pltpu.VMEM((5 * 128, 256), U32),
            pltpu.VMEM((NJ, TMX, 128), F32),
            pltpu.VMEM((NJ, TMX + HALO, 128), F32),
            pltpu.VMEM((NJ, TMX + HALO, 128), F32),
            pltpu.VMEM((TMX // 2, FP), U32),
            pltpu.VMEM((TMX // 2, D), U32),
            pltpu.VMEM((NHOLD * HM1, 128), F32),
            pltpu.SMEM((1,), jnp.int32),
            pltpu.SemaphoreType.DMA((10,)),
            pltpu.SemaphoreType.DMA((1,)),
        ],
        compiler_params=pltpu.CompilerParams(
            vmem_limit_bytes=100 * 1024 * 1024,
            disable_bounds_checks=True,
            disable_semaphore_checks=True,
        ),
    )(x, A_wqkv, A_wo, B_w_gate.T, B_w_up.T, B_w_down)
    return out.reshape(1, S, D)
```

```python
import contextlib
import functools

import jax
import jax.numpy as jnp
import jax.experimental.pallas as pl
import jax.experimental.pallas.tpu as pltpu

S, D, H, DH, W, DIL, F = 2048, 640, 32, 20, 8, 2, 1728
TM0 = 384
NL = 4
TM1 = (S - TM0) // NL
HM1 = TM1 // 2
HP = HM1 // 2
TMX = max(TM0, TM1)
TMP = (TMX + 63) // 64 * 64
HALO = 16
NJ = D // 128
LOG2E = 1.4426950408889634
FM = 1664
FP = 1792
FH = FP // 2
RC = 16
LC = 16
NHOLD = 14
G_EARLY = [[0], [1, 2], [3, 4, 5]]
G_Q, G_KV, G_R, G_D = [6], [7], [8, 9, 10, 11], [12]
LNSPAN = 24
NA2 = 6
A2SPAN = 7
AOFF = 4
NAR = 3
NAA = 8
NAB = 8
SPANA = 11
SPANB = 5
SPANC = 5
KVSPAN = 8
QPER = 1.5
QSPAN = 3.5
CH0 = 3
CHD = 2
UT = 16
UP = 32
UD = 16
UW = 64
SCOPES = 0

BF = jnp.bfloat16
F32 = jnp.float32
U32 = jnp.uint32
NT = (((1,), (1,)), ((), ()))
P = functools.partial


def _scope(name):
    return jax.named_scope(name) if SCOPES else contextlib.nullcontext()


def _gelu(g):
    c0 = 0.7978845608028654
    c1 = c0 * 0.044715
    t = jnp.tanh(g * (c0 + c1 * (g * g)))
    hg = 0.5 * g
    return hg + hg * t


def _pack(x):
    return pltpu.bitcast(x.astype(BF), U32)


def _unpack(u):
    return pltpu.bitcast(u, BF)


def _lhs_sums(a11, a12, a21, a22):
    return [a11 + a22, a21 + a22, a11 + a12, a21 - a11, a12 - a22]


def _rhs_sums(b11, b12, b21, b22):
    return [b11 + b22, b12 - b22, b21 - b11, b11 + b12, b21 + b22]


LS = {1: 0, 2: 1, 5: 2, 6: 3, 7: 4}
RS = {1: 0, 3: 1, 4: 2, 6: 3, 7: 4}

HK_R = {0: ((0, 0, 1), (0, 2, -1), (1, 0, 1)), 1: ((0, 0, 1), (0, 1, -1), (2, 0, 1)),
        2: ((1, 1, 1), (1, 0, -1), (2, 1, 1)), 3: ((0, 1, 1), (1, 1, 1), (1, 2, -1)),
        4: ((1, 2, 1), (2, 0, -1), (2, 2, 1)), 5: ((0, 2, 1), (2, 1, -1), (2, 2, 1)),
        6: ((0, 1, 1), (1, 0, 1)), 9: ((0, 2, 1), (2, 0, 1)), 12: ((1, 2, 1), (2, 1, 1))}
HK_RS = {r: i for i, r in enumerate(HK_R)}
HK_RP = {7: (1, 0), 8: (0, 1), 10: (2, 0), 11: (0, 2), 13: (2, 1), 14: (1, 2)}
HK_LP = {0: (0, 0), 3: (1, 1), 4: (0, 2), 5: (1, 2)}
HK_LS = {r: i for i, r in enumerate((1, 2, 6, 7, 8, 9, 10, 11, 12, 13, 14))}
NSUM = 16


def _hk_lhs_sums(x, y):
    s0, s1, s2 = x[0] + y[0], x[1] + y[1], x[2] + y[2]
    return [s0, s1, x[0] + y[1], x[1] - x[0], y[0] - y[1], s0 - y[2], s2 - s0, y[2] - y[0],
            s1 - x[2], s2 - s1, x[2] - x[1]]


def _nn(a, b):
    return jnp.dot(a, b, preferred_element_type=F32)


def _nt(a, b):
    return jax.lax.dot_general(a, b, NT, preferred_element_type=F32)


def _weave(*lists):
    items = []
    for lst in lists:
        items += [((k + 0.5) / len(lst), w) for k, w in enumerate(lst)]
    items.sort(key=lambda t: t[0])
    return [t[1] for t in items]


def _kernel(x_hbm, wqkv_hbm, wo_hbm, wg_hbm, wu_hbm, wd_hbm, out_hbm,
            x_s, xn_s, xs_s, xn2_s, xs2_s, out_s, wqkv_r, wqkv_p, wo_r, wo_f, wo_p,
            wg_s, wu_s, wt_s, wd_s, t1_s, td_s, to_s, q_s, k_s, v_s, h_s, a_s, hold_s,
            zero_s, sem_i, sem_o):

    def zrow():
        return pl.multiple_of(zero_s[0] * 8, 8)

    masks_ = {}

    def keep(shape):
        if shape not in masks_:
            masks_[shape] = jax.lax.broadcasted_iota(jnp.int32, shape, len(shape) - 1) >= zero_s[0]
        return masks_[shape]

    def after(val, trig):
        if trig is None:
            return val
        n = val.shape[0] // 8
        t = pltpu.bitcast(trig, val.dtype) if trig.dtype != val.dtype else trig
        if n > 1:
            t = jnp.concatenate([t] * n, axis=0)
        return jnp.where(keep(val.shape), val, t)

    def after_head(val, trig):
        if trig is None:
            return val
        if val.shape[1] == 128:
            return after(val, trig)
        return jnp.concatenate([after(val[:, 0:128], trig), val[:, 128:]], axis=1)

    toks = []
    credit = [0.0]
    chain = [0]
    prev = []

    anchor = [False]
    extra = []

    def reset(dist):
        anchor[0] = False
        masks_.clear()
        del extra[:]
        del toks[:]
        del prev[:]
        credit[0] = 0.0
        chain[0] = dist

    def note(ref, row):
        if all(r is not ref for r, _ in toks):
            toks.append((ref, row))

    def gate(lhs):
        if not toks and not extra:
            return lhs
        tok = functools.reduce(lambda p, q: p | q, extra + [
            pltpu.bitcast(ref[pl.ds(zrow() + row, 8), 0:128], U32) for ref, row in toks])
        del toks[:]
        del extra[:]
        u = pltpu.bitcast(lhs[0:16], U32)
        return jnp.concatenate([_unpack(after_head(u, tok)), lhs[16:]], axis=0)

    def fire(work, res, per):
        if not work:
            credit[0] = 0.0
            return
        pos = credit[0]
        while pos < 1.0 and work:
            r = int((res.shape[0] - 8) * pos) // 8 * 8
            trig = pltpu.bitcast(res[r:r + 8, :], U32)
            item = work.pop(0)
            if item.func in (attn_rows, ln_pair) and len(prev) >= chain[0]:
                trig = trig | prev[-chain[0]]
            tok = item(trig)
            if tok is not None:
                prev.append(pltpu.bitcast(tok, U32))
            pos += 1.0 / per
        credit[0] = max(pos - 1.0, 0.0)

    lane = jax.lax.broadcasted_iota(jnp.int32, (32, 128), 1)
    l5 = lane % 5
    masks = [l5 == r for r in range(5)]
    idx = [(DH * (lane % H) + 5 * (lane // H) + j) % 128 for j in range(NJ)]

    def permute_qkv(t, r0, trig):
        src = [pltpu.bitcast(wqkv_r[r0:r0 + 64, t * D + s * 128:t * D + (s + 1) * 128], U32)
               for s in range(NJ)]
        src[4] = after(src[4], trig)
        for j in range(NJ):
            mg = src[4]
            for s in range(3, -1, -1):
                mg = jnp.where(masks[(j - 3 * s) % 5], src[s], mg)
            res = jnp.take_along_axis(mg, idx[j], axis=1, mode="promise_in_bounds")
            wqkv_p[r0 // 2:r0 // 2 + 32, t * D + j * 128:t * D + (j + 1) * 128] = res

    def widen_wo(jj, r0, trig):
        w = after(pltpu.bitcast(wo_r[r0:r0 + UW, jj * 128:(jj + 1) * 128], U32), trig)
        wo_f[jj * D + r0:jj * D + r0 + UW, :] = _unpack(w).astype(F32)

    def gather_wo(jj, j, trig):
        for g in range(4):
            rows = wo_f[pl.ds(jj * D + 5 * g + j, H, stride=DH), :]
            rows = jnp.concatenate([after(rows[r:r + 8], trig) if r % 16 == 0 else rows[r:r + 8]
                                    for r in range(0, H, 8)], axis=0)
            r0 = (j * 128 + g * H) // 2
            wo_p[r0:r0 + H // 2, jj * 128:(jj + 1) * 128] = _pack(rows)

    def prep(b11, b12, b21, b22, store, trig):
        b11, b12, b21, b22 = [b.astype(F32) for b in (b11, b12, b21, b22)]
        b11 = after(b11, trig)
        b22 = after(b22, trig)
        for i, s in enumerate(_rhs_sums(b11, b12, b21, b22)):
            store(i, _pack(s))

    def wtile(mat, k, n, r0=0, nr=128):
        if mat == 3:
            return wtile(n, k, 12, r0, nr) if n else wt_s[r0:r0 + nr, k * 128:(k + 1) * 128]
        if mat == 0:
            return _unpack(wqkv_p[k * 64 + r0 // 2:k * 64 + (r0 + nr) // 2, n * 128:(n + 1) * 128])
        return (wg_s, wu_s)[mat - 1][n * 128 + r0:n * 128 + r0 + nr, k * 128:(k + 1) * 128]

    def t_tri(mat, n0, i):
        return ((0, 80, 146, 212)[mat] + n0 // 3 * 9 + i) * 64

    def t_pair(mat, n0, i):
        return ((45, 116, 182, 221)[mat] + n0 // 2 * 5 + i) * 64

    def prep_tri(mat, n0, r0, trig):
        b = [[wtile(mat, k, n0 + n, r0, UT).astype(F32) for n in range(3)] for k in range(3)]
        for k, n in ((1, 0), (0, 1), (0, 2), (1, 2)):
            b[k][n] = after(b[k][n], trig)
        for r, terms in HK_R.items():
            s = None
            for k, n, c in terms:
                s = b[k][n] if s is None else (s + b[k][n] if c > 0 else s - b[k][n])
            row = t_tri(mat, n0, HK_RS[r]) + r0 // 2
            t1_s[row:row + UT // 2, :] = _pack(s)
            note(t1_s, row)

    def prep_pair(mat, n0, r0, trig):
        def store(i, o):
            row = t_pair(mat, n0, i) + r0 // 2
            t1_s[row:row + UP // 2, :] = o
            note(t1_s, row)
        prep(wtile(mat, 3, n0, r0, UP), wtile(mat, 3, n0 + 1, r0, UP),
             wtile(mat, 4, n0, r0, UP), wtile(mat, 4, n0 + 1, r0, UP), store, trig)

    def preps(mat, tris, pairs):
        return ([P(prep_tri, mat, n0, r0) for n0 in tris for r0 in range(0, 128, UT)]
                + [P(prep_pair, mat, n0, r0) for n0 in pairs for r0 in range(0, 128, UP)])

    def prep_d(r0, c, trig):
        def store(i, o):
            row = i * (FH // 2) + r0 // 2
            td_s[row:row + UD // 2, c:c + 128] = o
        prep(wd_s[r0:r0 + UD, c:c + 128], wd_s[r0:r0 + UD, 256 + c:384 + c],
             wd_s[FH + r0:FH + r0 + UD, c:c + 128], wd_s[FH + r0:FH + r0 + UD, 256 + c:384 + c], store, trig)

    def prep_o(r0, c, trig):
        n = UD // 2

        def store(i, o):
            to_s[i * 128 + r0:i * 128 + r0 + n, c:c + 128] = o
        prep(_unpack(wo_p[r0:r0 + n, c:c + 128]), _unpack(wo_p[r0:r0 + n, 256 + c:384 + c]),
             _unpack(wo_p[128 + r0:128 + r0 + n, c:c + 128]), _unpack(wo_p[128 + r0:128 + r0 + n, 256 + c:384 + c]),
             store, trig)

    def ln_rows(blk, r0, trig=None):
        x = after_head(x_s[blk, r0:r0 + LC, :].astype(F32), trig)
        m = jnp.sum(x, axis=-1, keepdims=True) * (1.0 / D)
        mb = m.astype(BF).astype(F32)
        xc = x - mb
        dm = m - mb
        var = jnp.sum(xc * xc, axis=-1, keepdims=True) * (1.0 / D) - dm * dm
        return xc * jax.lax.rsqrt(jnp.maximum(var, 0.0) + 1e-5)

    def ln_pair(blk, r0, xn_d, xs_d, trig):
        top = ln_rows(blk, r0, trig)
        bot = ln_rows(blk, HM1 + r0, trig)
        xn_d[r0 // 2:(r0 + LC) // 2, :] = _pack(top)
        xn_d[(HM1 + r0) // 2:(HM1 + r0 + LC) // 2, :] = _pack(bot)
        x = [top[:, k * 128:(k + 1) * 128] for k in range(NJ)]
        y = [bot[:, k * 128:(k + 1) * 128] for k in range(NJ)]
        for i, s in enumerate(_hk_lhs_sums(x, y) + _lhs_sums(x[3], x[4], y[3], y[4])):
            xs_d[i * HP + r0 // 2:i * HP + (r0 + LC) // 2, :] = _pack(s)
        note(xn_d, r0 // 2)
        note(xs_d, r0 // 2)
        s0 = x[0] + y[0]
        return s0[0:8] + s0[8:16]

    def tail_h(t):
        ht = _gelu(t) * pltpu.roll(t, 64, 1)
        lo = jax.lax.broadcasted_iota(jnp.int32, ht.shape, 1) < 64
        return jnp.where(lo, ht, 0.0)

    def store_qkv(c, row0, val):
        t, j = divmod(c, NJ)
        n = val.shape[0]
        if t == 0:
            q_s[j, row0:row0 + n, :] = val * (DH ** -0.5 * LOG2E)
        elif t == 1:
            k_s[j, HALO + row0:HALO + row0 + n, :] = val
        else:
            v_s[j, HALO + row0:HALO + row0 + n, :] = val

    def attn_core(r0, first, trig):
        q = q_s[:, r0:r0 + 8, :]
        if trig is not None:
            q = jnp.where(keep((NJ, 8, 128)), q, pltpu.bitcast(trig, F32)[None])
        logits = []
        for w in range(W):
            st = HALO + r0 - DIL * w
            acc = jnp.sum(q * k_s[:, st:st + 8, :], axis=0)
            acc = acc + pltpu.roll(acc, 64, 1)
            acc = acc + pltpu.roll(acc, 32, 1)
            if first and r0 < DIL * w:
                rows = r0 + jax.lax.broadcasted_iota(jnp.int32, (8, 128), 0)
                acc = jnp.where(rows >= DIL * w, acc, -1e9 * LOG2E)
            logits.append(acc)
        mx = logits[0]
        for w in range(1, W):
            mx = jnp.maximum(mx, logits[w])
        ps = [jnp.exp2(l - mx) for l in logits]
        den = ps[0]
        for w in range(1, W):
            den = den + ps[w]
        r = pl.reciprocal(den, approx=True)
        inv = r * (2.0 - den * r)
        acc = ps[0][None] * v_s[:, HALO + r0:HALO + r0 + 8, :]
        for w in range(1, W):
            st = HALO + r0 - DIL * w
            acc = acc + ps[w][None] * v_s[:, st:st + 8, :]
        return acc * inv[None], mx

    def attn_rows(r0, first, trig):
        o1, t1 = attn_core(r0, first, trig)
        o2, t2 = attn_core(r0 + 8, first, t1)
        for j in range(NJ):
            a_s[r0 // 2:(r0 + RC) // 2, j * 128:(j + 1) * 128] = _pack(jnp.concatenate([o1[j], o2[j]], axis=0))
        if anchor[0]:
            extra.append(pltpu.bitcast(pltpu.roll(jnp.max(jnp.maximum(o1, o2), axis=0), 64, 1), U32))
        return t2

    def cp_o(blk, base, r0, n, j):
        return pltpu.make_async_copy(out_s.at[blk, pl.ds(r0, n), pl.ds(j * 128, 128)],
                                     out_hbm.at[pl.ds(base + r0, n), pl.ds(j * 128, 128)], sem_o.at[0])

    def emit(blk, base, *pieces):
        for r0, j, val in pieces:
            n = val.shape[0]
            x = x_s[blk, r0:r0 + n, j * 128:(j + 1) * 128].astype(F32)
            out_s[blk, r0:r0 + n, j * 128:(j + 1) * 128] = (x + val).astype(BF)
        for r0, j, val in pieces:
            cp_o(blk, base, r0, val.shape[0], j).start()

    def stage2(blk, base, tm, works, pers, gated=True):
        hm, hp = tm // 2, tm // 4
        anchor[0] = gated

        def half(ref, r, c0, c1):
            return _unpack(ref[r * hp:(r + 1) * hp, c0:c1])

        memo = {}

        def lhs(plain, kh, i):
            if i == 3:
                return half(plain, 0, 0, kh)
            if i == 4:
                return half(plain, 1, kh, 2 * kh)
            if (kh, i) not in memo:
                def b(r, c):
                    u = plain[pl.ds(zrow(), 2 * hp), c * kh:(c + 1) * kh]
                    return _unpack(u[r * hp:(r + 1) * hp]).astype(F32)
                s = {1: lambda: b(0, 0) + b(1, 1), 2: lambda: b(1, 0) + b(1, 1), 5: lambda: b(0, 0) + b(0, 1),
                     6: lambda: b(1, 0) - b(0, 0), 7: lambda: b(0, 1) - b(1, 1)}[i]()
                memo[(kh, i)] = s.astype(BF)
            return memo[(kh, i)]

        f4 = []
        for r in range(2):
            if works[0] is works[1]:
                f = _nn(half(h_s, r, 0, FP), wd_s[:, 512:D])
                fire(works[0], f, pers[0])
            else:
                f = None
                for k0 in range(0, FP, 512):
                    k1 = min(k0 + 512, FP)
                    part = _nn(half(h_s, r, k0, k1), wd_s[k0:k1, 512:D])
                    fire(works[0], part, pers[0])
                    f = part if f is None else f + part
            f4.append(f)
        ffn = []
        for c in range(2):
            assert works[c] is works[c + 1] or not works[c]
            if c == 0 or works[1] is not works[2]:
                credit[0] = 0.0
            cs = (c * 128, 256 + c * 128)

            def p(i):
                if i == 2:
                    wd = wd_s[0:FH, cs[0]:cs[0] + 128]
                elif i == 5:
                    wd = wd_s[FH:FP, cs[1]:cs[1] + 128]
                else:
                    wd = _unpack(td_s[RS[i] * (FH // 2):(RS[i] + 1) * (FH // 2), cs[0]:cs[0] + 128])
                m = _nn(lhs(h_s, FH, i), wd)
                fire(works[c + 1], m, pers[c + 1])
                return m
            m4 = p(4)
            m2 = p(2)
            m1 = p(1)
            t11 = m1 + m4
            t22 = m1 - m2
            m3 = p(3)
            m5 = p(5)
            ffn.append((t11 - m5 + p(7), m3 + m5, m4 + m2, t22 + m3 + p(6)))
        assert not works[2]
        if not gated:
            del toks[:]
        k_s[:, 0:HALO, :] = k_s[:, tm:tm + HALO, :]
        v_s[:, 0:HALO, :] = v_s[:, tm:tm + HALO, :]
        for r in range(2):
            emit(blk, base, (r * hm, 4, f4[r] + _nn(gate(half(a_s, r, 0, D)), _unpack(wo_p[:, 512:D]))))
        for c in range(2):
            cs = (c * 128, 256 + c * 128)

            def p(i):
                if i == 2:
                    wo = wo_p[0:128, cs[0]:cs[0] + 128]
                elif i == 5:
                    wo = wo_p[128:256, cs[1]:cs[1] + 128]
                else:
                    wo = to_s[RS[i] * 128:(RS[i] + 1) * 128, cs[0]:cs[0] + 128]
                return _nn(lhs(a_s, 256, i), _unpack(wo))

            def left(r, cc):
                return ffn[c][2 * r + cc] + _nn(half(a_s, r, 512, D), _unpack(wo_p[256:320, cs[cc]:cs[cc] + 128]))
            l21 = left(1, 0)
            m4 = p(4)
            m2 = p(2)
            c21 = l21 + m4 + m2
            m1 = p(1)
            t11 = m1 + m4
            t22 = m1 - m2
            m3 = p(3)
            m5 = p(5)
            c12 = m3 + m5 + left(0, 1)
            c11 = t11 - m5 + p(7) + left(0, 0)
            c22 = t22 + m3 + p(6) + left(1, 1)
            emit(blk, base, (hm, c, c21))
            emit(blk, base, (0, c + 2, c12))
            emit(blk, base, (0, c, c11), (hm, c + 2, c22))

    def step(b):
        blk = b + 1
        base = pl.multiple_of(TM0 + b * TM1, 16)
        nblk = jnp.minimum(blk + 1, NL)
        reset(1)
        side = {}

        def xt(r, k):
            return _unpack(xn_s[r * HP:(r + 1) * HP, k * 128:(k + 1) * 128])

        def xsum(i):
            return _unpack(xs_s[i * HP:(i + 1) * HP, :])

        def mm(mat, l, w):
            return (_nn if mat == 0 else _nt)(l, w)

        def tick(v):
            fire(side['work'], v, side['per'])

        def hk(mat, n0, r):
            l = xt(*HK_LP[r]) if r in HK_LP else xsum(HK_LS[r])
            if r in HK_RP:
                w = wtile(mat, HK_RP[r][0], n0 + HK_RP[r][1])
            else:
                row = t_tri(mat, n0, HK_RS[r])
                w = _unpack(t1_s[row:row + 64, :])
            return mm(mat, l, w)

        def st(mat, n0, i):
            l = xt(0, 3) if i == 3 else xt(1, 4) if i == 4 else xsum(11 + LS[i])
            if i == 2:
                w = wtile(mat, 3, n0)
            elif i == 5:
                w = wtile(mat, 4, n0 + 1)
            else:
                row = t_pair(mat, n0, RS[i])
                w = _unpack(t1_s[row:row + 64, :])
            return mm(mat, l, w)

        def add(acc, key, v):
            acc[key] = v if key not in acc else acc[key] + v

        def s_a(acc, mat, n0):
            m1, m4, m5, m7 = [st(mat, n0, i) for i in (1, 4, 5, 7)]
            add(acc, (0, n0), (m1 + m4) + (m7 - m5))
            tick(acc[(0, n0)])
            add(acc, (1, n0 + 1), m1)
            add(acc, (1, n0), m4)
            add(acc, (0, n0 + 1), m5)

        def s_b(acc, mat, n0):
            m2, m3, m6 = [st(mat, n0, i) for i in (2, 3, 6)]
            add(acc, (1, n0), m2)
            add(acc, (0, n0 + 1), m3)
            add(acc, (1, n0 + 1), (m3 - m2) + m6)
            tick(acc[(1, n0 + 1)])

        def h_a(acc, mat, n0):
            r0, r9, r11, r10 = [hk(mat, n0, r) for r in (0, 9, 11, 10)]
            t = r9 + r11
            w0 = r0 + t
            add(acc, (0, n0), w0 + r10)
            tick(acc[(0, n0)])
            acc[(1, n0)] = acc[(1, n0)] - w0
            add(acc, (0, n0 + 2), t + r10)
            acc[(1, n0 + 2)] = acc[(1, n0 + 2)] - r11 if (1, n0 + 2) in acc else -r11

        def h_b(acc, mat, n0):
            r7, r6, r8, r1 = [hk(mat, n0, r) for r in (7, 6, 8, 1)]
            add(acc, (0, n0), r7)
            add(acc, (1, n0), (r1 + r6) + r8)
            tick(acc[(1, n0)])
            add(acc, (0, n0 + 1), r6 + r7)
            add(acc, (1, n0 + 1), r8)

        def h_c(acc, mat, n0):
            r3, r12, r14, r13 = [hk(mat, n0, r) for r in (3, 12, 14, 13)]
            t = r12 + r14
            w1 = r3 + t
            acc[(0, n0 + 1)] = acc[(0, n0 + 1)] - w1
            add(acc, (1, n0 + 1), w1 + r13)
            tick(acc[(1, n0 + 1)])
            acc[(0, n0 + 2)] = acc[(0, n0 + 2)] - r14
            add(acc, (1, n0 + 2), t + r13)

        def h_1(acc, mat, n0, r):
            add(acc, {2: (0, n0 + 1), 4: (0, n0 + 2), 5: (1, n0 + 2)}[r], hk(mat, n0, r))

        def group6(mat, n0, done, filler):
            acc = {}

            def fin(*keys):
                for key in keys:
                    done(key[0], key[1], acc.pop(key))
            s_a(acc, mat, n0)
            s_b(acc, mat, n0)
            h_1(acc, mat, n0, 2)
            h_a(acc, mat, n0)
            h_b(acc, mat, n0)
            fin((0, n0), (1, n0))
            h_c(acc, mat, n0)
            fin((0, n0 + 1), (1, n0 + 1))
            s_a(acc, mat, n0 + 2)
            s_b(acc, mat, n0 + 2)
            h_1(acc, mat, n0, 5)
            fin((1, n0 + 2))
            s_a(acc, mat, n0 + 4)
            s_b(acc, mat, n0 + 4)
            h_1(acc, mat, n0, 4)
            fin((0, n0 + 2))
            h_a(acc, mat, n0 + 3)
            h_b(acc, mat, n0 + 3)
            fin((0, n0 + 3), (1, n0 + 3))
            h_c(acc, mat, n0 + 3)
            fin((1, n0 + 4))
            for r in (2, 4, 5):
                h_1(acc, mat, n0 + 3, r)
            fin((0, n0 + 4), (0, n0 + 5), (1, n0 + 5))
            assert not acc
            filler()

        work = [P(ln_pair, nblk, k * LC, xn2_s, xs2_s) for k in range(HM1 // LC)]
        side.update(work=work, per=len(work) / LNSPAN)
        acc = {}
        plain = [(r, k) for k in (3, 4) for r in range(2)]

        def fill_q():
            r, k = plain.pop(0)
            add(acc, (r, 14), mm(0, xt(r, k), wtile(0, k, 14)))

        def done_q(r, n, val):
            store_qkv(n, r * HM1, val)

        def fin_q(*keys):
            for key in keys:
                done_q(key[0], key[1], acc.pop(key))
        fill_q()
        fill_q()
        group6(0, 0, done_q, fill_q)
        group6(0, 6, done_q, fill_q)
        s_a(acc, 0, 12)
        s_b(acc, 0, 12)
        h_1(acc, 0, 12, 2)
        h_a(acc, 0, 12)
        h_b(acc, 0, 12)
        fin_q((0, 12), (1, 12))
        h_c(acc, 0, 12)
        fin_q((0, 13), (1, 13))
        h_1(acc, 0, 12, 4)
        h_1(acc, 0, 12, 5)
        fin_q((0, 14), (1, 14))
        assert not work and not acc

        work = [P(attn_rows, c * RC, False) for c in range(TM1 // RC)]
        side.update(work=work, per=(len(work) - NA2) / 53.0)
        credit[0] = AOFF

        def store_h(r, n, v):
            h_s[r * HP:(r + 1) * HP, n * 128:(n + 1) * 128] = _pack(v)

        h_1(acc, 3, 0, 4)
        h_1(acc, 3, 0, 5)
        s_a(acc, 3, 0)
        s_b(acc, 3, 0)
        h_1(acc, 3, 0, 2)
        h_a(acc, 3, 0)
        h_b(acc, 3, 0)
        for r in range(2):
            store_h(r, 13, tail_h(acc.pop((r, 0))))
        h_c(acc, 3, 0)
        for r in range(2):
            hold_s[(12 + r) * HM1:(13 + r) * HM1, :] = _gelu(acc.pop((r, 1)))
        plain = [(r, k) for r in range(2) for k in (3, 4)]

        def fill_g():
            r, k = plain.pop(0)
            l = xt(r, k)
            add(acc, (r, 2), mm(3, gate(l) if len(plain) == 3 else l, wtile(3, k, 2)))
            if k == 4:
                store_h(r, 12, hold_s[(12 + r) * HM1:(13 + r) * HM1, :] * acc.pop((r, 2)))
        for n0 in (0, 6):
            def slot(r, n):
                s = (n - n0) * 2 + r
                return slice(s * HM1, (s + 1) * HM1)

            def done_g(r, n, v):
                hold_s[slot(r, n), :] = _gelu(v) if (r + n) % 2 == 0 else v

            def done_u(r, n, v):
                g = hold_s[slot(r, n), :]
                store_h(r, n, (g if (r + n) % 2 == 0 else _gelu(g)) * v)
            group6(1, n0, done_g, fill_g)
            group6(2, n0, done_u, fill_g)
        assert not plain and not acc
        note(hold_s, 0)

        def copy_xn(dst, src, r0, c, trig):
            dst[r0:r0 + HP, c:c + 128] = after(src[pl.ds(zrow(), r0 + HP), c:c + 128][r0:r0 + HP], trig)
            if c == 0:
                note(dst, r0)
        copies = [P(copy_xn, xn_s, xn2_s, r, c) for r in (0, HP) for c in range(0, D, 128)]
        copies += [P(copy_xn, xs_s, xs2_s, i * HP, 0) for i in range(NSUM)]
        mixed = _weave(work, copies)
        per = len(mixed) / (A2SPAN + 4.0)
        stage2(blk, base, TM1, [mixed] * 3, [2 * per, per, per])

    def cp(src, dst, s):
        return pltpu.make_async_copy(src, dst, sem_i.at[s])

    def gu(groups, s):
        return [cp(h.at[pl.ds(g * 128, 128)], d.at[pl.ds(g * 128, 128)], s)
                for g in groups for h, d in ((wg_hbm, wg_s), (wu_hbm, wu_s))]

    def wcol(t, s):
        return cp(wqkv_hbm.at[:, pl.ds(t * D, D)], wqkv_r.at[:, pl.ds(t * D, D)], s)

    def xblk(b, s):
        return cp(x_hbm.at[pl.ds(TM0 + b * TM1, TM1)], x_s.at[b + 1, pl.ds(0, TM1)], s)

    HM = TM0 // 2
    cp_x0 = [cp(x_hbm.at[pl.ds(i * HM, HM)], x_s.at[0, pl.ds(i * HM, HM)], i) for i in range(2)]
    cp_gu = [gu(g, 2 + k) for k, g in enumerate(G_EARLY)]
    cp_q = gu(G_Q, 5) + [cp(wg_hbm.at[pl.ds(FM, 64)], wt_s.at[pl.ds(0, 64)], 5),
                         cp(wu_hbm.at[pl.ds(FM, 64)], wt_s.at[pl.ds(64, 64)], 5), wcol(0, 5), xblk(0, 5)]
    cp_kv = gu(G_KV, 6) + [wcol(1, 6), wcol(2, 6)]
    cp_r = gu(G_R + G_D, 7) + [cp(wo_hbm, wo_r, 7)]
    cp_d = [cp(wd_hbm, wd_s.at[pl.ds(0, F)], 8)]
    cp_xs = [xblk(b, 9) for b in range(1, NL)]

    for c in cp_x0 + sum(cp_gu, []) + cp_q + cp_kv + cp_r + cp_d + cp_xs:
        c.start()
    zero_s[0] = 0
    k_s[:, 0:HALO, :] = jnp.zeros((NJ, HALO, 128), F32)
    v_s[:, 0:HALO, :] = jnp.zeros((NJ, HALO, 128), F32)
    wd_s[F:FP, :] = jnp.zeros((FP - F, D), BF)

    def first_block():
        def wait(cps, name):
            reset(CH0)
            with _scope(name):
                for c in cps:
                    c.wait()

        parts = []
        for i in range(2):
            wait(cp_x0[i:i + 1], 'waitx')
            parts += [ln_rows(0, i * HM + k * LC).astype(BF) for k in range(HM // LC)]
        xn = jnp.concatenate(parts, axis=0)

        def ffn_group(x, row0, g0, work, per, gated=False):
            g = _nt(x, wg_s[g0 * 128:(g0 + 1) * 128, :])
            fire(work, g, per)
            u = _nt(gate(x) if gated else x, wu_s[g0 * 128:(g0 + 1) * 128, :])
            fire(work, u, per)
            h_s[row0 // 2:(row0 + x.shape[0]) // 2, g0 * 128:(g0 + 1) * 128] = _pack(_gelu(g) * u)

        def ffn_groups(groups, work, per, gate_last=False):
            groups = list(groups)
            if len(groups) % 2:
                g0 = groups.pop(0)
                ffn_group(xn[0:HM], 0, g0, work, per)
                ffn_group(xn[HM:], HM, g0, work, per)
            for k, g0 in enumerate(groups):
                ffn_group(xn, 0, g0, work, per, gate_last and k == len(groups) - 1)

        have, done = set(), set()

        def new_preps(groups):
            have.update(groups)
            tris = [n for n in (0, 3, 6, 9) if {n, n + 1, n + 2} <= have and ('t', n) not in done]
            pairs = [n for n in range(0, 12, 2) if {n, n + 1} <= have and ('p', n) not in done]
            done.update([('t', n) for n in tris] + [('p', n) for n in pairs])
            return preps(1, tris, pairs) + preps(2, tris, pairs)

        perm = [[P(permute_qkv, t, r0) for r0 in range(0, D, 64)] for t in range(3)]

        for k, (cps, groups) in enumerate(zip(cp_gu, G_EARLY)):
            wait(cps, 'waitgu')
            work = new_preps(groups)
            nres = 2 * len(groups) + 2 * (len(groups) % 2)
            ffn_groups(groups, work, max(len(work), 1) / max(nres - 2.0, 1.0), k == 2)
            assert not work

        wait(cp_q, 'waitq')
        work = perm[0]
        for _ in range(3):
            work.pop(0)(None)
        t = _nt(xn, wt_s[...])
        fire(work, t, 4)
        h_s[0:TM0 // 2, FM:FP] = _pack(tail_h(t))
        work += new_preps(G_Q) + [P(ln_pair, 1, k * LC, xn_s, xs_s) for k in range(HM1 // LC)]
        for g0 in G_Q:
            ffn_group(xn, 0, g0, work, QPER)
        assert all(w.func is ln_pair for w in work)
        per = len(work) / QSPAN
        for j in range(NJ):
            r = _nn(xn, _unpack(wqkv_p[:, j * 128:(j + 1) * 128]))
            fire(work, r, per)
            store_qkv(j, 0, r)
        assert not work

        wait(cp_kv, 'waitkv')
        work = perm[1]
        for _ in range(4):
            work.pop(0)(None)
        for g0 in G_KV:
            g = _nt(xn, wg_s[g0 * 128:(g0 + 1) * 128, :])
            fire(work, g, 6)
            u = _nt(xn, wu_s[g0 * 128:(g0 + 1) * 128, :])
            h_s[0:TM0 // 2, g0 * 128:(g0 + 1) * 128] = _pack(_gelu(g) * u)
        assert not work
        work = perm[2] + _weave(new_preps(G_KV), _weave(preps(0, range(0, 15, 3), []),
                                                        preps(0, [], range(0, 14, 2))))
        per = len(work) / KVSPAN
        fire(work, u, per)
        for c in range(NJ, 3 * NJ):
            assert c < 2 * NJ or all(w.func is not permute_qkv for w in work)
            r = _nn(gate(xn) if c == 3 * NJ - 1 else xn, _unpack(wqkv_p[:, c * 128:(c + 1) * 128]))
            fire(work, r, per)
            store_qkv(c, 0, r)
        assert not work

        wait(cp_r, 'waitr')
        att = [P(attn_rows, rc * RC, True) for rc in range(TM0 // RC)]
        work = _weave(new_preps(G_R + G_D) + preps(3, [0], [0]), att[:NAR])
        att = att[NAR:]
        ffn_groups(G_R, work, len(work) / (2 * len(G_R) - 2.0))
        assert not work

        wait(cp_d, 'waitd')
        chain[0] = CHD
        wo_work = []
        for jj in range(NJ):
            wo_work += [P(widen_wo, jj, r0) for r0 in range(0, D, UW)]
            wo_work += [P(gather_wo, jj, j) for j in range(NJ)]
        pd = [P(prep_d, r0, c) for c in (0, 128) for r0 in range(0, FH, UD)]
        po = [P(prep_o, r0, c) for r0 in range(0, 128, UD // 2) for c in (0, 128)]
        wa = _weave(pd, wo_work, att[:NAA])
        wb = _weave(po, att[NAA:NAA + NAB])
        wc = att[NAA + NAB:]
        for _ in range(2):
            wa.pop(0)(None)
        per = len(wa) / SPANA
        ffn_groups(G_D, wa, per)
        stage2(0, 0, TM0, [wa, wb, wc], [per, len(wb) / SPANB, len(wc) / SPANC], False)

    def main(i, carry):
        with _scope('step0'):
            first_block()
        for c in cp_xs:
            c.wait()

        def body(b, c):
            with _scope('stepb'):
                step(b)
            return c
        return jax.lax.fori_loop(0, NL, body, carry)

    jax.lax.fori_loop(0, zero_s[0] + 1, main, 0)

    with _scope('waitout'):
        for j in range(NJ):
            for r in range(2):
                cp_o(0, 0, r * HM, HM, j).wait()
        for b in range(NL):
            for j in range(NJ):
                for r in range(2):
                    cp_o(b + 1, TM0 + b * TM1, r * HM1, HM1, j).wait()


@jax.jit
def pallas_parallel_sum__sliding_local_dilated__geglu_ffn__prompt_kernel(
    A_x: jax.Array,
    A_wqkv: jax.Array,
    A_wo: jax.Array,
    B_x: jax.Array,
    B_w_gate: jax.Array,
    B_w_up: jax.Array,
    B_w_down: jax.Array,
):
    x = A_x.reshape(S, D)
    hbm = pl.BlockSpec(memory_space=pltpu.MemorySpace.HBM)
    out = pl.pallas_call(
        _kernel,
        in_specs=[hbm] * 6,
        out_specs=hbm,
        out_shape=jax.ShapeDtypeStruct((S, D), BF),
        scratch_shapes=[
            pltpu.VMEM((NL + 1, TMP, D), BF),
            pltpu.VMEM((TM1 // 2, D), U32),
            pltpu.VMEM((NSUM * HP, 128), U32),
            pltpu.VMEM((TM1 // 2, D), U32),
            pltpu.VMEM((NSUM * HP, 128), U32),
            pltpu.VMEM((NL + 1, TMP, D), BF),
            pltpu.VMEM((D, 3 * D), BF),
            pltpu.VMEM((D // 2, 3 * D), U32),
            pltpu.VMEM((D, D), BF),
            pltpu.VMEM((NJ * D, 128), F32),
            pltpu.VMEM((D // 2, D), U32),
            pltpu.VMEM((FM, D), BF),
            pltpu.VMEM((FM, D), BF),
            pltpu.VMEM((128, D), BF),
            pltpu.VMEM((FP, D), BF),
            pltpu.VMEM((226 * 64, 128), U32),
            pltpu.VMEM((5 * FH // 2, 256), U32),
            pltpu.VMEM((5 * 128, 256), U32),
            pltpu.VMEM((NJ, TMX, 128), F32),
            pltpu.VMEM((NJ, TMX + HALO, 128), F32),
            pltpu.VMEM((NJ, TMX + HALO, 128), F32),
            pltpu.VMEM((TMX // 2, FP), U32),
            pltpu.VMEM((TMX // 2, D), U32),
            pltpu.VMEM((NHOLD * HM1, 128), F32),
            pltpu.SMEM((1,), jnp.int32),
            pltpu.SemaphoreType.DMA((10,)),
            pltpu.SemaphoreType.DMA((1,)),
        ],
        compiler_params=pltpu.CompilerParams(
            vmem_limit_bytes=100 * 1024 * 1024,
            disable_bounds_checks=True,
            disable_semaphore_checks=True,
        ),
    )(x, A_wqkv, A_wo, B_w_gate.T, B_w_up.T, B_w_down)
    return out.reshape(1, S, D)
```

```python
import contextlib
import functools

import jax
import jax.numpy as jnp
import jax.experimental.pallas as pl
import jax.experimental.pallas.tpu as pltpu

S, D, H, DH, W, DIL, F = 2048, 640, 32, 20, 8, 2, 1728
TM0 = 384
NL = 4
TM1 = (S - TM0) // NL
HM1 = TM1 // 2
HP = HM1 // 2
TMX = max(TM0, TM1)
TMP = (TMX + 63) // 64 * 64
HALO = 16
NJ = D // 128
LOG2E = 1.4426950408889634
FM = 1664
FP = 1792
FH = FP // 2
RC = 16
LC = 16
NHOLD = 14
G_EARLY = [[0], [1, 2], [3, 4, 5]]
G_Q, G_KV, G_R, G_D = [6], [7], [8, 9, 10, 11], [12]
LNSPAN = 24
APER = 0.377
LOFF = 0
GPAT = 0x999
A2SPAN = 7
AOFF = 4
NAR = 3
NAA = 8
NAB = 8
SPANA = 11
SPANB = 5
SPANC = 5
KVSPAN = 8
QPER = 1.5
QSPAN = 3.5
CH0 = 3
CHD = 2
UT = 16
UP = 32
UD = 16
UW = 64
SCOPES = 0

BF = jnp.bfloat16
F32 = jnp.float32
U32 = jnp.uint32
NT = (((1,), (1,)), ((), ()))
P = functools.partial


def _scope(name):
    return jax.named_scope(name) if SCOPES else contextlib.nullcontext()


def _gelu(g):
    c0 = 0.7978845608028654
    c1 = c0 * 0.044715
    t = jnp.tanh(g * (c0 + c1 * (g * g)))
    hg = 0.5 * g
    return hg + hg * t


def _pack(x):
    return pltpu.bitcast(x.astype(BF), U32)


def _unpack(u):
    return pltpu.bitcast(u, BF)


def _lhs_sums(a11, a12, a21, a22):
    return [a11 + a22, a21 + a22, a11 + a12, a21 - a11, a12 - a22]


def _rhs_sums(b11, b12, b21, b22):
    return [b11 + b22, b12 - b22, b21 - b11, b11 + b12, b21 + b22]


LS = {1: 0, 2: 1, 5: 2, 6: 3, 7: 4}
RS = {1: 0, 3: 1, 4: 2, 6: 3, 7: 4}

HK_R = {0: ((0, 0, 1), (0, 2, -1), (1, 0, 1)), 1: ((0, 0, 1), (0, 1, -1), (2, 0, 1)),
        2: ((1, 1, 1), (1, 0, -1), (2, 1, 1)), 3: ((0, 1, 1), (1, 1, 1), (1, 2, -1)),
        4: ((1, 2, 1), (2, 0, -1), (2, 2, 1)), 5: ((0, 2, 1), (2, 1, -1), (2, 2, 1)),
        6: ((0, 1, 1), (1, 0, 1)), 9: ((0, 2, 1), (2, 0, 1)), 12: ((1, 2, 1), (2, 1, 1))}
HK_RS = {r: i for i, r in enumerate(HK_R)}
HK_RP = {7: (1, 0), 8: (0, 1), 10: (2, 0), 11: (0, 2), 13: (2, 1), 14: (1, 2)}
HK_LP = {0: (0, 0), 3: (1, 1), 4: (0, 2), 5: (1, 2)}
HK_LS = {r: i for i, r in enumerate((1, 2, 6, 7, 8, 9, 10, 11, 12, 13, 14))}
NSUM = 16


def _hk_lhs_sums(x, y):
    s0, s1, s2 = x[0] + y[0], x[1] + y[1], x[2] + y[2]
    return [s0, s1, x[0] + y[1], x[1] - x[0], y[0] - y[1], s0 - y[2], s2 - s0, y[2] - y[0],
            s1 - x[2], s2 - s1, x[2] - x[1]]


def _nn(a, b):
    return jnp.dot(a, b, preferred_element_type=F32)


def _nt(a, b):
    return jax.lax.dot_general(a, b, NT, preferred_element_type=F32)


def _weave(*lists):
    items = []
    for lst in lists:
        items += [((k + 0.5) / len(lst), w) for k, w in enumerate(lst)]
    items.sort(key=lambda t: t[0])
    return [t[1] for t in items]


def _kernel(x_hbm, wqkv_hbm, wo_hbm, wg_hbm, wu_hbm, wd_hbm, out_hbm,
            x_s, xn_s, xs_s, xn2_s, xs2_s, out_s, wqkv_r, wqkv_p, wo_r, wo_f, wo_p,
            wg_s, wu_s, wt_s, wd_s, t1_s, td_s, to_s, q_s, k_s, v_s, h_s, a_s, hold_s,
            zero_s, sem_i, sem_o):

    def zrow():
        return pl.multiple_of(zero_s[0] * 8, 8)

    masks_ = {}

    def keep(shape):
        if shape not in masks_:
            masks_[shape] = jax.lax.broadcasted_iota(jnp.int32, shape, len(shape) - 1) >= zero_s[0]
        return masks_[shape]

    def after(val, trig):
        if trig is None:
            return val
        n = val.shape[0] // 8
        t = pltpu.bitcast(trig, val.dtype) if trig.dtype != val.dtype else trig
        if n > 1:
            t = jnp.concatenate([t] * n, axis=0)
        return jnp.where(keep(val.shape), val, t)

    def after_head(val, trig):
        if trig is None:
            return val
        if val.shape[1] == 128:
            return after(val, trig)
        return jnp.concatenate([after(val[:, 0:128], trig), val[:, 128:]], axis=1)

    toks = []
    credit = [0.0]
    chain = [0]
    prev = []

    anchor = [False]
    extra = []

    def reset(dist):
        anchor[0] = False
        masks_.clear()
        del extra[:]
        del toks[:]
        del prev[:]
        credit[0] = 0.0
        chain[0] = dist

    def note(ref, row):
        if all(r is not ref for r, _ in toks):
            toks.append((ref, row))

    def gate(lhs):
        if not toks and not extra:
            return lhs
        tok = functools.reduce(lambda p, q: p | q, extra + [
            pltpu.bitcast(ref[pl.ds(zrow() + row, 8), 0:128], U32) for ref, row in toks])
        del toks[:]
        del extra[:]
        u = pltpu.bitcast(lhs[0:16], U32)
        return jnp.concatenate([_unpack(after_head(u, tok)), lhs[16:]], axis=0)

    def fire(work, res, per):
        if not work:
            credit[0] = 0.0
            return
        pos = credit[0]
        while pos < 1.0 and work:
            r = int((res.shape[0] - 8) * pos) // 8 * 8
            trig = pltpu.bitcast(res[r:r + 8, :], U32)
            item = work.pop(0)
            if item.func in (attn_rows, ln_pair) and len(prev) >= chain[0]:
                trig = trig | prev[-chain[0]]
            tok = item(trig)
            if tok is not None:
                prev.append(pltpu.bitcast(tok, U32))
            pos += 1.0 / per
        credit[0] = max(pos - 1.0, 0.0)

    lane = jax.lax.broadcasted_iota(jnp.int32, (32, 128), 1)
    l5 = lane % 5
    masks = [l5 == r for r in range(5)]
    idx = [(DH * (lane % H) + 5 * (lane // H) + j) % 128 for j in range(NJ)]

    def permute_qkv(t, r0, trig):
        src = [pltpu.bitcast(wqkv_r[r0:r0 + 64, t * D + s * 128:t * D + (s + 1) * 128], U32)
               for s in range(NJ)]
        src[4] = after(src[4], trig)
        for j in range(NJ):
            mg = src[4]
            for s in range(3, -1, -1):
                mg = jnp.where(masks[(j - 3 * s) % 5], src[s], mg)
            res = jnp.take_along_axis(mg, idx[j], axis=1, mode="promise_in_bounds")
            wqkv_p[r0 // 2:r0 // 2 + 32, t * D + j * 128:t * D + (j + 1) * 128] = res

    def widen_wo(jj, r0, trig):
        w = after(pltpu.bitcast(wo_r[r0:r0 + UW, jj * 128:(jj + 1) * 128], U32), trig)
        wo_f[jj * D + r0:jj * D + r0 + UW, :] = _unpack(w).astype(F32)

    def gather_wo(jj, j, trig):
        for g in range(4):
            rows = wo_f[pl.ds(jj * D + 5 * g + j, H, stride=DH), :]
            rows = jnp.concatenate([after(rows[r:r + 8], trig) if r % 16 == 0 else rows[r:r + 8]
                                    for r in range(0, H, 8)], axis=0)
            r0 = (j * 128 + g * H) // 2
            wo_p[r0:r0 + H // 2, jj * 128:(jj + 1) * 128] = _pack(rows)

    def prep(b11, b12, b21, b22, store, trig):
        b11, b12, b21, b22 = [b.astype(F32) for b in (b11, b12, b21, b22)]
        b11 = after(b11, trig)
        b22 = after(b22, trig)
        for i, s in enumerate(_rhs_sums(b11, b12, b21, b22)):
            store(i, _pack(s))

    def wtile(mat, k, n, r0=0, nr=128):
        if mat == 3:
            return wtile(n, k, 12, r0, nr) if n else wt_s[r0:r0 + nr, k * 128:(k + 1) * 128]
        if mat == 0:
            return _unpack(wqkv_p[k * 64 + r0 // 2:k * 64 + (r0 + nr) // 2, n * 128:(n + 1) * 128])
        return (wg_s, wu_s)[mat - 1][n * 128 + r0:n * 128 + r0 + nr, k * 128:(k + 1) * 128]

    def t_tri(mat, n0, i):
        return ((0, 80, 146, 212)[mat] + n0 // 3 * 9 + i) * 64

    def t_pair(mat, n0, i):
        return ((45, 116, 182, 221)[mat] + n0 // 2 * 5 + i) * 64

    def prep_tri(mat, n0, r0, trig):
        b = [[wtile(mat, k, n0 + n, r0, UT).astype(F32) for n in range(3)] for k in range(3)]
        for k, n in ((1, 0), (0, 1), (0, 2), (1, 2)):
            b[k][n] = after(b[k][n], trig)
        for r, terms in HK_R.items():
            s = None
            for k, n, c in terms:
                s = b[k][n] if s is None else (s + b[k][n] if c > 0 else s - b[k][n])
            row = t_tri(mat, n0, HK_RS[r]) + r0 // 2
            t1_s[row:row + UT // 2, :] = _pack(s)
            note(t1_s, row)

    def prep_pair(mat, n0, r0, trig):
        def store(i, o):
            row = t_pair(mat, n0, i) + r0 // 2
            t1_s[row:row + UP // 2, :] = o
            note(t1_s, row)
        prep(wtile(mat, 3, n0, r0, UP), wtile(mat, 3, n0 + 1, r0, UP),
             wtile(mat, 4, n0, r0, UP), wtile(mat, 4, n0 + 1, r0, UP), store, trig)

    def preps(mat, tris, pairs):
        return ([P(prep_tri, mat, n0, r0) for n0 in tris for r0 in range(0, 128, UT)]
                + [P(prep_pair, mat, n0, r0) for n0 in pairs for r0 in range(0, 128, UP)])

    def prep_d(r0, c, trig):
        def store(i, o):
            row = i * (FH // 2) + r0 // 2
            td_s[row:row + UD // 2, c:c + 128] = o
        prep(wd_s[r0:r0 + UD, c:c + 128], wd_s[r0:r0 + UD, 256 + c:384 + c],
             wd_s[FH + r0:FH + r0 + UD, c:c + 128], wd_s[FH + r0:FH + r0 + UD, 256 + c:384 + c], store, trig)

    def prep_o(r0, c, trig):
        n = UD // 2

        def store(i, o):
            to_s[i * 128 + r0:i * 128 + r0 + n, c:c + 128] = o
        prep(_unpack(wo_p[r0:r0 + n, c:c + 128]), _unpack(wo_p[r0:r0 + n, 256 + c:384 + c]),
             _unpack(wo_p[128 + r0:128 + r0 + n, c:c + 128]), _unpack(wo_p[128 + r0:128 + r0 + n, 256 + c:384 + c]),
             store, trig)

    def ln_rows(blk, r0, trig=None):
        x = after_head(x_s[blk, r0:r0 + LC, :].astype(F32), trig)
        m = jnp.sum(x, axis=-1, keepdims=True) * (1.0 / D)
        mb = m.astype(BF).astype(F32)
        xc = x - mb
        dm = m - mb
        var = jnp.sum(xc * xc, axis=-1, keepdims=True) * (1.0 / D) - dm * dm
        return xc * jax.lax.rsqrt(jnp.maximum(var, 0.0) + 1e-5)

    def ln_pair(blk, r0, xn_d, xs_d, trig):
        top = ln_rows(blk, r0, trig)
        bot = ln_rows(blk, HM1 + r0, trig)
        xn_d[r0 // 2:(r0 + LC) // 2, :] = _pack(top)
        xn_d[(HM1 + r0) // 2:(HM1 + r0 + LC) // 2, :] = _pack(bot)
        x = [top[:, k * 128:(k + 1) * 128] for k in range(NJ)]
        y = [bot[:, k * 128:(k + 1) * 128] for k in range(NJ)]
        for i, s in enumerate(_hk_lhs_sums(x, y) + _lhs_sums(x[3], x[4], y[3], y[4])):
            xs_d[i * HP + r0 // 2:i * HP + (r0 + LC) // 2, :] = _pack(s)
        note(xn_d, r0 // 2)
        note(xs_d, r0 // 2)
        s0 = x[0] + y[0]
        return s0[0:8] + s0[8:16]

    def tail_h(t):
        ht = _gelu(t) * pltpu.roll(t, 64, 1)
        lo = jax.lax.broadcasted_iota(jnp.int32, ht.shape, 1) < 64
        return jnp.where(lo, ht, 0.0)

    def store_qkv(c, row0, val):
        t, j = divmod(c, NJ)
        n = val.shape[0]
        if t == 0:
            q_s[j, row0:row0 + n, :] = val * (DH ** -0.5 * LOG2E)
        elif t == 1:
            k_s[j, HALO + row0:HALO + row0 + n, :] = val
        else:
            v_s[j, HALO + row0:HALO + row0 + n, :] = val

    def attn_core(r0, first, trig):
        q = q_s[:, r0:r0 + 8, :]
        if trig is not None:
            q = jnp.where(keep((NJ, 8, 128)), q, pltpu.bitcast(trig, F32)[None])
        logits = []
        for w in range(W):
            st = HALO + r0 - DIL * w
            acc = jnp.sum(q * k_s[:, st:st + 8, :], axis=0)
            acc = acc + pltpu.roll(acc, 64, 1)
            acc = acc + pltpu.roll(acc, 32, 1)
            if first and r0 < DIL * w:
                rows = r0 + jax.lax.broadcasted_iota(jnp.int32, (8, 128), 0)
                acc = jnp.where(rows >= DIL * w, acc, -1e9 * LOG2E)
            logits.append(acc)
        mx = logits[0]
        for w in range(1, W):
            mx = jnp.maximum(mx, logits[w])
        ps = [jnp.exp2(l - mx) for l in logits]
        den = ps[0]
        for w in range(1, W):
            den = den + ps[w]
        r = pl.reciprocal(den, approx=True)
        inv = r * (2.0 - den * r)
        acc = ps[0][None] * v_s[:, HALO + r0:HALO + r0 + 8, :]
        for w in range(1, W):
            st = HALO + r0 - DIL * w
            acc = acc + ps[w][None] * v_s[:, st:st + 8, :]
        return acc * inv[None], mx

    def attn_rows(r0, first, trig):
        o1, t1 = attn_core(r0, first, trig)
        o2, t2 = attn_core(r0 + 8, first, t1)
        for j in range(NJ):
            a_s[r0 // 2:(r0 + RC) // 2, j * 128:(j + 1) * 128] = _pack(jnp.concatenate([o1[j], o2[j]], axis=0))
        if anchor[0]:
            extra.append(pltpu.bitcast(pltpu.roll(jnp.max(jnp.maximum(o1, o2), axis=0), 64, 1), U32))
        return t2

    def cp_o(blk, base, r0, n, j):
        return pltpu.make_async_copy(out_s.at[blk, pl.ds(r0, n), pl.ds(j * 128, 128)],
                                     out_hbm.at[pl.ds(base + r0, n), pl.ds(j * 128, 128)], sem_o.at[0])

    def emit(blk, base, *pieces):
        for r0, j, val in pieces:
            n = val.shape[0]
            x = x_s[blk, r0:r0 + n, j * 128:(j + 1) * 128].astype(F32)
            out_s[blk, r0:r0 + n, j * 128:(j + 1) * 128] = (x + val).astype(BF)
        for r0, j, val in pieces:
            cp_o(blk, base, r0, val.shape[0], j).start()

    def stage2(blk, base, tm, works, pers, gated=True):
        hm, hp = tm // 2, tm // 4
        anchor[0] = gated

        def half(ref, r, c0, c1):
            return _unpack(ref[r * hp:(r + 1) * hp, c0:c1])

        memo = {}

        def lhs(plain, kh, i):
            if i == 3:
                return half(plain, 0, 0, kh)
            if i == 4:
                return half(plain, 1, kh, 2 * kh)
            if (kh, i) not in memo:
                def b(r, c):
                    u = plain[pl.ds(zrow(), 2 * hp), c * kh:(c + 1) * kh]
                    return _unpack(u[r * hp:(r + 1) * hp]).astype(F32)
                s = {1: lambda: b(0, 0) + b(1, 1), 2: lambda: b(1, 0) + b(1, 1), 5: lambda: b(0, 0) + b(0, 1),
                     6: lambda: b(1, 0) - b(0, 0), 7: lambda: b(0, 1) - b(1, 1)}[i]()
                memo[(kh, i)] = s.astype(BF)
            return memo[(kh, i)]

        f4 = []
        for r in range(2):
            if works[0] is works[1]:
                f = _nn(half(h_s, r, 0, FP), wd_s[:, 512:D])
                fire(works[0], f, pers[0])
            else:
                f = None
                for k0 in range(0, FP, 512):
                    k1 = min(k0 + 512, FP)
                    part = _nn(half(h_s, r, k0, k1), wd_s[k0:k1, 512:D])
                    fire(works[0], part, pers[0])
                    f = part if f is None else f + part
            f4.append(f)
        ffn = []
        for c in range(2):
            assert works[c] is works[c + 1] or not works[c]
            if c == 0 or works[1] is not works[2]:
                credit[0] = 0.0
            cs = (c * 128, 256 + c * 128)

            def p(i):
                if i == 2:
                    wd = wd_s[0:FH, cs[0]:cs[0] + 128]
                elif i == 5:
                    wd = wd_s[FH:FP, cs[1]:cs[1] + 128]
                else:
                    wd = _unpack(td_s[RS[i] * (FH // 2):(RS[i] + 1) * (FH // 2), cs[0]:cs[0] + 128])
                m = _nn(lhs(h_s, FH, i), wd)
                fire(works[c + 1], m, pers[c + 1])
                return m
            m4 = p(4)
            m2 = p(2)
            m1 = p(1)
            t11 = m1 + m4
            t22 = m1 - m2
            m3 = p(3)
            m5 = p(5)
            ffn.append((t11 - m5 + p(7), m3 + m5, m4 + m2, t22 + m3 + p(6)))
        assert not works[2]
        if not gated:
            del toks[:]
        k_s[:, 0:HALO, :] = k_s[:, tm:tm + HALO, :]
        v_s[:, 0:HALO, :] = v_s[:, tm:tm + HALO, :]
        for r in range(2):
            emit(blk, base, (r * hm, 4, f4[r] + _nn(gate(half(a_s, r, 0, D)), _unpack(wo_p[:, 512:D]))))
        for c in range(2):
            cs = (c * 128, 256 + c * 128)

            def p(i):
                if i == 2:
                    wo = wo_p[0:128, cs[0]:cs[0] + 128]
                elif i == 5:
                    wo = wo_p[128:256, cs[1]:cs[1] + 128]
                else:
                    wo = to_s[RS[i] * 128:(RS[i] + 1) * 128, cs[0]:cs[0] + 128]
                return _nn(lhs(a_s, 256, i), _unpack(wo))

            def left(r, cc):
                return ffn[c][2 * r + cc] + _nn(half(a_s, r, 512, D), _unpack(wo_p[256:320, cs[cc]:cs[cc] + 128]))
            l21 = left(1, 0)
            m4 = p(4)
            m2 = p(2)
            c21 = l21 + m4 + m2
            m1 = p(1)
            t11 = m1 + m4
            t22 = m1 - m2
            m3 = p(3)
            m5 = p(5)
            c12 = m3 + m5 + left(0, 1)
            c11 = t11 - m5 + p(7) + left(0, 0)
            c22 = t22 + m3 + p(6) + left(1, 1)
            emit(blk, base, (hm, c, c21))
            emit(blk, base, (0, c + 2, c12))
            emit(blk, base, (0, c, c11), (hm, c + 2, c22))

    def step(b):
        blk = b + 1
        base = pl.multiple_of(TM0 + b * TM1, 16)
        nblk = jnp.minimum(blk + 1, NL)
        reset(1)
        side = {}

        def xt(r, k):
            return _unpack(xn_s[r * HP:(r + 1) * HP, k * 128:(k + 1) * 128])

        def xsum(i):
            return _unpack(xs_s[i * HP:(i + 1) * HP, :])

        def mm(mat, l, w):
            return (_nn if mat == 0 else _nt)(l, w)

        def tick(v):
            fire(side['work'], v, side['per'])

        def hk(mat, n0, r):
            l = xt(*HK_LP[r]) if r in HK_LP else xsum(HK_LS[r])
            if r in HK_RP:
                w = wtile(mat, HK_RP[r][0], n0 + HK_RP[r][1])
            else:
                row = t_tri(mat, n0, HK_RS[r])
                w = _unpack(t1_s[row:row + 64, :])
            return mm(mat, l, w)

        def st(mat, n0, i):
            l = xt(0, 3) if i == 3 else xt(1, 4) if i == 4 else xsum(11 + LS[i])
            if i == 2:
                w = wtile(mat, 3, n0)
            elif i == 5:
                w = wtile(mat, 4, n0 + 1)
            else:
                row = t_pair(mat, n0, RS[i])
                w = _unpack(t1_s[row:row + 64, :])
            return mm(mat, l, w)

        def add(acc, key, v):
            acc[key] = v if key not in acc else acc[key] + v

        def s_a(acc, mat, n0):
            m1, m4, m5, m7 = [st(mat, n0, i) for i in (1, 4, 5, 7)]
            add(acc, (0, n0), (m1 + m4) + (m7 - m5))
            tick(acc[(0, n0)])
            add(acc, (1, n0 + 1), m1)
            add(acc, (1, n0), m4)
            add(acc, (0, n0 + 1), m5)

        def s_b(acc, mat, n0):
            m2, m3, m6 = [st(mat, n0, i) for i in (2, 3, 6)]
            add(acc, (1, n0), m2)
            add(acc, (0, n0 + 1), m3)
            add(acc, (1, n0 + 1), (m3 - m2) + m6)
            tick(acc[(1, n0 + 1)])

        def h_a(acc, mat, n0):
            r0, r9, r11, r10 = [hk(mat, n0, r) for r in (0, 9, 11, 10)]
            t = r9 + r11
            w0 = r0 + t
            add(acc, (0, n0), w0 + r10)
            tick(acc[(0, n0)])
            acc[(1, n0)] = acc[(1, n0)] - w0
            add(acc, (0, n0 + 2), t + r10)
            acc[(1, n0 + 2)] = acc[(1, n0 + 2)] - r11 if (1, n0 + 2) in acc else -r11

        def h_b(acc, mat, n0):
            r7, r6, r8, r1 = [hk(mat, n0, r) for r in (7, 6, 8, 1)]
            add(acc, (0, n0), r7)
            add(acc, (1, n0), (r1 + r6) + r8)
            tick(acc[(1, n0)])
            add(acc, (0, n0 + 1), r6 + r7)
            add(acc, (1, n0 + 1), r8)

        def h_c(acc, mat, n0):
            r3, r12, r14, r13 = [hk(mat, n0, r) for r in (3, 12, 14, 13)]
            t = r12 + r14
            w1 = r3 + t
            acc[(0, n0 + 1)] = acc[(0, n0 + 1)] - w1
            add(acc, (1, n0 + 1), w1 + r13)
            tick(acc[(1, n0 + 1)])
            acc[(0, n0 + 2)] = acc[(0, n0 + 2)] - r14
            add(acc, (1, n0 + 2), t + r13)

        def h_1(acc, mat, n0, r):
            add(acc, {2: (0, n0 + 1), 4: (0, n0 + 2), 5: (1, n0 + 2)}[r], hk(mat, n0, r))

        def group6(mat, n0, done, filler):
            acc = {}

            def fin(*keys):
                for key in keys:
                    done(key[0], key[1], acc.pop(key))
            s_a(acc, mat, n0)
            s_b(acc, mat, n0)
            h_1(acc, mat, n0, 2)
            h_a(acc, mat, n0)
            h_b(acc, mat, n0)
            fin((0, n0), (1, n0))
            h_c(acc, mat, n0)
            fin((0, n0 + 1), (1, n0 + 1))
            s_a(acc, mat, n0 + 2)
            s_b(acc, mat, n0 + 2)
            h_1(acc, mat, n0, 5)
            fin((1, n0 + 2))
            s_a(acc, mat, n0 + 4)
            s_b(acc, mat, n0 + 4)
            h_1(acc, mat, n0, 4)
            fin((0, n0 + 2))
            h_a(acc, mat, n0 + 3)
            h_b(acc, mat, n0 + 3)
            fin((0, n0 + 3), (1, n0 + 3))
            h_c(acc, mat, n0 + 3)
            fin((1, n0 + 4))
            for r in (2, 4, 5):
                h_1(acc, mat, n0 + 3, r)
            fin((0, n0 + 4), (0, n0 + 5), (1, n0 + 5))
            assert not acc
            filler()

        work = [P(ln_pair, nblk, k * LC, xn2_s, xs2_s) for k in range(HM1 // LC)]
        side.update(work=work, per=len(work) / LNSPAN)
        credit[0] = LOFF
        acc = {}
        plain = [(r, k) for k in (3, 4) for r in range(2)]

        def fill_q():
            r, k = plain.pop(0)
            add(acc, (r, 14), mm(0, xt(r, k), wtile(0, k, 14)))

        def done_q(r, n, val):
            store_qkv(n, r * HM1, val)

        def fin_q(*keys):
            for key in keys:
                done_q(key[0], key[1], acc.pop(key))
        fill_q()
        fill_q()
        group6(0, 0, done_q, fill_q)
        group6(0, 6, done_q, fill_q)
        s_a(acc, 0, 12)
        s_b(acc, 0, 12)
        h_1(acc, 0, 12, 2)
        h_a(acc, 0, 12)
        h_b(acc, 0, 12)
        fin_q((0, 12), (1, 12))
        h_c(acc, 0, 12)
        fin_q((0, 13), (1, 13))
        h_1(acc, 0, 12, 4)
        h_1(acc, 0, 12, 5)
        fin_q((0, 14), (1, 14))
        assert not work and not acc

        work = [P(attn_rows, c * RC, False) for c in range(TM1 // RC)]
        side.update(work=work, per=APER)
        credit[0] = AOFF

        def store_h(r, n, v):
            h_s[r * HP:(r + 1) * HP, n * 128:(n + 1) * 128] = _pack(v)

        h_1(acc, 3, 0, 4)
        h_1(acc, 3, 0, 5)
        s_a(acc, 3, 0)
        s_b(acc, 3, 0)
        h_1(acc, 3, 0, 2)
        h_a(acc, 3, 0)
        h_b(acc, 3, 0)
        for r in range(2):
            store_h(r, 13, tail_h(acc.pop((r, 0))))
        h_c(acc, 3, 0)
        for r in range(2):
            hold_s[(12 + r) * HM1:(13 + r) * HM1, :] = _gelu(acc.pop((r, 1)))
        plain = [(r, k) for r in range(2) for k in (3, 4)]

        def fill_g():
            r, k = plain.pop(0)
            l = xt(r, k)
            add(acc, (r, 2), mm(3, gate(l) if len(plain) == 3 else l, wtile(3, k, 2)))
            if k == 4:
                store_h(r, 12, hold_s[(12 + r) * HM1:(13 + r) * HM1, :] * acc.pop((r, 2)))
        for n0 in (0, 6):
            def slot(r, n):
                s = (n - n0) * 2 + r
                return slice(s * HM1, (s + 1) * HM1)

            def early(r, n):
                return (GPAT >> ((n - n0) * 2 + r)) & 1

            def done_g(r, n, v):
                hold_s[slot(r, n), :] = _gelu(v) if early(r, n) else v

            def done_u(r, n, v):
                g = hold_s[slot(r, n), :]
                store_h(r, n, (g if early(r, n) else _gelu(g)) * v)
            group6(1, n0, done_g, fill_g)
            group6(2, n0, done_u, fill_g)
        assert not plain and not acc
        note(hold_s, 0)

        def copy_xn(dst, src, r0, c, trig):
            dst[r0:r0 + HP, c:c + 128] = after(src[pl.ds(zrow(), r0 + HP), c:c + 128][r0:r0 + HP], trig)
            if c == 0:
                note(dst, r0)
        copies = [P(copy_xn, xn_s, xn2_s, r, c) for r in (0, HP) for c in range(0, D, 128)]
        copies += [P(copy_xn, xs_s, xs2_s, i * HP, 0) for i in range(NSUM)]
        mixed = _weave(work, copies)
        per = len(mixed) / (A2SPAN + 4.0)
        stage2(blk, base, TM1, [mixed] * 3, [2 * per, per, per])

    def cp(src, dst, s):
        return pltpu.make_async_copy(src, dst, sem_i.at[s])

    def gu(groups, s):
        return [cp(h.at[pl.ds(g * 128, 128)], d.at[pl.ds(g * 128, 128)], s)
                for g in groups for h, d in ((wg_hbm, wg_s), (wu_hbm, wu_s))]

    def wcol(t, s):
        return cp(wqkv_hbm.at[:, pl.ds(t * D, D)], wqkv_r.at[:, pl.ds(t * D, D)], s)

    def xblk(b, s):
        return cp(x_hbm.at[pl.ds(TM0 + b * TM1, TM1)], x_s.at[b + 1, pl.ds(0, TM1)], s)

    HM = TM0 // 2
    cp_x0 = [cp(x_hbm.at[pl.ds(i * HM, HM)], x_s.at[0, pl.ds(i * HM, HM)], i) for i in range(2)]
    cp_gu = [gu(g, 2 + k) for k, g in enumerate(G_EARLY)]
    cp_q = gu(G_Q, 5) + [cp(wg_hbm.at[pl.ds(FM, 64)], wt_s.at[pl.ds(0, 64)], 5),
                         cp(wu_hbm.at[pl.ds(FM, 64)], wt_s.at[pl.ds(64, 64)], 5), wcol(0, 5), xblk(0, 5)]
    cp_kv = gu(G_KV, 6) + [wcol(1, 6), wcol(2, 6)]
    cp_r = gu(G_R + G_D, 7) + [cp(wo_hbm, wo_r, 7)]
    cp_d = [cp(wd_hbm, wd_s.at[pl.ds(0, F)], 8)]
    cp_xs = [xblk(b, 9) for b in range(1, NL)]

    for c in cp_x0 + sum(cp_gu, []) + cp_q + cp_kv + cp_r + cp_d + cp_xs:
        c.start()
    zero_s[0] = 0
    k_s[:, 0:HALO, :] = jnp.zeros((NJ, HALO, 128), F32)
    v_s[:, 0:HALO, :] = jnp.zeros((NJ, HALO, 128), F32)
    wd_s[F:FP, :] = jnp.zeros((FP - F, D), BF)

    def first_block():
        def wait(cps, name):
            reset(CH0)
            with _scope(name):
                for c in cps:
                    c.wait()

        parts = []
        for i in range(2):
            wait(cp_x0[i:i + 1], 'waitx')
            parts += [ln_rows(0, i * HM + k * LC).astype(BF) for k in range(HM // LC)]
        xn = jnp.concatenate(parts, axis=0)

        def ffn_group(x, row0, g0, work, per, gated=False):
            g = _nt(x, wg_s[g0 * 128:(g0 + 1) * 128, :])
            fire(work, g, per)
            u = _nt(gate(x) if gated else x, wu_s[g0 * 128:(g0 + 1) * 128, :])
            fire(work, u, per)
            h_s[row0 // 2:(row0 + x.shape[0]) // 2, g0 * 128:(g0 + 1) * 128] = _pack(_gelu(g) * u)

        def ffn_groups(groups, work, per, gate_last=False):
            groups = list(groups)
            if len(groups) % 2:
                g0 = groups.pop(0)
                ffn_group(xn[0:HM], 0, g0, work, per)
                ffn_group(xn[HM:], HM, g0, work, per)
            for k, g0 in enumerate(groups):
                ffn_group(xn, 0, g0, work, per, gate_last and k == len(groups) - 1)

        have, done = set(), set()

        def new_preps(groups):
            have.update(groups)
            tris = [n for n in (0, 3, 6, 9) if {n, n + 1, n + 2} <= have and ('t', n) not in done]
            pairs = [n for n in range(0, 12, 2) if {n, n + 1} <= have and ('p', n) not in done]
            done.update([('t', n) for n in tris] + [('p', n) for n in pairs])
            return preps(1, tris, pairs) + preps(2, tris, pairs)

        perm = [[P(permute_qkv, t, r0) for r0 in range(0, D, 64)] for t in range(3)]

        for k, (cps, groups) in enumerate(zip(cp_gu, G_EARLY)):
            wait(cps, 'waitgu')
            work = new_preps(groups)
            nres = 2 * len(groups) + 2 * (len(groups) % 2)
            ffn_groups(groups, work, max(len(work), 1) / max(nres - 2.0, 1.0), k == 2)
            assert not work

        wait(cp_q, 'waitq')
        work = perm[0]
        for _ in range(3):
            work.pop(0)(None)
        t = _nt(xn, wt_s[...])
        fire(work, t, 4)
        h_s[0:TM0 // 2, FM:FP] = _pack(tail_h(t))
        work += new_preps(G_Q) + [P(ln_pair, 1, k * LC, xn_s, xs_s) for k in range(HM1 // LC)]
        for g0 in G_Q:
            ffn_group(xn, 0, g0, work, QPER)
        assert all(w.func is ln_pair for w in work)
        per = len(work) / QSPAN
        for j in range(NJ):
            r = _nn(xn, _unpack(wqkv_p[:, j * 128:(j + 1) * 128]))
            fire(work, r, per)
            store_qkv(j, 0, r)
        assert not work

        wait(cp_kv, 'waitkv')
        work = perm[1]
        for _ in range(4):
            work.pop(0)(None)
        for g0 in G_KV:
            g = _nt(xn, wg_s[g0 * 128:(g0 + 1) * 128, :])
            fire(work, g, 6)
            u = _nt(xn, wu_s[g0 * 128:(g0 + 1) * 128, :])
            h_s[0:TM0 // 2, g0 * 128:(g0 + 1) * 128] = _pack(_gelu(g) * u)
        assert not work
        work = perm[2] + _weave(new_preps(G_KV), _weave(preps(0, range(0, 15, 3), []),
                                                        preps(0, [], range(0, 14, 2))))
        per = len(work) / KVSPAN
        fire(work, u, per)
        for c in range(NJ, 3 * NJ):
            assert c < 2 * NJ or all(w.func is not permute_qkv for w in work)
            r = _nn(gate(xn) if c == 3 * NJ - 1 else xn, _unpack(wqkv_p[:, c * 128:(c + 1) * 128]))
            fire(work, r, per)
            store_qkv(c, 0, r)
        assert not work

        wait(cp_r, 'waitr')
        att = [P(attn_rows, rc * RC, True) for rc in range(TM0 // RC)]
        work = _weave(new_preps(G_R + G_D) + preps(3, [0], [0]), att[:NAR])
        att = att[NAR:]
        ffn_groups(G_R, work, len(work) / (2 * len(G_R) - 2.0))
        assert not work

        wait(cp_d, 'waitd')
        chain[0] = CHD
        wo_work = []
        for jj in range(NJ):
            wo_work += [P(widen_wo, jj, r0) for r0 in range(0, D, UW)]
            wo_work += [P(gather_wo, jj, j) for j in range(NJ)]
        pd = [P(prep_d, r0, c) for c in (0, 128) for r0 in range(0, FH, UD)]
        po = [P(prep_o, r0, c) for r0 in range(0, 128, UD // 2) for c in (0, 128)]
        wa = _weave(pd, wo_work, att[:NAA])
        wb = _weave(po, att[NAA:NAA + NAB])
        wc = att[NAA + NAB:]
        for _ in range(2):
            wa.pop(0)(None)
        per = len(wa) / SPANA
        ffn_groups(G_D, wa, per)
        stage2(0, 0, TM0, [wa, wb, wc], [per, len(wb) / SPANB, len(wc) / SPANC], False)

    def main(i, carry):
        with _scope('step0'):
            first_block()
        for c in cp_xs:
            c.wait()

        def body(b, c):
            with _scope('stepb'):
                step(b)
            return c
        return jax.lax.fori_loop(0, NL, body, carry)

    jax.lax.fori_loop(0, zero_s[0] + 1, main, 0)

    with _scope('waitout'):
        for j in range(NJ):
            for r in range(2):
                cp_o(0, 0, r * HM, HM, j).wait()
        for b in range(NL):
            for j in range(NJ):
                for r in range(2):
                    cp_o(b + 1, TM0 + b * TM1, r * HM1, HM1, j).wait()


@jax.jit
def pallas_parallel_sum__sliding_local_dilated__geglu_ffn__prompt_kernel(
    A_x: jax.Array,
    A_wqkv: jax.Array,
    A_wo: jax.Array,
    B_x: jax.Array,
    B_w_gate: jax.Array,
    B_w_up: jax.Array,
    B_w_down: jax.Array,
):
    x = A_x.reshape(S, D)
    hbm = pl.BlockSpec(memory_space=pltpu.MemorySpace.HBM)
    out = pl.pallas_call(
        _kernel,
        in_specs=[hbm] * 6,
        out_specs=hbm,
        out_shape=jax.ShapeDtypeStruct((S, D), BF),
        scratch_shapes=[
            pltpu.VMEM((NL + 1, TMP, D), BF),
            pltpu.VMEM((TM1 // 2, D), U32),
            pltpu.VMEM((NSUM * HP, 128), U32),
            pltpu.VMEM((TM1 // 2, D), U32),
            pltpu.VMEM((NSUM * HP, 128), U32),
            pltpu.VMEM((NL + 1, TMP, D), BF),
            pltpu.VMEM((D, 3 * D), BF),
            pltpu.VMEM((D // 2, 3 * D), U32),
            pltpu.VMEM((D, D), BF),
            pltpu.VMEM((NJ * D, 128), F32),
            pltpu.VMEM((D // 2, D), U32),
            pltpu.VMEM((FM, D), BF),
            pltpu.VMEM((FM, D), BF),
            pltpu.VMEM((128, D), BF),
            pltpu.VMEM((FP, D), BF),
            pltpu.VMEM((226 * 64, 128), U32),
            pltpu.VMEM((5 * FH // 2, 256), U32),
            pltpu.VMEM((5 * 128, 256), U32),
            pltpu.VMEM((NJ, TMX, 128), F32),
            pltpu.VMEM((NJ, TMX + HALO, 128), F32),
            pltpu.VMEM((NJ, TMX + HALO, 128), F32),
            pltpu.VMEM((TMX // 2, FP), U32),
            pltpu.VMEM((TMX // 2, D), U32),
            pltpu.VMEM((NHOLD * HM1, 128), F32),
            pltpu.SMEM((1,), jnp.int32),
            pltpu.SemaphoreType.DMA((10,)),
            pltpu.SemaphoreType.DMA((1,)),
        ],
        compiler_params=pltpu.CompilerParams(
            vmem_limit_bytes=100 * 1024 * 1024,
            disable_bounds_checks=True,
            disable_semaphore_checks=True,
        ),
    )(x, A_wqkv, A_wo, B_w_gate.T, B_w_up.T, B_w_down)
    return out.reshape(1, S, D)
```

```python
import functools

import jax
import jax.numpy as jnp
import jax.experimental.pallas as pl
import jax.experimental.pallas.tpu as pltpu

S, D, H, DH, W, DIL, F = 2048, 640, 32, 20, 8, 2, 1728
TM0 = 384
NL = 4
TM1 = (S - TM0) // NL
HM1 = TM1 // 2
HP = HM1 // 2
TMX = max(TM0, TM1)
TMP = (TMX + 63) // 64 * 64
HALO = 16
NJ = D // 128
LOG2E = 1.4426950408889634
FM = 1664
FP = 1792
FH = FP // 2
RC = 16
LC = 16
NHOLD = 14
G_EARLY = [[0], [1, 2], [3, 4, 5]]
G_Q, G_KV, G_R, G_D = [6], [7], [8, 9, 10, 11], [12]
LNSPAN = 24
APER = 0.377
GPAT = 0x999
A2SPAN = 7
AOFF = 4
NAR = 3
NAA = 8
NAB = 8
SPANA = 11
SPANB = 5
SPANC = 5
KVSPAN = 8
QPER = 1.5
QSPAN = 3.5
CH0 = 3
CHD = 2
UT = 16
UP = 32
UD = 16
UW = 64

BF = jnp.bfloat16
F32 = jnp.float32
U32 = jnp.uint32
NT = (((1,), (1,)), ((), ()))
P = functools.partial


def _gelu(g):
    c0 = 0.7978845608028654
    c1 = c0 * 0.044715
    t = jnp.tanh(g * (c0 + c1 * (g * g)))
    hg = 0.5 * g
    return hg + hg * t


def _pack(x):
    return pltpu.bitcast(x.astype(BF), U32)


def _unpack(u):
    return pltpu.bitcast(u, BF)


def _lhs_sums(a11, a12, a21, a22):
    return [a11 + a22, a21 + a22, a11 + a12, a21 - a11, a12 - a22]


def _rhs_sums(b11, b12, b21, b22):
    return [b11 + b22, b12 - b22, b21 - b11, b11 + b12, b21 + b22]


LS = {1: 0, 2: 1, 5: 2, 6: 3, 7: 4}
RS = {1: 0, 3: 1, 4: 2, 6: 3, 7: 4}

HK_R = {0: ((0, 0, 1), (0, 2, -1), (1, 0, 1)), 1: ((0, 0, 1), (0, 1, -1), (2, 0, 1)),
        2: ((1, 1, 1), (1, 0, -1), (2, 1, 1)), 3: ((0, 1, 1), (1, 1, 1), (1, 2, -1)),
        4: ((1, 2, 1), (2, 0, -1), (2, 2, 1)), 5: ((0, 2, 1), (2, 1, -1), (2, 2, 1)),
        6: ((0, 1, 1), (1, 0, 1)), 9: ((0, 2, 1), (2, 0, 1)), 12: ((1, 2, 1), (2, 1, 1))}
HK_RS = {r: i for i, r in enumerate(HK_R)}
HK_RP = {7: (1, 0), 8: (0, 1), 10: (2, 0), 11: (0, 2), 13: (2, 1), 14: (1, 2)}
HK_LP = {0: (0, 0), 3: (1, 1), 4: (0, 2), 5: (1, 2)}
HK_LS = {r: i for i, r in enumerate((1, 2, 6, 7, 8, 9, 10, 11, 12, 13, 14))}
NSUM = 16


def _hk_lhs_sums(x, y):
    s0, s1, s2 = x[0] + y[0], x[1] + y[1], x[2] + y[2]
    return [s0, s1, x[0] + y[1], x[1] - x[0], y[0] - y[1], s0 - y[2], s2 - s0, y[2] - y[0],
            s1 - x[2], s2 - s1, x[2] - x[1]]


def _nn(a, b):
    return jnp.dot(a, b, preferred_element_type=F32)


def _nt(a, b):
    return jax.lax.dot_general(a, b, NT, preferred_element_type=F32)


def _weave(*lists):
    items = []
    for lst in lists:
        items += [((k + 0.5) / len(lst), w) for k, w in enumerate(lst)]
    items.sort(key=lambda t: t[0])
    return [t[1] for t in items]


def _kernel(x_hbm, wqkv_hbm, wo_hbm, wg_hbm, wu_hbm, wd_hbm, out_hbm,
            x_s, xn_s, xs_s, xn2_s, xs2_s, out_s, wqkv_r, wqkv_p, wo_r, wo_f, wo_p,
            wg_s, wu_s, wt_s, wd_s, t1_s, td_s, to_s, q_s, k_s, v_s, h_s, a_s, hold_s,
            zero_s, sem_i, sem_o):

    def zrow():
        return pl.multiple_of(zero_s[0] * 8, 8)

    masks_ = {}

    def keep(shape):
        if shape not in masks_:
            masks_[shape] = jax.lax.broadcasted_iota(jnp.int32, shape, len(shape) - 1) >= zero_s[0]
        return masks_[shape]

    def after(val, trig):
        if trig is None:
            return val
        n = val.shape[0] // 8
        t = pltpu.bitcast(trig, val.dtype) if trig.dtype != val.dtype else trig
        if n > 1:
            t = jnp.concatenate([t] * n, axis=0)
        return jnp.where(keep(val.shape), val, t)

    def after_head(val, trig):
        if trig is None:
            return val
        if val.shape[1] == 128:
            return after(val, trig)
        return jnp.concatenate([after(val[:, 0:128], trig), val[:, 128:]], axis=1)

    toks = []
    credit = [0.0]
    chain = [0]
    prev = []

    anchor = [False]
    extra = []

    def reset(dist):
        anchor[0] = False
        masks_.clear()
        del extra[:]
        del toks[:]
        del prev[:]
        credit[0] = 0.0
        chain[0] = dist

    def note(ref, row):
        if all(r is not ref for r, _ in toks):
            toks.append((ref, row))

    def gate(lhs):
        if not toks and not extra:
            return lhs
        tok = functools.reduce(lambda p, q: p | q, extra + [
            pltpu.bitcast(ref[pl.ds(zrow() + row, 8), 0:128], U32) for ref, row in toks])
        del toks[:]
        del extra[:]
        u = pltpu.bitcast(lhs[0:16], U32)
        return jnp.concatenate([_unpack(after_head(u, tok)), lhs[16:]], axis=0)

    def fire(work, res, per):
        if not work:
            credit[0] = 0.0
            return
        pos = credit[0]
        while pos < 1.0 and work:
            r = int((res.shape[0] - 8) * pos) // 8 * 8
            trig = pltpu.bitcast(res[r:r + 8, :], U32)
            item = work.pop(0)
            if item.func in (attn_rows, ln_pair) and len(prev) >= chain[0]:
                trig = trig | prev[-chain[0]]
            tok = item(trig)
            if tok is not None:
                prev.append(pltpu.bitcast(tok, U32))
            pos += 1.0 / per
        credit[0] = max(pos - 1.0, 0.0)

    lane = jax.lax.broadcasted_iota(jnp.int32, (32, 128), 1)
    l5 = lane % 5
    masks = [l5 == r for r in range(5)]
    idx = [(DH * (lane % H) + 5 * (lane // H) + j) % 128 for j in range(NJ)]

    def permute_qkv(t, r0, trig):
        src = [pltpu.bitcast(wqkv_r[r0:r0 + 64, t * D + s * 128:t * D + (s + 1) * 128], U32)
               for s in range(NJ)]
        src[4] = after(src[4], trig)
        for j in range(NJ):
            mg = src[4]
            for s in range(3, -1, -1):
                mg = jnp.where(masks[(j - 3 * s) % 5], src[s], mg)
            res = jnp.take_along_axis(mg, idx[j], axis=1, mode="promise_in_bounds")
            wqkv_p[r0 // 2:r0 // 2 + 32, t * D + j * 128:t * D + (j + 1) * 128] = res

    def widen_wo(jj, r0, trig):
        w = after(pltpu.bitcast(wo_r[r0:r0 + UW, jj * 128:(jj + 1) * 128], U32), trig)
        wo_f[jj * D + r0:jj * D + r0 + UW, :] = _unpack(w).astype(F32)

    def gather_wo(jj, j, trig):
        for g in range(4):
            rows = wo_f[pl.ds(jj * D + 5 * g + j, H, stride=DH), :]
            rows = jnp.concatenate([after(rows[r:r + 8], trig) if r % 16 == 0 else rows[r:r + 8]
                                    for r in range(0, H, 8)], axis=0)
            r0 = (j * 128 + g * H) // 2
            wo_p[r0:r0 + H // 2, jj * 128:(jj + 1) * 128] = _pack(rows)

    def prep(b11, b12, b21, b22, store, trig):
        b11, b12, b21, b22 = [b.astype(F32) for b in (b11, b12, b21, b22)]
        b11 = after(b11, trig)
        b22 = after(b22, trig)
        for i, s in enumerate(_rhs_sums(b11, b12, b21, b22)):
            store(i, _pack(s))

    def wtile(mat, k, n, r0=0, nr=128):
        if mat == 3:
            return wtile(n, k, 12, r0, nr) if n else wt_s[r0:r0 + nr, k * 128:(k + 1) * 128]
        if mat == 0:
            return _unpack(wqkv_p[k * 64 + r0 // 2:k * 64 + (r0 + nr) // 2, n * 128:(n + 1) * 128])
        return (wg_s, wu_s)[mat - 1][n * 128 + r0:n * 128 + r0 + nr, k * 128:(k + 1) * 128]

    def t_tri(mat, n0, i):
        return ((0, 80, 146, 212)[mat] + n0 // 3 * 9 + i) * 64

    def t_pair(mat, n0, i):
        return ((45, 116, 182, 221)[mat] + n0 // 2 * 5 + i) * 64

    def prep_tri(mat, n0, r0, trig):
        b = [[wtile(mat, k, n0 + n, r0, UT).astype(F32) for n in range(3)] for k in range(3)]
        for k, n in ((1, 0), (0, 1), (0, 2), (1, 2)):
            b[k][n] = after(b[k][n], trig)
        for r, terms in HK_R.items():
            s = None
            for k, n, c in terms:
                s = b[k][n] if s is None else (s + b[k][n] if c > 0 else s - b[k][n])
            row = t_tri(mat, n0, HK_RS[r]) + r0 // 2
            t1_s[row:row + UT // 2, :] = _pack(s)
            note(t1_s, row)

    def prep_pair(mat, n0, r0, trig):
        def store(i, o):
            row = t_pair(mat, n0, i) + r0 // 2
            t1_s[row:row + UP // 2, :] = o
            note(t1_s, row)
        prep(wtile(mat, 3, n0, r0, UP), wtile(mat, 3, n0 + 1, r0, UP),
             wtile(mat, 4, n0, r0, UP), wtile(mat, 4, n0 + 1, r0, UP), store, trig)

    def preps(mat, tris, pairs):
        return ([P(prep_tri, mat, n0, r0) for n0 in tris for r0 in range(0, 128, UT)]
                + [P(prep_pair, mat, n0, r0) for n0 in pairs for r0 in range(0, 128, UP)])

    def prep_d(r0, c, trig):
        def store(i, o):
            row = i * (FH // 2) + r0 // 2
            td_s[row:row + UD // 2, c:c + 128] = o
        prep(wd_s[r0:r0 + UD, c:c + 128], wd_s[r0:r0 + UD, 256 + c:384 + c],
             wd_s[FH + r0:FH + r0 + UD, c:c + 128], wd_s[FH + r0:FH + r0 + UD, 256 + c:384 + c], store, trig)

    def prep_o(r0, c, trig):
        n = UD // 2

        def store(i, o):
            to_s[i * 128 + r0:i * 128 + r0 + n, c:c + 128] = o
        prep(_unpack(wo_p[r0:r0 + n, c:c + 128]), _unpack(wo_p[r0:r0 + n, 256 + c:384 + c]),
             _unpack(wo_p[128 + r0:128 + r0 + n, c:c + 128]), _unpack(wo_p[128 + r0:128 + r0 + n, 256 + c:384 + c]),
             store, trig)

    def ln_rows(blk, r0, trig=None):
        x = after_head(x_s[blk, r0:r0 + LC, :].astype(F32), trig)
        m = jnp.sum(x, axis=-1, keepdims=True) * (1.0 / D)
        mb = m.astype(BF).astype(F32)
        xc = x - mb
        dm = m - mb
        var = jnp.sum(xc * xc, axis=-1, keepdims=True) * (1.0 / D) - dm * dm
        return xc * jax.lax.rsqrt(jnp.maximum(var, 0.0) + 1e-5)

    def ln_pair(blk, r0, xn_d, xs_d, trig):
        top = ln_rows(blk, r0, trig)
        bot = ln_rows(blk, HM1 + r0, trig)
        xn_d[r0 // 2:(r0 + LC) // 2, :] = _pack(top)
        xn_d[(HM1 + r0) // 2:(HM1 + r0 + LC) // 2, :] = _pack(bot)
        x = [top[:, k * 128:(k + 1) * 128] for k in range(NJ)]
        y = [bot[:, k * 128:(k + 1) * 128] for k in range(NJ)]
        for i, s in enumerate(_hk_lhs_sums(x, y) + _lhs_sums(x[3], x[4], y[3], y[4])):
            xs_d[i * HP + r0 // 2:i * HP + (r0 + LC) // 2, :] = _pack(s)
        note(xn_d, r0 // 2)
        note(xs_d, r0 // 2)
        s0 = x[0] + y[0]
        return s0[0:8] + s0[8:16]

    def tail_h(t):
        ht = _gelu(t) * pltpu.roll(t, 64, 1)
        lo = jax.lax.broadcasted_iota(jnp.int32, ht.shape, 1) < 64
        return jnp.where(lo, ht, 0.0)

    def store_qkv(c, row0, val):
        t, j = divmod(c, NJ)
        n = val.shape[0]
        if t == 0:
            q_s[j, row0:row0 + n, :] = val * (DH ** -0.5 * LOG2E)
        elif t == 1:
            k_s[j, HALO + row0:HALO + row0 + n, :] = val
        else:
            v_s[j, HALO + row0:HALO + row0 + n, :] = val

    def attn_core(r0, first, trig):
        q = q_s[:, r0:r0 + 8, :]
        if trig is not None:
            q = jnp.where(keep((NJ, 8, 128)), q, pltpu.bitcast(trig, F32)[None])
        logits = []
        for w in range(W):
            st = HALO + r0 - DIL * w
            acc = jnp.sum(q * k_s[:, st:st + 8, :], axis=0)
            acc = acc + pltpu.roll(acc, 64, 1)
            acc = acc + pltpu.roll(acc, 32, 1)
            if first and r0 < DIL * w:
                rows = r0 + jax.lax.broadcasted_iota(jnp.int32, (8, 128), 0)
                acc = jnp.where(rows >= DIL * w, acc, -1e9 * LOG2E)
            logits.append(acc)
        mx = logits[0]
        for w in range(1, W):
            mx = jnp.maximum(mx, logits[w])
        ps = [jnp.exp2(l - mx) for l in logits]
        den = ps[0]
        for w in range(1, W):
            den = den + ps[w]
        r = pl.reciprocal(den, approx=True)
        inv = r * (2.0 - den * r)
        acc = ps[0][None] * v_s[:, HALO + r0:HALO + r0 + 8, :]
        for w in range(1, W):
            st = HALO + r0 - DIL * w
            acc = acc + ps[w][None] * v_s[:, st:st + 8, :]
        return acc * inv[None], mx

    def attn_rows(r0, first, trig):
        o1, t1 = attn_core(r0, first, trig)
        o2, t2 = attn_core(r0 + 8, first, t1)
        for j in range(NJ):
            a_s[r0 // 2:(r0 + RC) // 2, j * 128:(j + 1) * 128] = _pack(jnp.concatenate([o1[j], o2[j]], axis=0))
        if anchor[0]:
            extra.append(pltpu.bitcast(pltpu.roll(jnp.max(jnp.maximum(o1, o2), axis=0), 64, 1), U32))
        return t2

    def cp_o(blk, base, r0, n, j):
        return pltpu.make_async_copy(out_s.at[blk, pl.ds(r0, n), pl.ds(j * 128, 128)],
                                     out_hbm.at[pl.ds(base + r0, n), pl.ds(j * 128, 128)], sem_o.at[0])

    def emit(blk, base, *pieces):
        for r0, j, val in pieces:
            n = val.shape[0]
            x = x_s[blk, r0:r0 + n, j * 128:(j + 1) * 128].astype(F32)
            out_s[blk, r0:r0 + n, j * 128:(j + 1) * 128] = (x + val).astype(BF)
        for r0, j, val in pieces:
            cp_o(blk, base, r0, val.shape[0], j).start()

    def stage2(blk, base, tm, works, pers, gated=True):
        hm, hp = tm // 2, tm // 4
        anchor[0] = gated

        def half(ref, r, c0, c1):
            return _unpack(ref[r * hp:(r + 1) * hp, c0:c1])

        memo = {}

        def lhs(plain, kh, i):
            if i == 3:
                return half(plain, 0, 0, kh)
            if i == 4:
                return half(plain, 1, kh, 2 * kh)
            if (kh, i) not in memo:
                def b(r, c):
                    u = plain[pl.ds(zrow(), 2 * hp), c * kh:(c + 1) * kh]
                    return _unpack(u[r * hp:(r + 1) * hp]).astype(F32)
                s = {1: lambda: b(0, 0) + b(1, 1), 2: lambda: b(1, 0) + b(1, 1), 5: lambda: b(0, 0) + b(0, 1),
                     6: lambda: b(1, 0) - b(0, 0), 7: lambda: b(0, 1) - b(1, 1)}[i]()
                memo[(kh, i)] = s.astype(BF)
            return memo[(kh, i)]

        f4 = []
        for r in range(2):
            if works[0] is works[1]:
                f = _nn(half(h_s, r, 0, FP), wd_s[:, 512:D])
                fire(works[0], f, pers[0])
            else:
                f = None
                for k0 in range(0, FP, 512):
                    k1 = min(k0 + 512, FP)
                    part = _nn(half(h_s, r, k0, k1), wd_s[k0:k1, 512:D])
                    fire(works[0], part, pers[0])
                    f = part if f is None else f + part
            f4.append(f)
        ffn = []
        for c in range(2):
            assert works[c] is works[c + 1] or not works[c]
            if c == 0 or works[1] is not works[2]:
                credit[0] = 0.0
            cs = (c * 128, 256 + c * 128)

            def p(i):
                if i == 2:
                    wd = wd_s[0:FH, cs[0]:cs[0] + 128]
                elif i == 5:
                    wd = wd_s[FH:FP, cs[1]:cs[1] + 128]
                else:
                    wd = _unpack(td_s[RS[i] * (FH // 2):(RS[i] + 1) * (FH // 2), cs[0]:cs[0] + 128])
                m = _nn(lhs(h_s, FH, i), wd)
                fire(works[c + 1], m, pers[c + 1])
                return m
            m4 = p(4)
            m2 = p(2)
            m1 = p(1)
            t11 = m1 + m4
            t22 = m1 - m2
            m3 = p(3)
            m5 = p(5)
            ffn.append((t11 - m5 + p(7), m3 + m5, m4 + m2, t22 + m3 + p(6)))
        assert not works[2]
        if not gated:
            del toks[:]
        k_s[:, 0:HALO, :] = k_s[:, tm:tm + HALO, :]
        v_s[:, 0:HALO, :] = v_s[:, tm:tm + HALO, :]
        for r in range(2):
            emit(blk, base, (r * hm, 4, f4[r] + _nn(gate(half(a_s, r, 0, D)), _unpack(wo_p[:, 512:D]))))
        for c in range(2):
            cs = (c * 128, 256 + c * 128)

            def p(i):
                if i == 2:
                    wo = wo_p[0:128, cs[0]:cs[0] + 128]
                elif i == 5:
                    wo = wo_p[128:256, cs[1]:cs[1] + 128]
                else:
                    wo = to_s[RS[i] * 128:(RS[i] + 1) * 128, cs[0]:cs[0] + 128]
                return _nn(lhs(a_s, 256, i), _unpack(wo))

            def left(r, cc):
                return ffn[c][2 * r + cc] + _nn(half(a_s, r, 512, D), _unpack(wo_p[256:320, cs[cc]:cs[cc] + 128]))
            l21 = left(1, 0)
            m4 = p(4)
            m2 = p(2)
            c21 = l21 + m4 + m2
            m1 = p(1)
            t11 = m1 + m4
            t22 = m1 - m2
            m3 = p(3)
            m5 = p(5)
            c12 = m3 + m5 + left(0, 1)
            c11 = t11 - m5 + p(7) + left(0, 0)
            c22 = t22 + m3 + p(6) + left(1, 1)
            emit(blk, base, (hm, c, c21))
            emit(blk, base, (0, c + 2, c12))
            emit(blk, base, (0, c, c11), (hm, c + 2, c22))

    def step(b):
        blk = b + 1
        base = pl.multiple_of(TM0 + b * TM1, 16)
        nblk = jnp.minimum(blk + 1, NL)
        reset(1)
        side = {}

        def xt(r, k):
            return _unpack(xn_s[r * HP:(r + 1) * HP, k * 128:(k + 1) * 128])

        def xsum(i):
            return _unpack(xs_s[i * HP:(i + 1) * HP, :])

        def mm(mat, l, w):
            return (_nn if mat == 0 else _nt)(l, w)

        def tick(v):
            fire(side['work'], v, side['per'])

        def hk(mat, n0, r):
            l = xt(*HK_LP[r]) if r in HK_LP else xsum(HK_LS[r])
            if r in HK_RP:
                w = wtile(mat, HK_RP[r][0], n0 + HK_RP[r][1])
            else:
                row = t_tri(mat, n0, HK_RS[r])
                w = _unpack(t1_s[row:row + 64, :])
            return mm(mat, l, w)

        def st(mat, n0, i):
            l = xt(0, 3) if i == 3 else xt(1, 4) if i == 4 else xsum(11 + LS[i])
            if i == 2:
                w = wtile(mat, 3, n0)
            elif i == 5:
                w = wtile(mat, 4, n0 + 1)
            else:
                row = t_pair(mat, n0, RS[i])
                w = _unpack(t1_s[row:row + 64, :])
            return mm(mat, l, w)

        def add(acc, key, v):
            acc[key] = v if key not in acc else acc[key] + v

        def s_a(acc, mat, n0):
            m1, m4, m5, m7 = [st(mat, n0, i) for i in (1, 4, 5, 7)]
            add(acc, (0, n0), (m1 + m4) + (m7 - m5))
            tick(acc[(0, n0)])
            add(acc, (1, n0 + 1), m1)
            add(acc, (1, n0), m4)
            add(acc, (0, n0 + 1), m5)

        def s_b(acc, mat, n0):
            m2, m3, m6 = [st(mat, n0, i) for i in (2, 3, 6)]
            add(acc, (1, n0), m2)
            add(acc, (0, n0 + 1), m3)
            add(acc, (1, n0 + 1), (m3 - m2) + m6)
            tick(acc[(1, n0 + 1)])

        def h_a(acc, mat, n0):
            r0, r9, r11, r10 = [hk(mat, n0, r) for r in (0, 9, 11, 10)]
            t = r9 + r11
            w0 = r0 + t
            add(acc, (0, n0), w0 + r10)
            tick(acc[(0, n0)])
            acc[(1, n0)] = acc[(1, n0)] - w0
            add(acc, (0, n0 + 2), t + r10)
            acc[(1, n0 + 2)] = acc[(1, n0 + 2)] - r11 if (1, n0 + 2) in acc else -r11

        def h_b(acc, mat, n0):
            r7, r6, r8, r1 = [hk(mat, n0, r) for r in (7, 6, 8, 1)]
            add(acc, (0, n0), r7)
            add(acc, (1, n0), (r1 + r6) + r8)
            tick(acc[(1, n0)])
            add(acc, (0, n0 + 1), r6 + r7)
            add(acc, (1, n0 + 1), r8)

        def h_c(acc, mat, n0):
            r3, r12, r14, r13 = [hk(mat, n0, r) for r in (3, 12, 14, 13)]
            t = r12 + r14
            w1 = r3 + t
            acc[(0, n0 + 1)] = acc[(0, n0 + 1)] - w1
            add(acc, (1, n0 + 1), w1 + r13)
            tick(acc[(1, n0 + 1)])
            acc[(0, n0 + 2)] = acc[(0, n0 + 2)] - r14
            add(acc, (1, n0 + 2), t + r13)

        def h_1(acc, mat, n0, r):
            add(acc, {2: (0, n0 + 1), 4: (0, n0 + 2), 5: (1, n0 + 2)}[r], hk(mat, n0, r))

        def group6(mat, n0, done, filler):
            acc = {}

            def fin(*keys):
                for key in keys:
                    done(key[0], key[1], acc.pop(key))
            s_a(acc, mat, n0)
            s_b(acc, mat, n0)
            h_1(acc, mat, n0, 2)
            h_a(acc, mat, n0)
            h_b(acc, mat, n0)
            fin((0, n0), (1, n0))
            h_c(acc, mat, n0)
            fin((0, n0 + 1), (1, n0 + 1))
            s_a(acc, mat, n0 + 2)
            s_b(acc, mat, n0 + 2)
            h_1(acc, mat, n0, 5)
            fin((1, n0 + 2))
            s_a(acc, mat, n0 + 4)
            s_b(acc, mat, n0 + 4)
            h_1(acc, mat, n0, 4)
            fin((0, n0 + 2))
            h_a(acc, mat, n0 + 3)
            h_b(acc, mat, n0 + 3)
            fin((0, n0 + 3), (1, n0 + 3))
            h_c(acc, mat, n0 + 3)
            fin((1, n0 + 4))
            for r in (2, 4, 5):
                h_1(acc, mat, n0 + 3, r)
            fin((0, n0 + 4), (0, n0 + 5), (1, n0 + 5))
            assert not acc
            filler()

        work = [P(ln_pair, nblk, k * LC, xn2_s, xs2_s) for k in range(HM1 // LC)]
        side.update(work=work, per=len(work) / LNSPAN)
        acc = {}
        plain = [(r, k) for k in (3, 4) for r in range(2)]

        def fill_q():
            r, k = plain.pop(0)
            add(acc, (r, 14), mm(0, xt(r, k), wtile(0, k, 14)))

        def done_q(r, n, val):
            store_qkv(n, r * HM1, val)

        def fin_q(*keys):
            for key in keys:
                done_q(key[0], key[1], acc.pop(key))
        fill_q()
        fill_q()
        group6(0, 0, done_q, fill_q)
        group6(0, 6, done_q, fill_q)
        s_a(acc, 0, 12)
        s_b(acc, 0, 12)
        h_1(acc, 0, 12, 2)
        h_a(acc, 0, 12)
        h_b(acc, 0, 12)
        fin_q((0, 12), (1, 12))
        h_c(acc, 0, 12)
        fin_q((0, 13), (1, 13))
        h_1(acc, 0, 12, 4)
        h_1(acc, 0, 12, 5)
        fin_q((0, 14), (1, 14))
        assert not work and not acc

        work = [P(attn_rows, c * RC, False) for c in range(TM1 // RC)]
        side.update(work=work, per=APER)
        credit[0] = AOFF

        def store_h(r, n, v):
            h_s[r * HP:(r + 1) * HP, n * 128:(n + 1) * 128] = _pack(v)

        h_1(acc, 3, 0, 4)
        h_1(acc, 3, 0, 5)
        s_a(acc, 3, 0)
        s_b(acc, 3, 0)
        h_1(acc, 3, 0, 2)
        h_a(acc, 3, 0)
        h_b(acc, 3, 0)
        for r in range(2):
            store_h(r, 13, tail_h(acc.pop((r, 0))))
        h_c(acc, 3, 0)
        for r in range(2):
            hold_s[(12 + r) * HM1:(13 + r) * HM1, :] = _gelu(acc.pop((r, 1)))
        plain = [(r, k) for r in range(2) for k in (3, 4)]

        def fill_g():
            r, k = plain.pop(0)
            l = xt(r, k)
            add(acc, (r, 2), mm(3, gate(l) if len(plain) == 3 else l, wtile(3, k, 2)))
            if k == 4:
                store_h(r, 12, hold_s[(12 + r) * HM1:(13 + r) * HM1, :] * acc.pop((r, 2)))
        for n0 in (0, 6):
            def slot(r, n):
                s = (n - n0) * 2 + r
                return slice(s * HM1, (s + 1) * HM1)

            def early(r, n):
                return (GPAT >> ((n - n0) * 2 + r)) & 1

            def done_g(r, n, v):
                hold_s[slot(r, n), :] = _gelu(v) if early(r, n) else v

            def done_u(r, n, v):
                g = hold_s[slot(r, n), :]
                store_h(r, n, (g if early(r, n) else _gelu(g)) * v)
            group6(1, n0, done_g, fill_g)
            group6(2, n0, done_u, fill_g)
        assert not plain and not acc
        note(hold_s, 0)

        def copy_xn(dst, src, r0, c, trig):
            dst[r0:r0 + HP, c:c + 128] = after(src[pl.ds(zrow(), r0 + HP), c:c + 128][r0:r0 + HP], trig)
            if c == 0:
                note(dst, r0)
        copies = [P(copy_xn, xn_s, xn2_s, r, c) for r in (0, HP) for c in range(0, D, 128)]
        copies += [P(copy_xn, xs_s, xs2_s, i * HP, 0) for i in range(NSUM)]
        mixed = _weave(work, copies)
        per = len(mixed) / (A2SPAN + 4.0)
        stage2(blk, base, TM1, [mixed] * 3, [2 * per, per, per])

    def cp(src, dst, s):
        return pltpu.make_async_copy(src, dst, sem_i.at[s])

    def gu(groups, s):
        return [cp(h.at[pl.ds(g * 128, 128)], d.at[pl.ds(g * 128, 128)], s)
                for g in groups for h, d in ((wg_hbm, wg_s), (wu_hbm, wu_s))]

    def wcol(t, s):
        return cp(wqkv_hbm.at[:, pl.ds(t * D, D)], wqkv_r.at[:, pl.ds(t * D, D)], s)

    def xblk(b, s):
        return cp(x_hbm.at[pl.ds(TM0 + b * TM1, TM1)], x_s.at[b + 1, pl.ds(0, TM1)], s)

    HM = TM0 // 2
    cp_x0 = [cp(x_hbm.at[pl.ds(i * HM, HM)], x_s.at[0, pl.ds(i * HM, HM)], i) for i in range(2)]
    cp_gu = [gu(g, 2 + k) for k, g in enumerate(G_EARLY)]
    cp_q = gu(G_Q, 5) + [cp(wg_hbm.at[pl.ds(FM, 64)], wt_s.at[pl.ds(0, 64)], 5),
                         cp(wu_hbm.at[pl.ds(FM, 64)], wt_s.at[pl.ds(64, 64)], 5), wcol(0, 5), xblk(0, 5)]
    cp_kv = gu(G_KV, 6) + [wcol(1, 6), wcol(2, 6)]
    cp_r = gu(G_R + G_D, 7) + [cp(wo_hbm, wo_r, 7)]
    cp_d = [cp(wd_hbm, wd_s.at[pl.ds(0, F)], 8)]
    cp_xs = [xblk(b, 9) for b in range(1, NL)]

    for c in cp_x0 + sum(cp_gu, []) + cp_q + cp_kv + cp_r + cp_d + cp_xs:
        c.start()
    zero_s[0] = 0
    k_s[:, 0:HALO, :] = jnp.zeros((NJ, HALO, 128), F32)
    v_s[:, 0:HALO, :] = jnp.zeros((NJ, HALO, 128), F32)
    wd_s[F:FP, :] = jnp.zeros((FP - F, D), BF)

    def first_block():
        def wait(cps):
            reset(CH0)
            for c in cps:
                c.wait()

        parts = []
        for i in range(2):
            wait(cp_x0[i:i + 1])
            parts += [ln_rows(0, i * HM + k * LC).astype(BF) for k in range(HM // LC)]
        xn = jnp.concatenate(parts, axis=0)

        def ffn_group(x, row0, g0, work, per, gated=False):
            g = _nt(x, wg_s[g0 * 128:(g0 + 1) * 128, :])
            fire(work, g, per)
            u = _nt(gate(x) if gated else x, wu_s[g0 * 128:(g0 + 1) * 128, :])
            fire(work, u, per)
            h_s[row0 // 2:(row0 + x.shape[0]) // 2, g0 * 128:(g0 + 1) * 128] = _pack(_gelu(g) * u)

        def ffn_groups(groups, work, per, gate_last=False):
            groups = list(groups)
            if len(groups) % 2:
                g0 = groups.pop(0)
                ffn_group(xn[0:HM], 0, g0, work, per)
                ffn_group(xn[HM:], HM, g0, work, per)
            for k, g0 in enumerate(groups):
                ffn_group(xn, 0, g0, work, per, gate_last and k == len(groups) - 1)

        have, done = set(), set()

        def new_preps(groups):
            have.update(groups)
            tris = [n for n in (0, 3, 6, 9) if {n, n + 1, n + 2} <= have and ('t', n) not in done]
            pairs = [n for n in range(0, 12, 2) if {n, n + 1} <= have and ('p', n) not in done]
            done.update([('t', n) for n in tris] + [('p', n) for n in pairs])
            return preps(1, tris, pairs) + preps(2, tris, pairs)

        perm = [[P(permute_qkv, t, r0) for r0 in range(0, D, 64)] for t in range(3)]

        for k, (cps, groups) in enumerate(zip(cp_gu, G_EARLY)):
            wait(cps)
            work = new_preps(groups)
            nres = 2 * len(groups) + 2 * (len(groups) % 2)
            ffn_groups(groups, work, max(len(work), 1) / max(nres - 2.0, 1.0), k == 2)
            assert not work

        wait(cp_q)
        work = perm[0]
        for _ in range(3):
            work.pop(0)(None)
        t = _nt(xn, wt_s[...])
        fire(work, t, 4)
        h_s[0:TM0 // 2, FM:FP] = _pack(tail_h(t))
        work += new_preps(G_Q) + [P(ln_pair, 1, k * LC, xn_s, xs_s) for k in range(HM1 // LC)]
        for g0 in G_Q:
            ffn_group(xn, 0, g0, work, QPER)
        assert all(w.func is ln_pair for w in work)
        per = len(work) / QSPAN
        for j in range(NJ):
            r = _nn(xn, _unpack(wqkv_p[:, j * 128:(j + 1) * 128]))
            fire(work, r, per)
            store_qkv(j, 0, r)
        assert not work

        wait(cp_kv)
        work = perm[1]
        for _ in range(4):
            work.pop(0)(None)
        for g0 in G_KV:
            g = _nt(xn, wg_s[g0 * 128:(g0 + 1) * 128, :])
            fire(work, g, 6)
            u = _nt(xn, wu_s[g0 * 128:(g0 + 1) * 128, :])
            h_s[0:TM0 // 2, g0 * 128:(g0 + 1) * 128] = _pack(_gelu(g) * u)
        assert not work
        work = perm[2] + _weave(new_preps(G_KV), _weave(preps(0, range(0, 15, 3), []),
                                                        preps(0, [], range(0, 14, 2))))
        per = len(work) / KVSPAN
        fire(work, u, per)
        for c in range(NJ, 3 * NJ):
            assert c < 2 * NJ or all(w.func is not permute_qkv for w in work)
            r = _nn(gate(xn) if c == 3 * NJ - 1 else xn, _unpack(wqkv_p[:, c * 128:(c + 1) * 128]))
            fire(work, r, per)
            store_qkv(c, 0, r)
        assert not work

        wait(cp_r)
        att = [P(attn_rows, rc * RC, True) for rc in range(TM0 // RC)]
        work = _weave(new_preps(G_R + G_D) + preps(3, [0], [0]), att[:NAR])
        att = att[NAR:]
        ffn_groups(G_R, work, len(work) / (2 * len(G_R) - 2.0))
        assert not work

        wait(cp_d)
        chain[0] = CHD
        wo_work = []
        for jj in range(NJ):
            wo_work += [P(widen_wo, jj, r0) for r0 in range(0, D, UW)]
            wo_work += [P(gather_wo, jj, j) for j in range(NJ)]
        pd = [P(prep_d, r0, c) for c in (0, 128) for r0 in range(0, FH, UD)]
        po = [P(prep_o, r0, c) for r0 in range(0, 128, UD // 2) for c in (0, 128)]
        wa = _weave(pd, wo_work, att[:NAA])
        wb = _weave(po, att[NAA:NAA + NAB])
        wc = att[NAA + NAB:]
        for _ in range(2):
            wa.pop(0)(None)
        per = len(wa) / SPANA
        ffn_groups(G_D, wa, per)
        stage2(0, 0, TM0, [wa, wb, wc], [per, len(wb) / SPANB, len(wc) / SPANC], False)

    def main(i, carry):
        first_block()
        for c in cp_xs:
            c.wait()

        def body(b, c):
            step(b)
            return c
        return jax.lax.fori_loop(0, NL, body, carry)

    jax.lax.fori_loop(0, zero_s[0] + 1, main, 0)

    for j in range(NJ):
        for r in range(2):
            cp_o(0, 0, r * HM, HM, j).wait()
    for b in range(NL):
        for j in range(NJ):
            for r in range(2):
                cp_o(b + 1, TM0 + b * TM1, r * HM1, HM1, j).wait()


@jax.jit
def pallas_parallel_sum__sliding_local_dilated__geglu_ffn__prompt_kernel(
    A_x: jax.Array,
    A_wqkv: jax.Array,
    A_wo: jax.Array,
    B_x: jax.Array,
    B_w_gate: jax.Array,
    B_w_up: jax.Array,
    B_w_down: jax.Array,
):
    x = A_x.reshape(S, D)
    hbm = pl.BlockSpec(memory_space=pltpu.MemorySpace.HBM)
    out = pl.pallas_call(
        _kernel,
        in_specs=[hbm] * 6,
        out_specs=hbm,
        out_shape=jax.ShapeDtypeStruct((S, D), BF),
        scratch_shapes=[
            pltpu.VMEM((NL + 1, TMP, D), BF),
            pltpu.VMEM((TM1 // 2, D), U32),
            pltpu.VMEM((NSUM * HP, 128), U32),
            pltpu.VMEM((TM1 // 2, D), U32),
            pltpu.VMEM((NSUM * HP, 128), U32),
            pltpu.VMEM((NL + 1, TMP, D), BF),
            pltpu.VMEM((D, 3 * D), BF),
            pltpu.VMEM((D // 2, 3 * D), U32),
            pltpu.VMEM((D, D), BF),
            pltpu.VMEM((NJ * D, 128), F32),
            pltpu.VMEM((D // 2, D), U32),
            pltpu.VMEM((FM, D), BF),
            pltpu.VMEM((FM, D), BF),
            pltpu.VMEM((128, D), BF),
            pltpu.VMEM((FP, D), BF),
            pltpu.VMEM((226 * 64, 128), U32),
            pltpu.VMEM((5 * FH // 2, 256), U32),
            pltpu.VMEM((5 * 128, 256), U32),
            pltpu.VMEM((NJ, TMX, 128), F32),
            pltpu.VMEM((NJ, TMX + HALO, 128), F32),
            pltpu.VMEM((NJ, TMX + HALO, 128), F32),
            pltpu.VMEM((TMX // 2, FP), U32),
            pltpu.VMEM((TMX // 2, D), U32),
            pltpu.VMEM((NHOLD * HM1, 128), F32),
            pltpu.SMEM((1,), jnp.int32),
            pltpu.SemaphoreType.DMA((10,)),
            pltpu.SemaphoreType.DMA((1,)),
        ],
        compiler_params=pltpu.CompilerParams(
            vmem_limit_bytes=100 * 1024 * 1024,
            disable_bounds_checks=True,
            disable_semaphore_checks=True,
        ),
    )(x, A_wqkv, A_wo, B_w_gate.T, B_w_up.T, B_w_down)
    return out.reshape(1, S, D)
```

```python
import functools

import jax
import jax.numpy as jnp
import jax.experimental.pallas as pl
import jax.experimental.pallas.tpu as pltpu

S, D, H, DH, W, DIL, F = 2048, 640, 32, 20, 8, 2, 1728
TM0 = 384
NL = 4
TM1 = (S - TM0) // NL
HM1 = TM1 // 2
HP = HM1 // 2
TMX = max(TM0, TM1)
TMP = (TMX + 63) // 64 * 64
HALO = 16
NJ = D // 128
LOG2E = 1.4426950408889634
FM = 1664
FP = 1792
RC = 16
LC = 16
NHOLD = 14
G_EARLY = [[0], [1, 2], [3, 4, 5]]
G_Q, G_KV, G_R, G_D = [6], [7], [8, 9, 10, 11], [12]
LNSPAN = 24.7
APER = 0.344
GPAT = 0x999
A2SPAN = 12
AOFF = 2.9
NAR = 1
NAA = 10
NAB = 9
SPANA = 15.5
SPANB = 12.9
SPANC = 10
KVSPAN = 8
QPER = 1.5
QSPAN = 3.5
CH0 = 3
NPDB = 24
NPDD = 24
NPDA = 20
NA0 = 2
SPAN0 = 6.5
CHD = 2
UT = 16
UP = 32
UD = 16
UW = 64

BF = jnp.bfloat16
F32 = jnp.float32
U32 = jnp.uint32
NT = (((1,), (1,)), ((), ()))
P = functools.partial


def _gelu(g):
    c0 = 0.7978845608028654
    c1 = c0 * 0.044715
    t = jnp.tanh(g * (c0 + c1 * (g * g)))
    hg = 0.5 * g
    return hg + hg * t


def _pack(x):
    return pltpu.bitcast(x.astype(BF), U32)


def _unpack(u):
    return pltpu.bitcast(u, BF)


def _lhs_sums(a11, a12, a21, a22):
    return [a11 + a22, a21 + a22, a11 + a12, a21 - a11, a12 - a22]


def _rhs_sums(b11, b12, b21, b22):
    return [b11 + b22, b12 - b22, b21 - b11, b11 + b12, b21 + b22]


LS = {1: 0, 2: 1, 5: 2, 6: 3, 7: 4}
RS = {1: 0, 3: 1, 4: 2, 6: 3, 7: 4}

HK_R = {0: ((0, 0, 1), (0, 2, -1), (1, 0, 1)), 1: ((0, 0, 1), (0, 1, -1), (2, 0, 1)),
        2: ((1, 1, 1), (1, 0, -1), (2, 1, 1)), 3: ((0, 1, 1), (1, 1, 1), (1, 2, -1)),
        4: ((1, 2, 1), (2, 0, -1), (2, 2, 1)), 5: ((0, 2, 1), (2, 1, -1), (2, 2, 1)),
        6: ((0, 1, 1), (1, 0, 1)), 9: ((0, 2, 1), (2, 0, 1)), 12: ((1, 2, 1), (2, 1, 1))}
HK_RS = {r: i for i, r in enumerate(HK_R)}
HK_RP = {7: (1, 0), 8: (0, 1), 10: (2, 0), 11: (0, 2), 13: (2, 1), 14: (1, 2)}
HK_LP = {0: (0, 0), 3: (1, 1), 4: (0, 2), 5: (1, 2)}
HK_LS = {r: i for i, r in enumerate((1, 2, 6, 7, 8, 9, 10, 11, 12, 13, 14))}
NSUM = 16
HK_O = {0: ((0, 0, 1), (1, 0, -1)), 1: ((1, 0, 1),), 2: ((0, 1, 1),), 3: ((0, 1, -1), (1, 1, 1)),
        4: ((0, 2, 1),), 5: ((1, 2, 1),), 6: ((1, 0, 1), (0, 1, 1)), 7: ((0, 0, 1), (0, 1, 1)),
        8: ((1, 0, 1), (1, 1, 1)), 9: ((0, 0, 1), (1, 0, -1), (0, 2, 1)), 10: ((0, 0, 1), (0, 2, 1)),
        11: ((0, 0, 1), (1, 0, -1), (0, 2, 1), (1, 2, -1)), 12: ((0, 1, -1), (1, 1, 1), (1, 2, 1)),
        13: ((1, 1, 1), (1, 2, 1)), 14: ((0, 1, -1), (1, 1, 1), (0, 2, -1), (1, 2, 1))}
KB = ((0, 1, 6, 7), (2, 3, 8, 9), (4, 5, 10, 11))
EB = ((4, 10, 12), (5, 11, 13))
LB = ((12,), (13,))
SUB_RS = {r: i for i, r in enumerate((0, 1, 2, 3, 6))}


def _hk_lhs_sums(x, y):
    s0, s1, s2 = x[0] + y[0], x[1] + y[1], x[2] + y[2]
    return [s0, s1, x[0] + y[1], x[1] - x[0], y[0] - y[1], s0 - y[2], s2 - s0, y[2] - y[0],
            s1 - x[2], s2 - s1, x[2] - x[1]]


def _nn(a, b):
    return jnp.dot(a, b, preferred_element_type=F32)


def _nt(a, b):
    return jax.lax.dot_general(a, b, NT, preferred_element_type=F32)


def _weave(*lists):
    items = []
    for lst in lists:
        items += [((k + 0.5) / len(lst), w) for k, w in enumerate(lst)]
    items.sort(key=lambda t: t[0])
    return [t[1] for t in items]


def _kernel(x_hbm, wqkv_hbm, wo_hbm, wg_hbm, wu_hbm, wd_hbm, out_hbm,
            x_s, xn_s, xs_s, xn2_s, xs2_s, out_s, wqkv_r, wqkv_p, wo_r, wo_f, wo_p,
            wg_s, wu_s, wt_s, wd_s, t1_s, td_s, to_s, q_s, k_s, v_s, h_s, hs_s, a_s, hold_s,
            zero_s, sem_i, sem_o):

    def zrow():
        return pl.multiple_of(zero_s[0] * 8, 8)

    masks_ = {}

    def keep(shape):
        if shape not in masks_:
            masks_[shape] = jax.lax.broadcasted_iota(jnp.int32, shape, len(shape) - 1) >= zero_s[0]
        return masks_[shape]

    def after(val, trig):
        if trig is None:
            return val
        n = val.shape[0] // 8
        t = pltpu.bitcast(trig, val.dtype) if trig.dtype != val.dtype else trig
        if n > 1:
            t = jnp.concatenate([t] * n, axis=0)
        return jnp.where(keep(val.shape), val, t)

    def after_head(val, trig):
        if trig is None:
            return val
        if val.shape[1] == 128:
            return after(val, trig)
        return jnp.concatenate([after(val[:, 0:128], trig), val[:, 128:]], axis=1)

    toks = []
    credit = [0.0]
    chain = [0]
    prev = []

    anchor = [False]
    extra = []

    def reset(dist):
        anchor[0] = False
        masks_.clear()
        del extra[:]
        del toks[:]
        del prev[:]
        credit[0] = 0.0
        chain[0] = dist

    def note(ref, row):
        if all(r is not ref for r, _ in toks):
            toks.append((ref, row))

    def gate(lhs):
        if not toks and not extra:
            return lhs
        tok = functools.reduce(lambda p, q: p | q, extra + [
            pltpu.bitcast(ref[pl.ds(zrow() + row, 8), 0:128], U32) for ref, row in toks])
        del toks[:]
        del extra[:]
        u = pltpu.bitcast(lhs[0:16], U32)
        return jnp.concatenate([_unpack(after_head(u, tok)), lhs[16:]], axis=0)

    def fire(work, res, per):
        if not work:
            credit[0] = 0.0
            return
        pos = credit[0]
        while pos < 1.0 and work:
            r = int((res.shape[0] - 8) * pos) // 8 * 8
            trig = pltpu.bitcast(res[r:r + 8, :], U32)
            item = work.pop(0)
            if item.func in (attn_rows, ln_pair) and len(prev) >= chain[0]:
                trig = trig | prev[-chain[0]]
            tok = item(trig)
            if tok is not None:
                prev.append(pltpu.bitcast(tok, U32))
            pos += 1.0 / per
        credit[0] = max(pos - 1.0, 0.0)

    lane = jax.lax.broadcasted_iota(jnp.int32, (32, 128), 1)
    l5 = lane % 5
    masks = [l5 == r for r in range(5)]
    idx = [(DH * (lane % H) + 5 * (lane // H) + j) % 128 for j in range(NJ)]

    def permute_qkv(t, r0, trig):
        src = [pltpu.bitcast(wqkv_r[r0:r0 + 64, t * D + s * 128:t * D + (s + 1) * 128], U32)
               for s in range(NJ)]
        src[4] = after(src[4], trig)
        for j in range(NJ):
            mg = src[4]
            for s in range(3, -1, -1):
                mg = jnp.where(masks[(j - 3 * s) % 5], src[s], mg)
            res = jnp.take_along_axis(mg, idx[j], axis=1, mode="promise_in_bounds")
            wqkv_p[r0 // 2:r0 // 2 + 32, t * D + j * 128:t * D + (j + 1) * 128] = res

    def widen_wo(jj, r0, trig):
        w = after(pltpu.bitcast(wo_r[r0:r0 + UW, jj * 128:(jj + 1) * 128], U32), trig)
        wo_f[jj * D + r0:jj * D + r0 + UW, :] = _unpack(w).astype(F32)

    def gather_wo(jj, j, trig):
        for g in range(4):
            rows = wo_f[pl.ds(jj * D + 5 * g + j, H, stride=DH), :]
            rows = jnp.concatenate([after(rows[r:r + 8], trig) if r % 16 == 0 else rows[r:r + 8]
                                    for r in range(0, H, 8)], axis=0)
            r0 = (j * 128 + g * H) // 2
            wo_p[r0:r0 + H // 2, jj * 128:(jj + 1) * 128] = _pack(rows)

    def prep(b11, b12, b21, b22, store, trig):
        b11, b12, b21, b22 = [b.astype(F32) for b in (b11, b12, b21, b22)]
        b11 = after(b11, trig)
        b22 = after(b22, trig)
        for i, s in enumerate(_rhs_sums(b11, b12, b21, b22)):
            store(i, _pack(s))

    def wtile(mat, k, n, r0=0, nr=128):
        if mat == 3:
            return wtile(n, k, 12, r0, nr) if n else wt_s[r0:r0 + nr, k * 128:(k + 1) * 128]
        if mat == 0:
            return _unpack(wqkv_p[k * 64 + r0 // 2:k * 64 + (r0 + nr) // 2, n * 128:(n + 1) * 128])
        return (wg_s, wu_s)[mat - 1][n * 128 + r0:n * 128 + r0 + nr, k * 128:(k + 1) * 128]

    def t_tri(mat, n0, i):
        return ((0, 80, 146, 212)[mat] + n0 // 3 * 9 + i) * 64

    def t_pair(mat, n0, i):
        return ((45, 116, 182, 221)[mat] + n0 // 2 * 5 + i) * 64

    def prep_tri(mat, n0, r0, trig):
        b = [[wtile(mat, k, n0 + n, r0, UT).astype(F32) for n in range(3)] for k in range(3)]
        for k, n in ((1, 0), (0, 1), (0, 2), (1, 2)):
            b[k][n] = after(b[k][n], trig)
        for r, terms in HK_R.items():
            s = None
            for k, n, c in terms:
                s = b[k][n] if s is None else (s + b[k][n] if c > 0 else s - b[k][n])
            row = t_tri(mat, n0, HK_RS[r]) + r0 // 2
            t1_s[row:row + UT // 2, :] = _pack(s)
            note(t1_s, row)

    def prep_pair(mat, n0, r0, trig):
        def store(i, o):
            row = t_pair(mat, n0, i) + r0 // 2
            t1_s[row:row + UP // 2, :] = o
            note(t1_s, row)
        prep(wtile(mat, 3, n0, r0, UP), wtile(mat, 3, n0 + 1, r0, UP),
             wtile(mat, 4, n0, r0, UP), wtile(mat, 4, n0 + 1, r0, UP), store, trig)

    def preps(mat, tris, pairs):
        return ([P(prep_tri, mat, n0, r0) for n0 in tris for r0 in range(0, 128, UT)]
                + [P(prep_pair, mat, n0, r0) for n0 in pairs for r0 in range(0, 128, UP)])

    def td_row(part, i, o):
        return ((0, 36, 56, 71)[part] + i * (4, 4, 3, 1)[part] + o) * 64

    def prep_d(part, o, r0, trig):
        kt = [blk[o] for blk in (KB, KB[:2], EB, LB)[part]]
        n0 = (0, 3, 3, 0)[part]
        b = [[wd_s[k * 128 + r0:k * 128 + r0 + UD, (n0 + n) * 128:(n0 + n + 1) * 128].astype(F32)
              for n in range(len(kt))] for k in kt]
        for k, n in ((1, 0), (0, 1), (0, 2), (1, 2))[:2 * len(kt) - 2]:
            b[k][n] = after(b[k][n], trig)
        for r, i in (HK_RS if part == 0 else SUB_RS).items():
            s = None
            for k, n, c in HK_R[r]:
                if k < len(kt) and n < len(kt):
                    s = b[k][n] if s is None else (s + b[k][n] if c > 0 else s - b[k][n])
            row = td_row(part, i, o) + r0 // 2
            td_s[row:row + UD // 2, :] = _pack(s)

    def sum_h(hp, part, o, r0, trig):
        kt = [blk[o] for blk in (KB, EB)[part]]
        x, y = [[_unpack(after(h_s[r * hp + r0:r * hp + r0 + 8, k * 128:(k + 1) * 128], trig)).astype(F32)
                 for k in kt] for r in range(2)]
        sums = _hk_lhs_sums(x, y) if part == 0 else _hk_lhs_sums(x + x[:1], y + y[:1])[:5]
        for i, s in enumerate(sums):
            row = (i + 11 * part) * hp + r0
            hs_s[row:row + 8, o * 128:(o + 1) * 128] = _pack(s)

    def sum_items(hp, g):
        return [P(sum_h, hp, part, o, r0) for r0 in range(0, hp, 8)
                for part, o in (((0, 0), (0, 1), (1, 0)), ((0, 2), (0, 3), (1, 1), (1, 2)))[g]]

    def prep_o(r0, c, trig):
        n = UD // 2

        def store(i, o):
            to_s[i * 128 + r0:i * 128 + r0 + n, c:c + 128] = o
        prep(_unpack(wo_p[r0:r0 + n, c:c + 128]), _unpack(wo_p[r0:r0 + n, 256 + c:384 + c]),
             _unpack(wo_p[128 + r0:128 + r0 + n, c:c + 128]), _unpack(wo_p[128 + r0:128 + r0 + n, 256 + c:384 + c]),
             store, trig)

    def ln_rows(blk, r0, trig=None):
        x = after_head(x_s[blk, r0:r0 + LC, :].astype(F32), trig)
        m = jnp.sum(x, axis=-1, keepdims=True) * (1.0 / D)
        mb = m.astype(BF).astype(F32)
        xc = x - mb
        dm = m - mb
        var = jnp.sum(xc * xc, axis=-1, keepdims=True) * (1.0 / D) - dm * dm
        return xc * jax.lax.rsqrt(jnp.maximum(var, 0.0) + 1e-5)

    def ln_pair(blk, r0, xn_d, xs_d, trig):
        top = ln_rows(blk, r0, trig)
        bot = ln_rows(blk, HM1 + r0, trig)
        xn_d[r0 // 2:(r0 + LC) // 2, :] = _pack(top)
        xn_d[(HM1 + r0) // 2:(HM1 + r0 + LC) // 2, :] = _pack(bot)
        x = [top[:, k * 128:(k + 1) * 128] for k in range(NJ)]
        y = [bot[:, k * 128:(k + 1) * 128] for k in range(NJ)]
        for i, s in enumerate(_hk_lhs_sums(x, y) + _lhs_sums(x[3], x[4], y[3], y[4])):
            xs_d[i * HP + r0 // 2:i * HP + (r0 + LC) // 2, :] = _pack(s)
        note(xn_d, r0 // 2)
        note(xs_d, r0 // 2)
        s0 = x[0] + y[0]
        return s0[0:8] + s0[8:16]

    def tail_h(t):
        ht = _gelu(t) * pltpu.roll(t, 64, 1)
        lo = jax.lax.broadcasted_iota(jnp.int32, ht.shape, 1) < 64
        return jnp.where(lo, ht, 0.0)

    def store_qkv(c, row0, val):
        t, j = divmod(c, NJ)
        n = val.shape[0]
        if t == 0:
            q_s[j, row0:row0 + n, :] = val * (DH ** -0.5 * LOG2E)
        elif t == 1:
            k_s[j, HALO + row0:HALO + row0 + n, :] = val
        else:
            v_s[j, HALO + row0:HALO + row0 + n, :] = val

    def attn_core(r0, first, trig):
        q = q_s[:, r0:r0 + 8, :]
        if trig is not None:
            q = jnp.where(keep((NJ, 8, 128)), q, pltpu.bitcast(trig, F32)[None])
        logits = []
        for w in range(W):
            st = HALO + r0 - DIL * w
            acc = jnp.sum(q * k_s[:, st:st + 8, :], axis=0)
            acc = acc + pltpu.roll(acc, 64, 1)
            acc = acc + pltpu.roll(acc, 32, 1)
            if first and r0 < DIL * w:
                rows = r0 + jax.lax.broadcasted_iota(jnp.int32, (8, 128), 0)
                acc = jnp.where(rows >= DIL * w, acc, -1e9 * LOG2E)
            logits.append(acc)
        mx = logits[0]
        for w in range(1, W):
            mx = jnp.maximum(mx, logits[w])
        ps = [jnp.exp2(l - mx) for l in logits]
        den = ps[0]
        for w in range(1, W):
            den = den + ps[w]
        r = pl.reciprocal(den, approx=True)
        inv = r * (2.0 - den * r)
        acc = ps[0][None] * v_s[:, HALO + r0:HALO + r0 + 8, :]
        for w in range(1, W):
            st = HALO + r0 - DIL * w
            acc = acc + ps[w][None] * v_s[:, st:st + 8, :]
        return acc * inv[None], mx

    def attn_rows(r0, first, trig):
        o1, t1 = attn_core(r0, first, trig)
        o2, t2 = attn_core(r0 + 8, first, t1)
        for j in range(NJ):
            a_s[r0 // 2:(r0 + RC) // 2, j * 128:(j + 1) * 128] = _pack(jnp.concatenate([o1[j], o2[j]], axis=0))
        if anchor[0]:
            extra.append(pltpu.bitcast(pltpu.roll(jnp.max(jnp.maximum(o1, o2), axis=0), 64, 1), U32))
        return t2

    def cp_o(blk, base, r0, n, j):
        return pltpu.make_async_copy(out_s.at[blk, pl.ds(r0, n), pl.ds(j * 128, 128)],
                                     out_hbm.at[pl.ds(base + r0, n), pl.ds(j * 128, 128)], sem_o.at[0])

    def emit(blk, base, *pieces):
        for r0, j, val in pieces:
            n = val.shape[0]
            x = x_s[blk, r0:r0 + n, j * 128:(j + 1) * 128].astype(F32)
            out_s[blk, r0:r0 + n, j * 128:(j + 1) * 128] = (x + val).astype(BF)
        for r0, j, val in pieces:
            cp_o(blk, base, r0, val.shape[0], j).start()

    def stage2(blk, base, tm, works, pers, gated=True, late=None, last=None):
        hm, hp = tm // 2, tm // 4
        anchor[0] = gated

        def half(ref, r, c0, c1):
            return _unpack(ref[r * hp:(r + 1) * hp, c0:c1])

        memo = {}

        def lhs(plain, kh, i):
            if i == 3:
                return half(plain, 0, 0, kh)
            if i == 4:
                return half(plain, 1, kh, 2 * kh)
            if (kh, i) not in memo:
                def b(r, c):
                    u = plain[pl.ds(zrow(), 2 * hp), c * kh:(c + 1) * kh]
                    return _unpack(u[r * hp:(r + 1) * hp]).astype(F32)
                s = {1: lambda: b(0, 0) + b(1, 1), 2: lambda: b(1, 0) + b(1, 1), 5: lambda: b(0, 0) + b(0, 1),
                     6: lambda: b(1, 0) - b(0, 0), 7: lambda: b(0, 1) - b(1, 1)}[i]()
                memo[(kh, i)] = s.astype(BF)
            return memo[(kh, i)]

        acc = {}

        def htiles(r, tiles):
            return jnp.concatenate([half(h_s, r, k * 128, (k + 1) * 128) for k in tiles], axis=1)

        def prod(part, r, phase):
            blocks = (KB, KB, EB, LB)[part]
            n0, nk = (0, 3, 3, 0)[part], len(blocks[0])
            if r in HK_LP:
                l = htiles(HK_LP[r][0], blocks[HK_LP[r][1]])
            else:
                row = (HK_LS[r] + (11 if part >= 2 else 0)) * hp
                c0 = 256 if part == 3 else 0
                l = _unpack(hs_s[row:row + hp, c0:c0 + nk * 128])
            if r in HK_RP:
                k, n = HK_RP[r]
                w = jnp.concatenate([wd_s[t * 128:(t + 1) * 128, (n0 + n) * 128:(n0 + n + 1) * 128]
                                     for t in blocks[k]], axis=0)
            else:
                row = td_row(part, (HK_RS if part == 0 else SUB_RS)[r], 0)
                w = _unpack(td_s[row:row + nk * 64, :])
            m = _nn(l, w)
            if part < 3:
                fire(works[phase], m, pers[phase])
            for rr, n, c in HK_O[r]:
                key = (rr, n0 + n)
                if key not in acc:
                    acc[key] = m if c > 0 else -m
                else:
                    acc[key] = acc[key] + m if c > 0 else acc[key] - m

        def direct(r, n, tiles, phase, split=False):
            w = jnp.concatenate([wd_s[t * 128:(t + 1) * 128, n * 128:(n + 1) * 128] for t in tiles], axis=0)
            l = htiles(r, tiles)
            if split:
                m = jnp.concatenate([_nn(l[0:hm // 2], w), _nn(l[hm // 2:], w)], axis=0)
            else:
                m = _nn(l, w)
            if phase < 3:
                fire(works[phase], m, pers[phase])
            acc[(r, n)] = m if (r, n) not in acc else acc[(r, n)] + m

        def next_phase(k):
            assert works[k] is works[k + 1] or not works[k]
            if works[k] is not works[k + 1]:
                credit[0] = 0.0

        if not gated:
            jobs = [(r, n, blk) for n in range(NJ) for r in range(2) for blk in KB]
            jobs += [(r, n, (12, 13)) for n in range(NJ) for r in range(2)]
            for i, job in enumerate(jobs):
                if i in (13, 26):
                    next_phase(i // 13 - 1)
                direct(*job, min(i // 13, 2), i == 30)
        else:
            late()
            direct(0, 2, (13,), 0)
            direct(1, 2, (13,), 3)
            for part, r in ((0, 0), (1, 0), (0, 3), (1, 3), (0, 4), (0, 5), (2, 0), (3, 0), (2, 3), (3, 3)):
                prod(part, r, 0)
            next_phase(0)
            for r in (1, 2, 6, 7, 8):
                prod(0, r, 1)
                prod(1, r, 1)
            assert all(w.func is not sum_h for w in works[1])
            next_phase(1)
            for r in range(9, 15):
                prod(0, r, 2)
            for r in (1, 2, 6, 7, 8):
                prod(2, r, 2)
                prod(3, r, 2)
            direct(0, 2, (12,), 3)
            direct(1, 2, (12,), 3)
        note(h_s, 0)
        note(hs_s, 0)
        assert not works[2]
        if not gated:
            del toks[:]
        k_s[:, 0:HALO, :] = k_s[:, tm:tm + HALO, :]
        v_s[:, 0:HALO, :] = v_s[:, tm:tm + HALO, :]
        for r in range(2):
            emit(blk, base, (r * hm, 4, acc[(r, 4)] + _nn(gate(half(a_s, r, 0, D)), _unpack(wo_p[:, 512:D]))))
        for c in range(2):
            cs = (c * 128, 256 + c * 128)

            def p(i):
                if i == 2:
                    wo = wo_p[0:128, cs[0]:cs[0] + 128]
                elif i == 5:
                    wo = wo_p[128:256, cs[1]:cs[1] + 128]
                else:
                    wo = to_s[RS[i] * 128:(RS[i] + 1) * 128, cs[0]:cs[0] + 128]
                m = _nn(lhs(a_s, 256, i), _unpack(wo))
                fire(last, m, NPDD / 9.0 + 0.01)
                return m

            def left(r, cc):
                return acc[(r, c + 2 * cc)] + _nn(half(a_s, r, 512, D), _unpack(wo_p[256:320, cs[cc]:cs[cc] + 128]))
            l21 = left(1, 0)
            m4 = p(4)
            m2 = p(2)
            c21 = l21 + m4 + m2
            m1 = p(1)
            t11 = m1 + m4
            t22 = m1 - m2
            m3 = p(3)
            m5 = p(5)
            c12 = m3 + m5 + left(0, 1)
            c11 = t11 - m5 + p(7) + left(0, 0)
            c22 = t22 + m3 + p(6) + left(1, 1)
            emit(blk, base, (hm, c, c21))
            emit(blk, base, (0, c + 2, c12))
            emit(blk, base, (0, c, c11), (hm, c + 2, c22))
        assert not last

    def step(b):
        blk = b + 1
        base = pl.multiple_of(TM0 + b * TM1, 16)
        nblk = jnp.minimum(blk + 1, NL)
        reset(1)
        side = {}

        def xt(r, k):
            return _unpack(xn_s[r * HP:(r + 1) * HP, k * 128:(k + 1) * 128])

        def xsum(i):
            return _unpack(xs_s[i * HP:(i + 1) * HP, :])

        def mm(mat, l, w):
            return (_nn if mat == 0 else _nt)(l, w)

        def tick(v):
            fire(side['work'], v, side['per'])

        def hk(mat, n0, r):
            l = xt(*HK_LP[r]) if r in HK_LP else xsum(HK_LS[r])
            if r in HK_RP:
                w = wtile(mat, HK_RP[r][0], n0 + HK_RP[r][1])
            else:
                row = t_tri(mat, n0, HK_RS[r])
                w = _unpack(t1_s[row:row + 64, :])
            return mm(mat, l, w)

        def st(mat, n0, i):
            l = xt(0, 3) if i == 3 else xt(1, 4) if i == 4 else xsum(11 + LS[i])
            if i == 2:
                w = wtile(mat, 3, n0)
            elif i == 5:
                w = wtile(mat, 4, n0 + 1)
            else:
                row = t_pair(mat, n0, RS[i])
                w = _unpack(t1_s[row:row + 64, :])
            return mm(mat, l, w)

        def add(acc, key, v):
            acc[key] = v if key not in acc else acc[key] + v

        def s_a(acc, mat, n0):
            m1, m4, m5, m7 = [st(mat, n0, i) for i in (1, 4, 5, 7)]
            add(acc, (0, n0), (m1 + m4) + (m7 - m5))
            tick(acc[(0, n0)])
            add(acc, (1, n0 + 1), m1)
            add(acc, (1, n0), m4)
            add(acc, (0, n0 + 1), m5)

        def s_b(acc, mat, n0):
            m2, m3, m6 = [st(mat, n0, i) for i in (2, 3, 6)]
            add(acc, (1, n0), m2)
            add(acc, (0, n0 + 1), m3)
            add(acc, (1, n0 + 1), (m3 - m2) + m6)
            tick(acc[(1, n0 + 1)])

        def h_a(acc, mat, n0):
            r0, r9, r11, r10 = [hk(mat, n0, r) for r in (0, 9, 11, 10)]
            t = r9 + r11
            w0 = r0 + t
            add(acc, (0, n0), w0 + r10)
            tick(acc[(0, n0)])
            acc[(1, n0)] = acc[(1, n0)] - w0
            add(acc, (0, n0 + 2), t + r10)
            acc[(1, n0 + 2)] = acc[(1, n0 + 2)] - r11 if (1, n0 + 2) in acc else -r11

        def h_b(acc, mat, n0):
            r7, r6, r8, r1 = [hk(mat, n0, r) for r in (7, 6, 8, 1)]
            add(acc, (0, n0), r7)
            add(acc, (1, n0), (r1 + r6) + r8)
            tick(acc[(1, n0)])
            add(acc, (0, n0 + 1), r6 + r7)
            add(acc, (1, n0 + 1), r8)

        def h_c(acc, mat, n0):
            r3, r12, r14, r13 = [hk(mat, n0, r) for r in (3, 12, 14, 13)]
            t = r12 + r14
            w1 = r3 + t
            acc[(0, n0 + 1)] = acc[(0, n0 + 1)] - w1
            add(acc, (1, n0 + 1), w1 + r13)
            tick(acc[(1, n0 + 1)])
            acc[(0, n0 + 2)] = acc[(0, n0 + 2)] - r14
            add(acc, (1, n0 + 2), t + r13)

        def h_1(acc, mat, n0, r):
            add(acc, {2: (0, n0 + 1), 4: (0, n0 + 2), 5: (1, n0 + 2)}[r], hk(mat, n0, r))

        def group6(mat, n0, done, filler):
            acc = {}

            def fin(*keys):
                for key in keys:
                    done(key[0], key[1], acc.pop(key))
            s_a(acc, mat, n0)
            s_b(acc, mat, n0)
            h_1(acc, mat, n0, 2)
            h_a(acc, mat, n0)
            h_b(acc, mat, n0)
            fin((0, n0), (1, n0))
            h_c(acc, mat, n0)
            fin((0, n0 + 1), (1, n0 + 1))
            s_a(acc, mat, n0 + 2)
            s_b(acc, mat, n0 + 2)
            h_1(acc, mat, n0, 5)
            fin((1, n0 + 2))
            s_a(acc, mat, n0 + 4)
            s_b(acc, mat, n0 + 4)
            h_1(acc, mat, n0, 4)
            fin((0, n0 + 2))
            h_a(acc, mat, n0 + 3)
            h_b(acc, mat, n0 + 3)
            fin((0, n0 + 3), (1, n0 + 3))
            h_c(acc, mat, n0 + 3)
            fin((1, n0 + 4))
            for r in (2, 4, 5):
                h_1(acc, mat, n0 + 3, r)
            fin((0, n0 + 4), (0, n0 + 5), (1, n0 + 5))
            assert not acc
            filler()

        work = [P(ln_pair, nblk, k * LC, xn2_s, xs2_s) for k in range(HM1 // LC)]
        side.update(work=work, per=len(work) / LNSPAN)
        acc = {}
        plain = [(r, k) for k in (3, 4) for r in range(2)]

        def fill_q():
            r, k = plain.pop(0)
            add(acc, (r, 14), mm(0, xt(r, k), wtile(0, k, 14)))

        def done_q(r, n, val):
            store_qkv(n, r * HM1, val)

        def fin_q(*keys):
            for key in keys:
                done_q(key[0], key[1], acc.pop(key))
        group6(0, 0, done_q, fill_q)
        group6(0, 6, done_q, fill_q)
        s_a(acc, 0, 12)
        s_b(acc, 0, 12)
        h_1(acc, 0, 12, 2)
        h_a(acc, 0, 12)
        h_b(acc, 0, 12)
        fin_q((0, 12), (1, 12))
        h_c(acc, 0, 12)
        fin_q((0, 13), (1, 13))
        h_1(acc, 0, 12, 4)
        h_1(acc, 0, 12, 5)
        fill_q()
        fill_q()
        fin_q((0, 14), (1, 14))
        assert not work and not acc

        work = [P(attn_rows, c * RC, False) for c in range(TM1 // RC)]
        side.update(work=work, per=APER)
        credit[0] = AOFF

        def store_h(r, n, v):
            h_s[r * HP:(r + 1) * HP, n * 128:(n + 1) * 128] = _pack(v)

        s_a(acc, 3, 0)
        s_b(acc, 3, 0)
        h_1(acc, 3, 0, 2)
        h_a(acc, 3, 0)
        h_b(acc, 3, 0)
        for r in range(2):
            store_h(r, 13, tail_h(acc.pop((r, 0))))
        h_c(acc, 3, 0)
        for r in range(2):
            hold_s[(12 + r) * HM1:(13 + r) * HM1, :] = _gelu(acc.pop((r, 1)))
        plain = [(r, k) for r in range(2) for k in (3, 4)]

        def fill_g():
            r, k = plain.pop(0)
            l = xt(r, k)
            add(acc, (r, 2), mm(3, gate(l) if len(plain) == 3 else l, wtile(3, k, 2)))

        def late():
            for r in range(2):
                h_1(acc, 3, 0, 4 + r)
                store_h(r, 12, hold_s[(12 + r) * HM1:(13 + r) * HM1, :] * acc.pop((r, 2)))
        for n0 in (0, 6):
            def slot(r, n):
                s = (n - n0) * 2 + r
                return slice(s * HM1, (s + 1) * HM1)

            def early(r, n):
                return (GPAT >> ((n - n0) * 2 + r)) & 1

            def done_g(r, n, v):
                hold_s[slot(r, n), :] = _gelu(v) if early(r, n) else v

            def done_u(r, n, v):
                g = hold_s[slot(r, n), :]
                store_h(r, n, (g if early(r, n) else _gelu(g)) * v)
            if n0 == 6:
                n_att = int(24 * APER)
                work[:] = _weave(work[:n_att], sum_items(HP, 0)) + work[n_att:]
                side.update(per=(n_att + 3 * HP // 8) / 24.0)
            group6(1, n0, done_g, fill_g)
            group6(2, n0, done_u, fill_g)
        assert not plain
        note(hold_s, 0)

        def copy_xn(dst, src, r0, c, trig):
            dst[r0:r0 + HP, c:c + 128] = after(src[pl.ds(zrow(), r0 + HP), c:c + 128][r0:r0 + HP], trig)
            if c == 0:
                note(dst, r0)
        copies = [P(copy_xn, xn_s, xn2_s, r, c) for r in (0, HP) for c in range(0, D, 128)]
        copies += [P(copy_xn, xs_s, xs2_s, i * HP, 0) for i in range(NSUM)]
        sums = [w for w in work if w.func is sum_h] + sum_items(HP, 1)
        work = [w for w in work if w.func is not sum_h]
        s12 = [w for w in sums if w.args[1:3] == (1, 2)]
        w0 = _weave([w for w in sums if w.args[1:3] != (1, 2)], work[:NA0])
        w1 = _weave(work[NA0:], s12 + copies)
        credit[0] = 0.0
        stage2(blk, base, TM1, [w0, w1, w1], [len(w0) / SPAN0, len(w1) / A2SPAN, len(w1) / A2SPAN], True, late)

    def cp(src, dst, s):
        return pltpu.make_async_copy(src, dst, sem_i.at[s])

    def gu(groups, s):
        return [cp(h.at[pl.ds(g * 128, 128)], d.at[pl.ds(g * 128, 128)], s)
                for g in groups for h, d in ((wg_hbm, wg_s), (wu_hbm, wu_s))]

    def wcol(t, s):
        return cp(wqkv_hbm.at[:, pl.ds(t * D, D)], wqkv_r.at[:, pl.ds(t * D, D)], s)

    def xblk(b, s):
        return cp(x_hbm.at[pl.ds(TM0 + b * TM1, TM1)], x_s.at[b + 1, pl.ds(0, TM1)], s)

    HM = TM0 // 2
    cp_x0 = [cp(x_hbm.at[pl.ds(i * HM, HM)], x_s.at[0, pl.ds(i * HM, HM)], i) for i in range(2)]
    cp_gu = [gu(g, 2 + k) for k, g in enumerate(G_EARLY)]
    cp_q = gu(G_Q, 5) + [cp(wg_hbm.at[pl.ds(FM, 64)], wt_s.at[pl.ds(0, 64)], 5),
                         cp(wu_hbm.at[pl.ds(FM, 64)], wt_s.at[pl.ds(64, 64)], 5), wcol(0, 5), xblk(0, 5)]
    cp_kv = gu(G_KV, 6) + [wcol(1, 6), wcol(2, 6)]
    cp_r = gu(G_R + G_D, 7) + [cp(wo_hbm, wo_r, 7)]
    cp_d = [cp(wd_hbm, wd_s.at[pl.ds(0, F)], 8)]
    cp_xs = [xblk(b, 9) for b in range(1, NL)]

    for c in cp_x0 + sum(cp_gu, []) + cp_q + cp_kv + cp_r + cp_d + cp_xs:
        c.start()
    zero_s[0] = 0
    k_s[:, 0:HALO, :] = jnp.zeros((NJ, HALO, 128), F32)
    v_s[:, 0:HALO, :] = jnp.zeros((NJ, HALO, 128), F32)
    wd_s[F:FP, :] = jnp.zeros((FP - F, D), BF)

    def first_block():
        def wait(cps):
            reset(CH0)
            for c in cps:
                c.wait()

        parts = []
        for i in range(2):
            wait(cp_x0[i:i + 1])
            parts += [ln_rows(0, i * HM + k * LC).astype(BF) for k in range(HM // LC)]
        xn = jnp.concatenate(parts, axis=0)

        def ffn_group(x, row0, g0, work, per, gated=False):
            g = _nt(x, wg_s[g0 * 128:(g0 + 1) * 128, :])
            fire(work, g, per)
            u = _nt(gate(x) if gated else x, wu_s[g0 * 128:(g0 + 1) * 128, :])
            fire(work, u, per)
            h_s[row0 // 2:(row0 + x.shape[0]) // 2, g0 * 128:(g0 + 1) * 128] = _pack(_gelu(g) * u)

        def ffn_groups(groups, work, per, gate_last=False):
            groups = list(groups)
            if len(groups) % 2:
                g0 = groups.pop(0)
                ffn_group(xn[0:HM], 0, g0, work, per)
                ffn_group(xn[HM:], HM, g0, work, per)
            for k, g0 in enumerate(groups):
                ffn_group(xn, 0, g0, work, per, gate_last and k == len(groups) - 1)

        have, done = set(), set()

        def new_preps(groups):
            have.update(groups)
            tris = [n for n in (0, 3, 6, 9) if {n, n + 1, n + 2} <= have and ('t', n) not in done]
            pairs = [n for n in range(0, 12, 2) if {n, n + 1} <= have and ('p', n) not in done]
            done.update([('t', n) for n in tris] + [('p', n) for n in pairs])
            return preps(1, tris, pairs) + preps(2, tris, pairs)

        perm = [[P(permute_qkv, t, r0) for r0 in range(0, D, 64)] for t in range(3)]

        for k, (cps, groups) in enumerate(zip(cp_gu, G_EARLY)):
            wait(cps)
            work = new_preps(groups)
            nres = 2 * len(groups) + 2 * (len(groups) % 2)
            ffn_groups(groups, work, max(len(work), 1) / max(nres - 2.0, 1.0), k == 2)
            assert not work

        wait(cp_q)
        work = perm[0]
        for _ in range(3):
            work.pop(0)(None)
        t = _nt(xn, wt_s[...])
        fire(work, t, 4)
        h_s[0:TM0 // 2, FM:FP] = _pack(tail_h(t))
        work += new_preps(G_Q) + [P(ln_pair, 1, k * LC, xn_s, xs_s) for k in range(HM1 // LC)]
        for g0 in G_Q:
            ffn_group(xn, 0, g0, work, QPER)
        assert all(w.func is ln_pair for w in work)
        per = len(work) / QSPAN
        for j in range(NJ):
            r = _nn(xn, _unpack(wqkv_p[:, j * 128:(j + 1) * 128]))
            fire(work, r, per)
            store_qkv(j, 0, r)
        assert not work

        wait(cp_kv)
        work = perm[1]
        for _ in range(4):
            work.pop(0)(None)
        for g0 in G_KV:
            g = _nt(xn, wg_s[g0 * 128:(g0 + 1) * 128, :])
            fire(work, g, 6)
            u = _nt(xn, wu_s[g0 * 128:(g0 + 1) * 128, :])
            h_s[0:TM0 // 2, g0 * 128:(g0 + 1) * 128] = _pack(_gelu(g) * u)
        assert not work
        work = perm[2] + _weave(new_preps(G_KV), _weave(preps(0, range(0, 15, 3), []),
                                                        preps(0, [], range(0, 14, 2))))
        per = len(work) / KVSPAN
        fire(work, u, per)
        for c in range(NJ, 3 * NJ):
            assert c < 2 * NJ or all(w.func is not permute_qkv for w in work)
            r = _nn(gate(xn) if c == 3 * NJ - 1 else xn, _unpack(wqkv_p[:, c * 128:(c + 1) * 128]))
            fire(work, r, per)
            store_qkv(c, 0, r)
        assert not work

        wait(cp_r)
        att = [P(attn_rows, rc * RC, True) for rc in range(TM0 // RC)]
        work = _weave(new_preps(G_R + G_D) + preps(3, [0], [0]), att[:NAR])
        att = att[NAR:]
        ffn_groups(G_R, work, len(work) / (2 * len(G_R) - 2.0))
        assert not work

        wait(cp_d)
        chain[0] = CHD
        wo_work = []
        for jj in range(NJ):
            wo_work += [P(widen_wo, jj, r0) for r0 in range(0, D, UW)]
            wo_work += [P(gather_wo, jj, j) for j in range(NJ)]
        pd = [P(prep_d, part, o, r0) for part, no in ((0, 4), (1, 4), (2, 3), (3, 1)) for o in range(no)
              for r0 in range(0, 128, UD)]
        po = [P(prep_o, r0, c) for r0 in range(0, 128, UD // 2) for c in (0, 128)]
        wa = _weave(*[l for l in (wo_work, pd[:NPDA], att[:NAA]) if l])
        wd_ = pd[len(pd) - NPDD:]
        pd = pd[:len(pd) - NPDD]
        wb = _weave(*[l for l in (pd[NPDA:NPDA + NPDB], po, att[NAA:NAA + NAB]) if l])
        wc = _weave(*[l for l in (pd[NPDA + NPDB:], att[NAA + NAB:]) if l])
        per = len(wa) / SPANA
        ffn_groups(G_D, wa, per)
        stage2(0, 0, TM0, [wa, wb, wc], [per, len(wb) / SPANB, max(len(wc), 1) / SPANC], False, None, wd_)

    def main(i, carry):
        first_block()
        for c in cp_xs:
            c.wait()

        def body(b, c):
            step(b)
            return c
        return jax.lax.fori_loop(0, NL, body, carry)

    jax.lax.fori_loop(0, zero_s[0] + 1, main, 0)

    for j in range(NJ):
        for r in range(2):
            cp_o(0, 0, r * HM, HM, j).wait()
    for b in range(NL):
        for j in range(NJ):
            for r in range(2):
                cp_o(b + 1, TM0 + b * TM1, r * HM1, HM1, j).wait()


@jax.jit
def pallas_parallel_sum__sliding_local_dilated__geglu_ffn__prompt_kernel(
    A_x: jax.Array,
    A_wqkv: jax.Array,
    A_wo: jax.Array,
    B_x: jax.Array,
    B_w_gate: jax.Array,
    B_w_up: jax.Array,
    B_w_down: jax.Array,
):
    x = A_x.reshape(S, D)
    hbm = pl.BlockSpec(memory_space=pltpu.MemorySpace.HBM)
    out = pl.pallas_call(
        _kernel,
        in_specs=[hbm] * 6,
        out_specs=hbm,
        out_shape=jax.ShapeDtypeStruct((S, D), BF),
        scratch_shapes=[
            pltpu.VMEM((NL + 1, TMP, D), BF),
            pltpu.VMEM((TM1 // 2, D), U32),
            pltpu.VMEM((NSUM * HP, 128), U32),
            pltpu.VMEM((TM1 // 2, D), U32),
            pltpu.VMEM((NSUM * HP, 128), U32),
            pltpu.VMEM((NL + 1, TMP, D), BF),
            pltpu.VMEM((D, 3 * D), BF),
            pltpu.VMEM((D // 2, 3 * D), U32),
            pltpu.VMEM((D, D), BF),
            pltpu.VMEM((NJ * D, 128), F32),
            pltpu.VMEM((D // 2, D), U32),
            pltpu.VMEM((FM, D), BF),
            pltpu.VMEM((FM, D), BF),
            pltpu.VMEM((128, D), BF),
            pltpu.VMEM((FP, D), BF),
            pltpu.VMEM((226 * 64, 128), U32),
            pltpu.VMEM((76 * 64, 128), U32),
            pltpu.VMEM((5 * 128, 256), U32),
            pltpu.VMEM((NJ, TMX, 128), F32),
            pltpu.VMEM((NJ, TMX + HALO, 128), F32),
            pltpu.VMEM((NJ, TMX + HALO, 128), F32),
            pltpu.VMEM((TMX // 2, FP), U32),
            pltpu.VMEM((NSUM * TMX // 4, 512), U32),
            pltpu.VMEM((TMX // 2, D), U32),
            pltpu.VMEM((NHOLD * HM1, 128), F32),
            pltpu.SMEM((1,), jnp.int32),
            pltpu.SemaphoreType.DMA((10,)),
            pltpu.SemaphoreType.DMA((1,)),
        ],
        compiler_params=pltpu.CompilerParams(
            vmem_limit_bytes=100 * 1024 * 1024,
            disable_bounds_checks=True,
            disable_semaphore_checks=True,
        ),
    )(x, A_wqkv, A_wo, B_w_gate.T, B_w_up.T, B_w_down)
    return out.reshape(1, S, D)
```

```python
import functools

import jax
import jax.numpy as jnp
import jax.experimental.pallas as pl
import jax.experimental.pallas.tpu as pltpu

S, D, H, DH, W, DIL, F = 2048, 640, 32, 20, 8, 2, 1728
TM0 = 384
NL = 4
TM1 = (S - TM0) // NL
HM1 = TM1 // 2
HP = HM1 // 2
TMX = max(TM0, TM1)
TMP = (TMX + 63) // 64 * 64
HALO = 16
NJ = D // 128
LOG2E = 1.4426950408889634
FM = 1664
FP = 1792
RC = 16
LC = 16
NHOLD = 14
G_EARLY = [[0], [1, 2], [3, 4, 5]]
G_Q, G_KV, G_R, G_D = [6], [7], [8, 9, 10, 11], [12]
QORD = (0, 1, 2, 3, 4, 5, 10, 11, 12, 13, 14, 6, 7, 8, 9)
LNSPAN = 22
APER = 0.344
GPAT = 0x999
A2SPAN = 18
AOFF = 2.9
NAR = 1
NAA = 10
NAB = 9
SPANA = 15.5
SPANB = 12.9
SPANC = 10
KVSPAN = 9.4
QPER = 1.5
QSPAN = 3.5
CH0 = 3
ESLACK = 0.8
KLATE = 1
RSPAN = 7.2
RFREE = 8
NPDB = 24
NPDD = 16
NPDA = 20
NA0 = 2
SPAN0 = 6.5
CHD = 2
UT = 16
UP = 32
UD = 16
UW = 64

BF = jnp.bfloat16
F32 = jnp.float32
U32 = jnp.uint32
NT = (((1,), (1,)), ((), ()))
P = functools.partial


def _gelu(g):
    c0 = 0.7978845608028654
    c1 = c0 * 0.044715
    t = jnp.tanh(g * (c0 + c1 * (g * g)))
    hg = 0.5 * g
    return hg + hg * t


def _pack(x):
    return pltpu.bitcast(x.astype(BF), U32)


def _unpack(u):
    return pltpu.bitcast(u, BF)


def _lhs_sums(a11, a12, a21, a22):
    return [a11 + a22, a21 + a22, a11 + a12, a21 - a11, a12 - a22]


def _rhs_sums(b11, b12, b21, b22):
    return [b11 + b22, b12 - b22, b21 - b11, b11 + b12, b21 + b22]


LS = {1: 0, 2: 1, 5: 2, 6: 3, 7: 4}
RS = {1: 0, 3: 1, 4: 2, 6: 3, 7: 4}

HK_R = {0: ((0, 0, 1), (0, 2, -1), (1, 0, 1)), 1: ((0, 0, 1), (0, 1, -1), (2, 0, 1)),
        2: ((1, 1, 1), (1, 0, -1), (2, 1, 1)), 3: ((0, 1, 1), (1, 1, 1), (1, 2, -1)),
        4: ((1, 2, 1), (2, 0, -1), (2, 2, 1)), 5: ((0, 2, 1), (2, 1, -1), (2, 2, 1)),
        6: ((0, 1, 1), (1, 0, 1)), 9: ((0, 2, 1), (2, 0, 1)), 12: ((1, 2, 1), (2, 1, 1))}
HK_RS = {r: i for i, r in enumerate(HK_R)}
HK_RP = {7: (1, 0), 8: (0, 1), 10: (2, 0), 11: (0, 2), 13: (2, 1), 14: (1, 2)}
HK_LP = {0: (0, 0), 3: (1, 1), 4: (0, 2), 5: (1, 2)}
HK_LS = {r: i for i, r in enumerate((1, 2, 6, 7, 8, 9, 10, 11, 12, 13, 14))}
NSUM = 16
HK_O = {0: ((0, 0, 1), (1, 0, -1)), 1: ((1, 0, 1),), 2: ((0, 1, 1),), 3: ((0, 1, -1), (1, 1, 1)),
        4: ((0, 2, 1),), 5: ((1, 2, 1),), 6: ((1, 0, 1), (0, 1, 1)), 7: ((0, 0, 1), (0, 1, 1)),
        8: ((1, 0, 1), (1, 1, 1)), 9: ((0, 0, 1), (1, 0, -1), (0, 2, 1)), 10: ((0, 0, 1), (0, 2, 1)),
        11: ((0, 0, 1), (1, 0, -1), (0, 2, 1), (1, 2, -1)), 12: ((0, 1, -1), (1, 1, 1), (1, 2, 1)),
        13: ((1, 1, 1), (1, 2, 1)), 14: ((0, 1, -1), (1, 1, 1), (0, 2, -1), (1, 2, 1))}
KB = ((0, 1, 6, 7), (2, 3, 8, 9), (4, 5, 10, 11))
EB = ((4, 10, 12), (5, 11, 13))
LB = ((12,), (13,))
SUB_RS = {r: i for i, r in enumerate((0, 1, 2, 3, 6))}


def _hk_lhs_sums(x, y):
    s0, s1, s2 = x[0] + y[0], x[1] + y[1], x[2] + y[2]
    return [s0, s1, x[0] + y[1], x[1] - x[0], y[0] - y[1], s0 - y[2], s2 - s0, y[2] - y[0],
            s1 - x[2], s2 - s1, x[2] - x[1]]


def _nn(a, b):
    return jnp.dot(a, b, preferred_element_type=F32)


def _nt(a, b):
    return jax.lax.dot_general(a, b, NT, preferred_element_type=F32)


def _weave(*lists):
    items = []
    for lst in lists:
        items += [((k + 0.5) / len(lst), w) for k, w in enumerate(lst)]
    items.sort(key=lambda t: t[0])
    return [t[1] for t in items]


def _kernel(x_hbm, wqkv_hbm, wo_hbm, wg_hbm, wu_hbm, wd_hbm, out_hbm,
            x_s, xn_s, xs_s, xn2_s, out_s, wqkv_r, wqkv_p, wo_r, wo_f, wo_p,
            wg_s, wu_s, wt_s, wd_s, t1_s, td_s, to_s, q_s, k_s, v_s, h_s, hs_s, a_s, hold_s, w3_s, w4_s, sc_s,
            zero_s, sem_i, sem_o):

    def zrow():
        return pl.multiple_of(zero_s[0] * 8, 8)

    masks_ = {}

    def keep(shape):
        if shape not in masks_:
            masks_[shape] = jax.lax.broadcasted_iota(jnp.int32, shape, len(shape) - 1) >= zero_s[0]
        return masks_[shape]

    def after(val, trig):
        if trig is None:
            return val
        n = val.shape[0] // 8
        t = pltpu.bitcast(trig, val.dtype) if trig.dtype != val.dtype else trig
        if n > 1:
            t = jnp.concatenate([t] * n, axis=0)
        return jnp.where(keep(val.shape), val, t)

    def after_head(val, trig):
        if trig is None:
            return val
        if val.shape[1] == 128:
            return after(val, trig)
        return jnp.concatenate([after(val[:, 0:128], trig), val[:, 128:]], axis=1)

    toks = []
    credit = [0.0]
    chain = [0]
    prev = []

    anchor = [False]
    extra = []

    def reset(dist):
        anchor[0] = False
        masks_.clear()
        del extra[:]
        del toks[:]
        del prev[:]
        credit[0] = 0.0
        chain[0] = dist

    def note(ref, row):
        if all(r is not ref for r, _ in toks):
            toks.append((ref, row))

    def gate(lhs):
        if not toks and not extra:
            return lhs
        tok = functools.reduce(lambda p, q: p | q, extra + [
            pltpu.bitcast(ref[pl.ds(zrow() + row, 8), 0:128], U32) for ref, row in toks])
        del toks[:]
        del extra[:]
        u = pltpu.bitcast(lhs[0:16], U32)
        return jnp.concatenate([_unpack(after_head(u, tok)), lhs[16:]], axis=0)

    def fire(work, res, per):
        if not work:
            credit[0] = 0.0
            return
        pos = credit[0]
        while pos < 1.0 and work:
            r = int((res.shape[0] - 8) * pos) // 8 * 8
            trig = pltpu.bitcast(res[r:r + 8, :], U32)
            item = work.pop(0)
            if item.func in (attn_rows, ln_pair) and len(prev) >= chain[0]:
                trig = trig | prev[-chain[0]]
            tok = item(trig)
            if tok is not None:
                prev.append(pltpu.bitcast(tok, U32))
            pos += 1.0 / per
        credit[0] = max(pos - 1.0, 0.0)

    lane = jax.lax.broadcasted_iota(jnp.int32, (32, 128), 1)
    l5 = lane % 5
    masks = [l5 == r for r in range(5)]
    idx = [(DH * (lane % H) + 5 * (lane // H) + j) % 128 for j in range(NJ)]

    def permute_qkv(t, r0, trig):
        src = [pltpu.bitcast(wqkv_r[r0:r0 + 64, t * D + s * 128:t * D + (s + 1) * 128], U32)
               for s in range(NJ)]
        src[4] = after(src[4], trig)
        for j in range(NJ):
            mg = src[4]
            for s in range(3, -1, -1):
                mg = jnp.where(masks[(j - 3 * s) % 5], src[s], mg)
            res = jnp.take_along_axis(mg, idx[j], axis=1, mode="promise_in_bounds")
            wqkv_p[r0 // 2:r0 // 2 + 32, t * D + j * 128:t * D + (j + 1) * 128] = res

    def widen_wo(jj, r0, trig):
        w = after(pltpu.bitcast(wo_r[r0:r0 + UW, jj * 128:(jj + 1) * 128], U32), trig)
        wo_f[jj * D + r0:jj * D + r0 + UW, :] = _unpack(w).astype(F32)

    def gather_wo(jj, j, trig):
        for g in range(4):
            rows = wo_f[pl.ds(jj * D + 5 * g + j, H, stride=DH), :]
            rows = jnp.concatenate([after(rows[r:r + 8], trig) if r % 16 == 0 else rows[r:r + 8]
                                    for r in range(0, H, 8)], axis=0)
            r0 = (j * 128 + g * H) // 2
            wo_p[r0:r0 + H // 2, jj * 128:(jj + 1) * 128] = _pack(rows)

    def prep(b11, b12, b21, b22, store, trig):
        b11, b12, b21, b22 = [b.astype(F32) for b in (b11, b12, b21, b22)]
        b11 = after(b11, trig)
        b22 = after(b22, trig)
        for i, s in enumerate(_rhs_sums(b11, b12, b21, b22)):
            store(i, _pack(s))

    def wtile(mat, k, n, r0=0, nr=128):
        if mat == 3:
            if n == 1:
                return wtile(1, k, 12, r0, nr)
            return _unpack(w3_s[n * 32 + r0 // 2:n * 32 + (r0 + nr) // 2, k * 128:(k + 1) * 128])
        if mat == 0:
            ref, c = (w4_s, n // 6) if n in (5, 11) else (wqkv_p, QORD[n])
            return _unpack(ref[k * 64 + r0 // 2:k * 64 + (r0 + nr) // 2, c * 128:(c + 1) * 128])
        return (wg_s, wu_s)[mat - 1][n * 128 + r0:n * 128 + r0 + nr, k * 128:(k + 1) * 128]

    peak = {}

    def scan_peak(w, ref, r0, n, c0, c1, trig):
        u = ref[r0:r0 + n, c0:c1]
        u = u if u.dtype == U32 else pltpu.bitcast(u, U32)
        m = pltpu.bitcast(after_head(u, trig) & jnp.uint32(0x7FFFFFFF), F32)
        m = functools.reduce(jnp.maximum, [m[r:r + 8, c:c + 128] for r in range(0, m.shape[0], 8)
                                           for c in range(0, m.shape[1], 128)])
        peak[w] = m if w not in peak else jnp.maximum(peak[w], m)

    def set_scale(i, trig):
        e = [pltpu.bitcast(jnp.broadcast_to(jnp.max(peak.pop(w), keepdims=True), (8, 128)), jnp.int32) >> 23
             for w in range(2)]
        d = jnp.where(jnp.minimum(e[0], e[1]) > 0, jnp.clip(e[0] - e[1], -60, 60), 0)
        sc_s[16 * i:16 * i + 8, :] = pltpu.bitcast((127 + d) << 23, F32)
        sc_s[16 * i + 8:16 * i + 16, :] = pltpu.bitcast((127 - d) << 23, F32)

    def rescale_k(i, r0, trig):
        w = _unpack(wqkv_p[r0:r0 + 32, (5 + i) * 128:(6 + i) * 128]).astype(F32)
        w4_s[r0:r0 + 32, i * 128:(i + 1) * 128] = _pack(w * after(sc_s[16 * i + 16:16 * i + 24, :], trig)[0:1])

    def balance_k():
        items = []
        for i, c in enumerate((4, 14)):
            items += [P(scan_peak, w, wqkv_p, 0, 64, cc * 128, (cc + 1) * 128) for w, cc in enumerate((c, 5 + i))]
            items += [P(set_scale, 1 + i)]
        return items, [P(rescale_k, i, r0) for i in range(2) for r0 in range(0, D // 2, 32)]

    def rescale(r0, trig):
        w = wt_s[r0:r0 + 16, :] if r0 < 128 else wu_s[11 * 128 + r0:11 * 128 + r0 + 16, :]
        s = after(sc_s[0:8, :], trig)[0:1] if r0 >= 64 else after(jnp.ones((8, 128), F32), trig)[0:1]
        for c in range(0, D, 128):
            w3_s[r0 // 2:r0 // 2 + 8, c:c + 128] = _pack(w[:, c:c + 128].astype(F32) * s)

    def balance_items():
        items = [P(scan_peak, w, ref, 12 * 128, 32, 0, D) for w, ref in enumerate((wg_s, wu_s))]
        return items + [P(set_scale, 0)], [P(rescale, r0) for r0 in range(0, 256, 16)]

    def t_tri(mat, n0, i):
        return ((0, 80, 146, 212)[mat] + n0 // 3 * 9 + i) * 64

    def t_pair(mat, n0, i):
        return ((45, 116, 182, 221)[mat] + n0 // 2 * 5 + i) * 64

    def prep_tri(mat, n0, r0, trig):
        b = [[wtile(mat, k, n0 + n, r0, UT).astype(F32) for n in range(3)] for k in range(3)]
        for k, n in ((1, 0), (0, 1), (0, 2), (1, 2)):
            b[k][n] = after(b[k][n], trig)
        for r, terms in HK_R.items():
            s = None
            for k, n, c in terms:
                s = b[k][n] if s is None else (s + b[k][n] if c > 0 else s - b[k][n])
            row = t_tri(mat, n0, HK_RS[r]) + r0 // 2
            t1_s[row:row + UT // 2, :] = _pack(s)

    def prep_pair(mat, n0, r0, trig):
        def store(i, o):
            row = t_pair(mat, n0, i) + r0 // 2
            t1_s[row:row + UP // 2, :] = o
        prep(wtile(mat, 3, n0, r0, UP), wtile(mat, 3, n0 + 1, r0, UP),
             wtile(mat, 4, n0, r0, UP), wtile(mat, 4, n0 + 1, r0, UP), store, trig)

    def preps(mat, tris, pairs):
        return ([P(prep_tri, mat, n0, r0) for n0 in tris for r0 in range(0, 128, UT)]
                + [P(prep_pair, mat, n0, r0) for n0 in pairs for r0 in range(0, 128, UP)])

    def td_row(part, i, o):
        return ((0, 36, 56, 71)[part] + i * (4, 4, 3, 1)[part] + o) * 64

    def prep_d(part, o, r0, trig):
        kt = [blk[o] for blk in (KB, KB[:2], EB, LB)[part]]
        n0 = (0, 3, 3, 0)[part]
        b = [[wd_s[k * 128 + r0:k * 128 + r0 + UD, (n0 + n) * 128:(n0 + n + 1) * 128].astype(F32)
              for n in range(len(kt))] for k in kt]
        for k, n in ((1, 0), (0, 1), (0, 2), (1, 2))[:2 * len(kt) - 2]:
            b[k][n] = after(b[k][n], trig)
        for r, i in (HK_RS if part == 0 else SUB_RS).items():
            s = None
            for k, n, c in HK_R[r]:
                if k < len(kt) and n < len(kt):
                    s = b[k][n] if s is None else (s + b[k][n] if c > 0 else s - b[k][n])
            row = td_row(part, i, o) + r0 // 2
            td_s[row:row + UD // 2, :] = _pack(s)

    def sum_h(hp, part, o, r0, trig):
        kt = [blk[o] for blk in (KB, EB)[part]]
        x, y = [[_unpack(after(h_s[r * hp + r0:r * hp + r0 + 8, k * 128:(k + 1) * 128], trig)).astype(F32)
                 for k in kt] for r in range(2)]
        sums = _hk_lhs_sums(x, y) if part == 0 else _hk_lhs_sums(x + x[:1], y + y[:1])[:5]
        for i, s in enumerate(sums):
            row = (i + 11 * part) * hp + r0
            hs_s[row:row + 8, o * 128:(o + 1) * 128] = _pack(s)

    def sum_items(hp, g):
        return [P(sum_h, hp, part, o, r0) for r0 in range(0, hp, 8)
                for part, o in (((0, 0), (0, 1), (1, 0)), ((0, 2), (0, 3), (1, 1), (1, 2)))[g]]

    def prep_o(r0, c, trig):
        n = UD // 2

        def store(i, o):
            to_s[i * 128 + r0:i * 128 + r0 + n, c:c + 128] = o
        prep(_unpack(wo_p[r0:r0 + n, c:c + 128]), _unpack(wo_p[r0:r0 + n, 256 + c:384 + c]),
             _unpack(wo_p[128 + r0:128 + r0 + n, c:c + 128]), _unpack(wo_p[128 + r0:128 + r0 + n, 256 + c:384 + c]),
             store, trig)

    def ln_rows(blk, r0, trig=None):
        x = after_head(x_s[blk, r0:r0 + LC, :].astype(F32), trig)
        m = jnp.sum(x, axis=-1, keepdims=True) * (1.0 / D)
        mb = m.astype(BF).astype(F32)
        xc = x - mb
        dm = m - mb
        var = jnp.sum(xc * xc, axis=-1, keepdims=True) * (1.0 / D) - dm * dm
        return xc * jax.lax.rsqrt(jnp.maximum(var, 0.0) + 1e-5)

    def ln_pair(blk, r0, xn_d, xs_d, trig):
        top = ln_rows(blk, r0, trig)
        bot = ln_rows(blk, HM1 + r0, trig)
        xn_d[r0 // 2:(r0 + LC) // 2, :] = _pack(top)
        xn_d[(HM1 + r0) // 2:(HM1 + r0 + LC) // 2, :] = _pack(bot)
        x = [top[:, k * 128:(k + 1) * 128] for k in range(NJ)]
        y = [bot[:, k * 128:(k + 1) * 128] for k in range(NJ)]
        note(xn_d, r0 // 2)
        if xs_d is not None:
            for i, s in enumerate(_hk_lhs_sums(x, y) + _lhs_sums(x[3], x[4], y[3], y[4])):
                xs_d[i * HP + r0 // 2:i * HP + (r0 + LC) // 2, :] = _pack(s)
            note(xs_d, r0 // 2)
        s0 = x[0] + y[0]
        return s0[0:8] + s0[8:16]

    def tail_h(t):
        ht = _gelu(t) * pltpu.roll(t, 64, 1)
        lo = jax.lax.broadcasted_iota(jnp.int32, ht.shape, 1) < 64
        return jnp.where(lo, ht, 0.0)

    def store_qkv(c, row0, val):
        t, j = divmod(c, NJ)
        n = val.shape[0]
        if t == 0:
            q_s[j, row0:row0 + n, :] = val * (DH ** -0.5 * LOG2E)
        elif t == 1:
            k_s[j, HALO + row0:HALO + row0 + n, :] = val
        else:
            v_s[j, HALO + row0:HALO + row0 + n, :] = val

    def attn_core(r0, first, trig):
        q = q_s[:, r0:r0 + 8, :]
        if trig is not None:
            q = jnp.where(keep((NJ, 8, 128)), q, pltpu.bitcast(trig, F32)[None])
        logits = []
        for w in range(W):
            st = HALO + r0 - DIL * w
            acc = jnp.sum(q * k_s[:, st:st + 8, :], axis=0)
            acc = acc + pltpu.roll(acc, 64, 1)
            acc = acc + pltpu.roll(acc, 32, 1)
            if first and r0 < DIL * w:
                rows = r0 + jax.lax.broadcasted_iota(jnp.int32, (8, 128), 0)
                acc = jnp.where(rows >= DIL * w, acc, -1e9 * LOG2E)
            logits.append(acc)
        mx = logits[0]
        for w in range(1, W):
            mx = jnp.maximum(mx, logits[w])
        ps = [jnp.exp2(l - mx) for l in logits]
        den = ps[0]
        for w in range(1, W):
            den = den + ps[w]
        r = pl.reciprocal(den, approx=True)
        inv = r * (2.0 - den * r)
        acc = ps[0][None] * v_s[:, HALO + r0:HALO + r0 + 8, :]
        for w in range(1, W):
            st = HALO + r0 - DIL * w
            acc = acc + ps[w][None] * v_s[:, st:st + 8, :]
        return acc * inv[None], mx

    def attn_rows(r0, first, trig):
        o1, t1 = attn_core(r0, first, trig)
        o2, t2 = attn_core(r0 + 8, first, t1)
        for j in range(NJ):
            a_s[r0 // 2:(r0 + RC) // 2, j * 128:(j + 1) * 128] = _pack(jnp.concatenate([o1[j], o2[j]], axis=0))
        if anchor[0]:
            extra.append(pltpu.bitcast(pltpu.roll(jnp.max(jnp.maximum(o1, o2), axis=0), 64, 1), U32))
        return t2

    def cp_o(blk, base, r0, n, j):
        return pltpu.make_async_copy(out_s.at[blk, pl.ds(r0, n), pl.ds(j * 128, 128)],
                                     out_hbm.at[pl.ds(base + r0, n), pl.ds(j * 128, 128)], sem_o.at[0])

    def emit(blk, base, *pieces):
        for r0, j, val in pieces:
            n = val.shape[0]
            x = x_s[blk, r0:r0 + n, j * 128:(j + 1) * 128].astype(F32)
            out_s[blk, r0:r0 + n, j * 128:(j + 1) * 128] = (x + val).astype(BF)
        for r0, j, val in pieces:
            cp_o(blk, base, r0, val.shape[0], j).start()

    def stage2(blk, base, tm, works, pers, gated=True, late=None, last=None):
        hm, hp = tm // 2, tm // 4
        anchor[0] = gated

        def half(ref, r, c0, c1):
            return _unpack(ref[r * hp:(r + 1) * hp, c0:c1])

        memo = {}

        def lhs(plain, kh, i):
            if i == 3:
                return half(plain, 0, 0, kh)
            if i == 4:
                return half(plain, 1, kh, 2 * kh)
            if (kh, i) not in memo:
                def b(r, c):
                    u = plain[pl.ds(zrow(), 2 * hp), c * kh:(c + 1) * kh]
                    return _unpack(u[r * hp:(r + 1) * hp]).astype(F32)
                s = {1: lambda: b(0, 0) + b(1, 1), 2: lambda: b(1, 0) + b(1, 1), 5: lambda: b(0, 0) + b(0, 1),
                     6: lambda: b(1, 0) - b(0, 0), 7: lambda: b(0, 1) - b(1, 1)}[i]()
                memo[(kh, i)] = s.astype(BF)
            return memo[(kh, i)]

        acc = {}

        def htiles(r, tiles):
            return jnp.concatenate([half(h_s, r, k * 128, (k + 1) * 128) for k in tiles], axis=1)

        def prod(part, r, phase):
            blocks = (KB, KB, EB, LB)[part]
            n0, nk = (0, 3, 3, 0)[part], len(blocks[0])
            if r in HK_LP:
                l = htiles(HK_LP[r][0], blocks[HK_LP[r][1]])
            else:
                row = (HK_LS[r] + (11 if part >= 2 else 0)) * hp
                c0 = 256 if part == 3 else 0
                l = _unpack(hs_s[row:row + hp, c0:c0 + nk * 128])
            if r in HK_RP:
                k, n = HK_RP[r]
                w = jnp.concatenate([wd_s[t * 128:(t + 1) * 128, (n0 + n) * 128:(n0 + n + 1) * 128]
                                     for t in blocks[k]], axis=0)
            else:
                row = td_row(part, (HK_RS if part == 0 else SUB_RS)[r], 0)
                w = _unpack(td_s[row:row + nk * 64, :])
            m = _nn(l, w)
            if part < 3:
                fire(works[phase], m, pers[phase])
            for rr, n, c in HK_O[r]:
                key = (rr, n0 + n)
                if key not in acc:
                    acc[key] = m if c > 0 else -m
                else:
                    acc[key] = acc[key] + m if c > 0 else acc[key] - m

        def direct(r, n, tiles, phase, split=False):
            w = jnp.concatenate([wd_s[t * 128:(t + 1) * 128, n * 128:(n + 1) * 128] for t in tiles], axis=0)
            l = htiles(r, tiles)
            if split:
                m = jnp.concatenate([_nn(l[0:hm // 2], w), _nn(l[hm // 2:], w)], axis=0)
            else:
                m = _nn(l, w)
            if phase < 3:
                fire(works[phase], m, pers[phase])
            acc[(r, n)] = m if (r, n) not in acc else acc[(r, n)] + m

        def next_phase(k):
            assert works[k] is works[k + 1] or not works[k]
            if works[k] is not works[k + 1]:
                credit[0] = 0.0

        if not gated:
            jobs = [(r, n, blk) for n in range(NJ) for r in range(2) for blk in KB]
            jobs += [(r, n, (12, 13)) for n in range(NJ) for r in range(2)]
            for i, job in enumerate(jobs):
                if i in (13, 26):
                    next_phase(i // 13 - 1)
                direct(*job, min(i // 13, 2), i == 30)
        else:
            late()
            direct(0, 2, (13,), 0)
            direct(1, 2, (13,), 3)
            for part, r in ((0, 0), (1, 0), (0, 3), (1, 3), (0, 4), (0, 5), (2, 0), (3, 0), (2, 3), (3, 3)):
                prod(part, r, 0)
            next_phase(0)
            for r in (1, 2, 6, 7, 8):
                prod(0, r, 1)
                prod(1, r, 1)
            assert all(w.func is not sum_h for w in works[1])
            next_phase(1)
            for r in range(9, 15):
                prod(0, r, 2)
            for r in (1, 2, 6, 7, 8):
                prod(2, r, 2)
                prod(3, r, 2)
            direct(0, 2, (12,), 3)
            direct(1, 2, (12,), 3)
        note(h_s, 0)
        note(hs_s, 0)
        assert not works[2]
        if not gated:
            del toks[:]
        k_s[:, 0:HALO, :] = k_s[:, tm:tm + HALO, :]
        v_s[:, 0:HALO, :] = v_s[:, tm:tm + HALO, :]
        for r in range(2):
            emit(blk, base, (r * hm, 4, acc[(r, 4)] + _nn(gate(half(a_s, r, 0, D)), _unpack(wo_p[:, 512:D]))))
        for c in range(2):
            cs = (c * 128, 256 + c * 128)

            def p(i):
                if i == 2:
                    wo = wo_p[0:128, cs[0]:cs[0] + 128]
                elif i == 5:
                    wo = wo_p[128:256, cs[1]:cs[1] + 128]
                else:
                    wo = to_s[RS[i] * 128:(RS[i] + 1) * 128, cs[0]:cs[0] + 128]
                m = _nn(lhs(a_s, 256, i), _unpack(wo))
                fire(last, m, NPDD / 9.0 + 0.01)
                return m

            def left(r, cc):
                return acc[(r, c + 2 * cc)] + _nn(half(a_s, r, 512, D), _unpack(wo_p[256:320, cs[cc]:cs[cc] + 128]))
            l21 = left(1, 0)
            m4 = p(4)
            m2 = p(2)
            c21 = l21 + m4 + m2
            m1 = p(1)
            t11 = m1 + m4
            t22 = m1 - m2
            m3 = p(3)
            m5 = p(5)
            c12 = m3 + m5 + left(0, 1)
            c11 = t11 - m5 + p(7) + left(0, 0)
            c22 = t22 + m3 + p(6) + left(1, 1)
            emit(blk, base, (hm, c, c21))
            emit(blk, base, (0, c + 2, c12))
            emit(blk, base, (0, c, c11), (hm, c + 2, c22))
        assert not last

    def step(b):
        blk = b + 1
        base = pl.multiple_of(TM0 + b * TM1, 16)
        nblk = jnp.minimum(blk + 1, NL)
        reset(1)
        side = {}

        def xt(r, k):
            return _unpack(xn_s[r * HP:(r + 1) * HP, k * 128:(k + 1) * 128])

        def xsum(i):
            return _unpack(xs_s[i * HP:(i + 1) * HP, :])

        def mm(mat, l, w):
            return (_nn if mat == 0 else _nt)(l, w)

        def tick(v):
            fire(side['work'], v, side['per'])

        def hk(mat, n0, r):
            l = xt(*HK_LP[r]) if r in HK_LP else xsum(HK_LS[r])
            if r in HK_RP:
                w = wtile(mat, HK_RP[r][0], n0 + HK_RP[r][1])
            else:
                row = t_tri(mat, n0, HK_RS[r])
                w = _unpack(t1_s[row:row + 64, :])
            return mm(mat, l, w)

        def st(mat, n0, i):
            l = xt(0, 3) if i == 3 else xt(1, 4) if i == 4 else xsum(11 + LS[i])
            if i == 2:
                w = wtile(mat, 3, n0)
            elif i == 5:
                w = wtile(mat, 4, n0 + 1)
            else:
                row = t_pair(mat, n0, RS[i])
                w = _unpack(t1_s[row:row + 64, :])
            return mm(mat, l, w)

        def add(acc, key, v):
            acc[key] = v if key not in acc else acc[key] + v

        def s_a(acc, mat, n0):
            m1, m4, m5, m7 = [st(mat, n0, i) for i in (1, 4, 5, 7)]
            add(acc, (0, n0), (m1 + m4) + (m7 - m5))
            tick(acc[(0, n0)])
            add(acc, (1, n0 + 1), m1)
            add(acc, (1, n0), m4)
            add(acc, (0, n0 + 1), m5)

        def s_b(acc, mat, n0):
            m2, m3, m6 = [st(mat, n0, i) for i in (2, 3, 6)]
            add(acc, (1, n0), m2)
            add(acc, (0, n0 + 1), m3)
            add(acc, (1, n0 + 1), (m3 - m2) + m6)
            tick(acc[(1, n0 + 1)])

        def h_a(acc, mat, n0):
            r0, r9, r11, r10 = [hk(mat, n0, r) for r in (0, 9, 11, 10)]
            t = r9 + r11
            w0 = r0 + t
            add(acc, (0, n0), w0 + r10)
            tick(acc[(0, n0)])
            acc[(1, n0)] = acc[(1, n0)] - w0
            add(acc, (0, n0 + 2), t + r10)
            acc[(1, n0 + 2)] = acc[(1, n0 + 2)] - r11 if (1, n0 + 2) in acc else -r11

        def h_b(acc, mat, n0):
            r7, r6, r8, r1 = [hk(mat, n0, r) for r in (7, 6, 8, 1)]
            add(acc, (0, n0), r7)
            add(acc, (1, n0), (r1 + r6) + r8)
            tick(acc[(1, n0)])
            add(acc, (0, n0 + 1), r6 + r7)
            add(acc, (1, n0 + 1), r8)

        def h_c(acc, mat, n0):
            r3, r12, r14, r13 = [hk(mat, n0, r) for r in (3, 12, 14, 13)]
            t = r12 + r14
            w1 = r3 + t
            acc[(0, n0 + 1)] = acc[(0, n0 + 1)] - w1
            add(acc, (1, n0 + 1), w1 + r13)
            tick(acc[(1, n0 + 1)])
            acc[(0, n0 + 2)] = acc[(0, n0 + 2)] - r14
            add(acc, (1, n0 + 2), t + r13)

        def h_1(acc, mat, n0, r):
            add(acc, {2: (0, n0 + 1), 4: (0, n0 + 2), 5: (1, n0 + 2)}[r], hk(mat, n0, r))

        def group6(mat, n0, done, filler):
            acc = {}

            def fin(*keys):
                for key in keys:
                    done(key[0], key[1], acc.pop(key))
            s_a(acc, mat, n0)
            s_b(acc, mat, n0)
            h_1(acc, mat, n0, 2)
            h_a(acc, mat, n0)
            h_b(acc, mat, n0)
            fin((0, n0), (1, n0))
            h_c(acc, mat, n0)
            fin((0, n0 + 1), (1, n0 + 1))
            s_a(acc, mat, n0 + 2)
            s_b(acc, mat, n0 + 2)
            h_1(acc, mat, n0, 5)
            fin((1, n0 + 2))
            s_a(acc, mat, n0 + 4)
            s_b(acc, mat, n0 + 4)
            h_1(acc, mat, n0, 4)
            fin((0, n0 + 2))
            h_a(acc, mat, n0 + 3)
            h_b(acc, mat, n0 + 3)
            fin((0, n0 + 3), (1, n0 + 3))
            h_c(acc, mat, n0 + 3)
            fin((1, n0 + 4))
            for r in (2, 4, 5):
                h_1(acc, mat, n0 + 3, r)
            fin((0, n0 + 4), (0, n0 + 5), (1, n0 + 5))
            assert not acc
            filler()

        work = [P(ln_pair, nblk, k * LC, xn2_s, None) for k in range(HM1 // LC)]
        side.update(work=work, per=len(work) / LNSPAN)
        acc = {}
        plain = [(r, k) for k in (3, 4) for r in range(2)]

        def fill_q():
            r, k = plain.pop(0)
            add(acc, (r, 14), mm(0, xt(r, k), wtile(0, k, 14)))

        def done_q(r, n, val):
            if n in (5, 11):
                val = val * sc_s[16 * (n // 6) + 24:16 * (n // 6) + 25, :]
            store_qkv(QORD[n], r * HM1, val)

        def fin_q(*keys):
            for key in keys:
                done_q(key[0], key[1], acc.pop(key))
        group6(0, 0, done_q, fill_q)
        group6(0, 6, done_q, fill_q)
        s_a(acc, 0, 12)
        s_b(acc, 0, 12)
        h_1(acc, 0, 12, 2)
        h_a(acc, 0, 12)
        h_b(acc, 0, 12)
        fin_q((0, 12), (1, 12))
        h_c(acc, 0, 12)
        fin_q((0, 13), (1, 13))
        h_1(acc, 0, 12, 4)
        h_1(acc, 0, 12, 5)
        fill_q()
        fill_q()
        fin_q((0, 14), (1, 14))
        assert not work and not acc

        work = [P(attn_rows, c * RC, False) for c in range(TM1 // RC)]
        side.update(work=work, per=APER)
        credit[0] = AOFF

        def store_h(r, n, v):
            h_s[r * HP:(r + 1) * HP, n * 128:(n + 1) * 128] = _pack(v)

        s_a(acc, 3, 0)
        s_b(acc, 3, 0)
        h_1(acc, 3, 0, 2)
        h_a(acc, 3, 0)
        h_b(acc, 3, 0)
        for r in range(2):
            store_h(r, 13, tail_h(acc.pop((r, 0))) * sc_s[8:9, :])
        h_c(acc, 3, 0)
        for r in range(2):
            hold_s[(12 + r) * HM1:(13 + r) * HM1, :] = _gelu(acc.pop((r, 1))) * sc_s[8:9, :]
        plain = [(r, k) for r in range(2) for k in (3, 4)]

        def fill_g():
            r, k = plain.pop(0)
            l = xt(r, k)
            add(acc, (r, 2), mm(3, gate(l) if len(plain) == 3 else l, wtile(3, k, 2)))

        def late():
            for r in range(2):
                h_1(acc, 3, 0, 4 + r)
                store_h(r, 12, hold_s[(12 + r) * HM1:(13 + r) * HM1, :] * acc.pop((r, 2)))
        for n0 in (0, 6):
            def slot(r, n):
                s = (n - n0) * 2 + r
                return slice(s * HM1, (s + 1) * HM1)

            def early(r, n):
                return (GPAT >> ((n - n0) * 2 + r)) & 1

            def done_g(r, n, v):
                hold_s[slot(r, n), :] = _gelu(v) if early(r, n) else v

            def done_u(r, n, v):
                g = hold_s[slot(r, n), :]
                store_h(r, n, (g if early(r, n) else _gelu(g)) * v)
            if n0 == 6:
                n_att = int(24 * APER)
                work[:] = _weave(work[:n_att], sum_items(HP, 0)) + work[n_att:]
                side.update(per=(n_att + 3 * HP // 8) / 24.0)
            group6(1, n0, done_g, fill_g)
            group6(2, n0, done_u, fill_g)
        assert not plain
        note(hold_s, 0)

        def move_xn(r0, part, trig):
            ks = ((0, 1, 2), (3, 4))[part]
            xy = []
            for r in range(2):
                row = r * HP + r0
                u = {k: after(xn2_s[row:row + 8, k * 128:(k + 1) * 128], trig) for k in ks}
                for k in ks:
                    xn_s[row:row + 8, k * 128:(k + 1) * 128] = u[k]
                xy.append({k: _unpack(u[k]).astype(F32) for k in ks})
            x, y = xy
            sums = _hk_lhs_sums(x, y) if part == 0 else _lhs_sums(x[3], x[4], y[3], y[4])
            for i, s in enumerate(sums):
                row = (i + 11 * part) * HP + r0
                xs_s[row:row + 8, :] = _pack(s)
            if part == 0:
                note(xn_s, r0)
                note(xs_s, r0)
        copies = [P(move_xn, r0, part) for r0 in range(0, HP, 8) for part in range(2)]
        sums = [w for w in work if w.func is sum_h] + sum_items(HP, 1)
        work = [w for w in work if w.func is not sum_h]
        s12 = [w for w in sums if w.args[1:3] == (1, 2)]
        w0 = _weave([w for w in sums if w.args[1:3] != (1, 2)], work[:NA0])
        w1 = _weave(work[NA0:], s12 + copies)
        credit[0] = 0.0
        stage2(blk, base, TM1, [w0, w1, w1], [len(w0) / SPAN0, len(w1) / A2SPAN, len(w1) / A2SPAN], True, late)

    def cp(src, dst, s):
        return pltpu.make_async_copy(src, dst, sem_i.at[s])

    def gu(groups, s):
        return [cp(h.at[pl.ds(g * 128, 128)], d.at[pl.ds(g * 128, 128)], s)
                for g in groups for h, d in ((wg_hbm, wg_s), (wu_hbm, wu_s))]

    def wcol(t, s):
        return cp(wqkv_hbm.at[:, pl.ds(t * D, D)], wqkv_r.at[:, pl.ds(t * D, D)], s)

    def xblk(b, s):
        return cp(x_hbm.at[pl.ds(TM0 + b * TM1, TM1)], x_s.at[b + 1, pl.ds(0, TM1)], s)

    HM = TM0 // 2
    cp_x0 = [cp(x_hbm.at[pl.ds(i * HM, HM)], x_s.at[0, pl.ds(i * HM, HM)], i) for i in range(2)]
    cp_gu = [gu(g, 2 + k) for k, g in enumerate(G_EARLY)]
    cp_q = gu(G_Q, 5) + [cp(wg_hbm.at[pl.ds(FM, 64)], wt_s.at[pl.ds(0, 64)], 5),
                         cp(wu_hbm.at[pl.ds(FM, 64)], wt_s.at[pl.ds(64, 64)], 5), wcol(0, 5), xblk(0, 5)]
    cp_kv = gu(G_KV, 6) + [wcol(1, 6), wcol(2, 6)]
    cp_r = gu(G_R + G_D, 7) + [cp(wo_hbm, wo_r, 7)]
    cp_d = [cp(wd_hbm, wd_s.at[pl.ds(0, F)], 8)]
    cp_xs = [xblk(b, 9) for b in range(1, NL)]

    for c in cp_x0 + sum(cp_gu, []) + cp_q + cp_kv + cp_r + cp_d + cp_xs:
        c.start()
    zero_s[0] = 0
    k_s[:, 0:HALO, :] = jnp.zeros((NJ, HALO, 128), F32)
    v_s[:, 0:HALO, :] = jnp.zeros((NJ, HALO, 128), F32)
    wd_s[F:FP, :] = jnp.zeros((FP - F, D), BF)

    def first_block():
        def wait(cps):
            reset(CH0)
            for c in cps:
                c.wait()

        parts = []
        for i in range(2):
            wait(cp_x0[i:i + 1])
            parts += [ln_rows(0, i * HM + k * LC).astype(BF) for k in range(HM // LC)]
        xn = jnp.concatenate(parts, axis=0)

        def ffn_group(x, row0, g0, work, per):
            g = _nt(x, wg_s[g0 * 128:(g0 + 1) * 128, :])
            fire(work, g, per)
            u = _nt(x, wu_s[g0 * 128:(g0 + 1) * 128, :])
            fire(work, u, per)
            h_s[row0 // 2:(row0 + x.shape[0]) // 2, g0 * 128:(g0 + 1) * 128] = _pack(_gelu(g) * u)

        def ffn_groups(groups, work, per):
            groups = list(groups)
            if len(groups) % 2:
                g0 = groups.pop(0)
                ffn_group(xn[0:HM], 0, g0, work, per)
                ffn_group(xn[HM:], HM, g0, work, per)
            for g0 in groups:
                ffn_group(xn, 0, g0, work, per)

        have, done = set(), set()

        def new_preps(groups):
            have.update(groups)
            tris = [n for n in (0, 3, 6, 9) if {n, n + 1, n + 2} <= have and ('t', n) not in done]
            pairs = [n for n in range(0, 12, 2) if {n, n + 1} <= have and ('p', n) not in done]
            done.update([('t', n) for n in tris] + [('p', n) for n in pairs])
            return preps(1, tris, pairs) + preps(2, tris, pairs)

        perm = [[P(permute_qkv, t, r0) for r0 in range(0, D, 64)] for t in range(3)]

        for cps, groups in zip(cp_gu, G_EARLY):
            wait(cps)
            work = new_preps(groups)
            nres = 2 * len(groups) + 2 * (len(groups) % 2)
            ffn_groups(groups, work, max(len(work), 1) / (nres - ESLACK))
            assert not work

        wait(cp_q)
        work = perm[0]
        for _ in range(3):
            work.pop(0)(None)
        t = _nt(xn, wt_s[...])
        fire(work, t, 4)
        h_s[0:TM0 // 2, FM:FP] = _pack(tail_h(t))
        work += new_preps(G_Q) + [P(ln_pair, 1, k * LC, xn_s, xs_s) for k in range(HM1 // LC)]
        for g0 in G_Q:
            ffn_group(xn, 0, g0, work, QPER)
        assert all(w.func is ln_pair for w in work)
        per = len(work) / QSPAN
        for j in range(NJ):
            r = _nn(xn, _unpack(wqkv_p[:, j * 128:(j + 1) * 128]))
            fire(work, r, per)
            store_qkv(j, 0, r)
        assert not work

        wait(cp_kv)
        work = perm[1]
        for _ in range(4):
            work.pop(0)(None)
        for g0 in G_KV:
            g = _nt(xn, wg_s[g0 * 128:(g0 + 1) * 128, :])
            fire(work, g, 6)
            u = _nt(xn, wu_s[g0 * 128:(g0 + 1) * 128, :])
            h_s[0:TM0 // 2, g0 * 128:(g0 + 1) * 128] = _pack(_gelu(g) * u)
        assert not work
        scan, scale = balance_k()
        free = _weave(new_preps(G_KV), preps(0, (0, 12, 6), []), preps(0, [], (0, 2, 12, 6, 8)))
        work = (perm[2][:2] + scan + perm[2][2:]
                + _weave(free, scale + _weave(preps(0, (3, 9), []), preps(0, [], (4, 10)))))
        spill, work = work[len(work) - KLATE:], work[:len(work) - KLATE]
        per = len(work) / KVSPAN
        fire(work, u, per)
        for c in range(NJ, 3 * NJ):
            assert c < 2 * NJ or all(w.func is not permute_qkv for w in work)
            r = _nn(xn, _unpack(wqkv_p[:, c * 128:(c + 1) * 128]))
            fire(work, r, per)
            store_qkv(c, 0, r)
        assert not work

        wait(cp_r)
        att = [P(attn_rows, rc * RC, True) for rc in range(TM0 // RC)]
        scan, scale = balance_items()
        free = _weave(new_preps(G_R + G_D), att[:NAR])
        work = scan + free[:RFREE] + _weave(free[RFREE:], scale + preps(3, [0], [0]))
        att = att[NAR:]
        ffn_groups(G_R, work, len(work) / RSPAN)
        assert not work

        wait(cp_d)
        chain[0] = CHD
        wo_work = []
        for jj in range(NJ):
            wo_work += [P(widen_wo, jj, r0) for r0 in range(0, D, UW)]
            wo_work += [P(gather_wo, jj, j) for j in range(NJ)]
        pd = [P(prep_d, part, o, r0) for part, no in ((0, 4), (1, 4), (2, 3), (3, 1)) for o in range(no)
              for r0 in range(0, 128, UD)]
        po = [P(prep_o, r0, c) for r0 in range(0, 128, UD // 2) for c in (0, 128)]
        wa = _weave(*[l for l in (wo_work, pd[:NPDA], att[:NAA]) if l])
        pd += spill
        wd_ = pd[len(pd) - NPDD:]
        pd = pd[:len(pd) - NPDD]
        wb = _weave(*[l for l in (pd[NPDA:NPDA + NPDB], po, att[NAA:NAA + NAB]) if l])
        wc = _weave(*[l for l in (pd[NPDA + NPDB:], att[NAA + NAB:]) if l])
        per = len(wa) / SPANA
        ffn_groups(G_D, wa, per)
        stage2(0, 0, TM0, [wa, wb, wc], [per, len(wb) / SPANB, max(len(wc), 1) / SPANC], False, None, wd_)

    def main(i, carry):
        first_block()
        for c in cp_xs:
            c.wait()

        def body(b, c):
            step(b)
            return c
        return jax.lax.fori_loop(0, NL, body, carry)

    jax.lax.fori_loop(0, zero_s[0] + 1, main, 0)

    for j in range(NJ):
        for r in range(2):
            cp_o(0, 0, r * HM, HM, j).wait()
    for b in range(NL):
        for j in range(NJ):
            for r in range(2):
                cp_o(b + 1, TM0 + b * TM1, r * HM1, HM1, j).wait()


@jax.jit
def pallas_parallel_sum__sliding_local_dilated__geglu_ffn__prompt_kernel(
    A_x: jax.Array,
    A_wqkv: jax.Array,
    A_wo: jax.Array,
    B_x: jax.Array,
    B_w_gate: jax.Array,
    B_w_up: jax.Array,
    B_w_down: jax.Array,
):
    x = A_x.reshape(S, D)
    hbm = pl.BlockSpec(memory_space=pltpu.MemorySpace.HBM)
    out = pl.pallas_call(
        _kernel,
        in_specs=[hbm] * 6,
        out_specs=hbm,
        out_shape=jax.ShapeDtypeStruct((S, D), BF),
        scratch_shapes=[
            pltpu.VMEM((NL + 1, TMP, D), BF),
            pltpu.VMEM((TM1 // 2, D), U32),
            pltpu.VMEM((NSUM * HP, 128), U32),
            pltpu.VMEM((TM1 // 2, D), U32),
            pltpu.VMEM((NL + 1, TMP, D), BF),
            pltpu.VMEM((D, 3 * D), BF),
            pltpu.VMEM((D // 2, 3 * D), U32),
            pltpu.VMEM((D, D), BF),
            pltpu.VMEM((NJ * D, 128), F32),
            pltpu.VMEM((D // 2, D), U32),
            pltpu.VMEM((FM, D), BF),
            pltpu.VMEM((FM, D), BF),
            pltpu.VMEM((128, D), BF),
            pltpu.VMEM((FP, D), BF),
            pltpu.VMEM((226 * 64, 128), U32),
            pltpu.VMEM((76 * 64, 128), U32),
            pltpu.VMEM((5 * 128, 256), U32),
            pltpu.VMEM((NJ, TMX, 128), F32),
            pltpu.VMEM((NJ, TMX + HALO, 128), F32),
            pltpu.VMEM((NJ, TMX + HALO, 128), F32),
            pltpu.VMEM((TMX // 2, FP), U32),
            pltpu.VMEM((NSUM * TMX // 4, 512), U32),
            pltpu.VMEM((TMX // 2, D), U32),
            pltpu.VMEM((NHOLD * HM1, 128), F32),
            pltpu.VMEM((128, D), U32),
            pltpu.VMEM((D // 2, 256), U32),
            pltpu.VMEM((48, 128), F32),
            pltpu.SMEM((1,), jnp.int32),
            pltpu.SemaphoreType.DMA((10,)),
            pltpu.SemaphoreType.DMA((1,)),
        ],
        compiler_params=pltpu.CompilerParams(
            vmem_limit_bytes=100 * 1024 * 1024,
            disable_bounds_checks=True,
            disable_semaphore_checks=True,
        ),
    )(x, A_wqkv, A_wo, B_w_gate.T, B_w_up.T, B_w_down)
    return out.reshape(1, S, D)
```
